```python
import jax
import jax.numpy as jnp

def _softmax(x, axis=-1):
    return jax.nn.softmax(x, axis=axis)
def _gelu(x):
    return jax.nn.gelu(x, approximate=True)
def _silu(x):
    return jax.nn.silu(x)
def _sigmoid(x):
    return jax.nn.sigmoid(x)
def _layernorm(x, axis=-1, eps=1e-5):
    m = jnp.mean(x, axis=axis, keepdims=True)
    v = jnp.var(x, axis=axis, keepdims=True)
    return (x - m) / jnp.sqrt(v + eps)
def _scatter_add(tgt, idx, src, axis=0):
    return tgt.at[idx].add(src)
def _segment_sum(src, seg, n):
    return jax.ops.segment_sum(src, seg, n)
class _Rng:
    def __init__(self, key):
        self._k = key
    def _next(self):
        self._k, sub = jax.random.split(self._k)
        return sub
    def normal(self, shape):
        return jax.random.normal(self._next(), shape, dtype=jnp.bfloat16)
    def randint(self, lo, hi, shape):
        return jax.random.randint(self._next(), shape, lo, hi, dtype=jnp.int32)
    def uniform(self, shape, lo=0.0, hi=1.0):
        return jax.random.uniform(self._next(), shape, jnp.bfloat16, lo, hi)
    def permutation(self, n):
        return jax.random.permutation(self._next(), n)


kernel_name = 'recurrent_scan__ssm_conv_s4__moe_arch_mod__prompt'

def setup_inputs():
    _rng = _Rng(jax.random.key(int.from_bytes(__import__("os").urandom(4), "little")))
    _w = (lambda a: (lambda t: t.astype(jnp.bfloat16) if jnp.issubdtype(t.dtype, jnp.floating) else t)(jnp.asarray(a)))
    def _A_setup():
        B, L, D, N = 1, 2048, 576, 128
        A_re = -jnp.exp((lambda *s: _rng.normal(s) * 0.05)(D, N))
        A_im = jnp.pi * (lambda *s: _rng.normal(s) * 0.05)(D, N)
        B_re = (lambda *s: _rng.normal(s) * 0.05)(D, N)
        B_im = (lambda *s: _rng.normal(s) * 0.05)(D, N)
        C_re = (lambda *s: _rng.normal(s) * 0.05)(D, N)
        C_im = (lambda *s: _rng.normal(s) * 0.05)(D, N)
        log_dt = (lambda *s: _rng.normal(s) * 0.05)(D) * 0.5 - 4.0
        Dskip = (lambda *s: _rng.normal(s) * 0.05)(D)
        return {
            "u": _w((lambda *s: _rng.normal(s) * 0.05)(B, L, D)),
            "A_re": _w(A_re),
            "A_im": _w(A_im),
            "B_re": _w(B_re),
            "B_im": _w(B_im),
            "C_re": _w(C_re),
            "C_im": _w(C_im),
            "log_dt": _w(log_dt),
            "Dskip": _w(Dskip),
        }
    _A_in = _A_setup()

    def _B_setup():
        B, S, D, F, C = 1, 2048, 576, 4608, 8
        return {
            "x": _w((lambda *s: _rng.normal(s) * 0.05)(B, S, D)),
            "w_r": _w((lambda *s: _rng.normal(s) * 0.05)(D)),
            "w_gate": _w((lambda *s: _rng.normal(s) * 0.05)(D, F)),
            "w_up": _w((lambda *s: _rng.normal(s) * 0.05)(D, F)),
            "w_down": _w((lambda *s: _rng.normal(s) * 0.05)(F, D)),
        }
    _B_in = _B_setup()

    return {
        "A_u": _A_in["u"],
        "A_A_re": _A_in["A_re"],
        "A_A_im": _A_in["A_im"],
        "A_B_re": _A_in["B_re"],
        "A_B_im": _A_in["B_im"],
        "A_C_re": _A_in["C_re"],
        "A_C_im": _A_in["C_im"],
        "A_log_dt": _A_in["log_dt"],
        "A_Dskip": _A_in["Dskip"],
        "B_x": _B_in["x"],
        "B_w_r": _B_in["w_r"],
        "B_w_gate": _B_in["w_gate"],
        "B_w_up": _B_in["w_up"],
        "B_w_down": _B_in["w_down"],
    }

def reference(A_u, A_A_re, A_A_im, A_B_re, A_B_im, A_C_re, A_C_im, A_log_dt, A_Dskip, B_x, B_w_r, B_w_gate, B_w_up, B_w_down):
    def _A_ref(u, A_re, A_im, B_re, B_im, C_re, C_im, log_dt, Dskip):
        Bsz, L, D = u.shape
        dt = jnp.exp(log_dt)[:, None]
        A = A_re + 1j * A_im
        Bc = B_re + 1j * B_im
        Cc = C_re + 1j * C_im
        logdA = dt * A
        dB = dt * Bc
        l = (lambda x, dt: x.astype(dt))(jnp.arange(L), A_re.dtype)
        P = jnp.exp(logdA[:, :, None] * l[None, None, :])
        K = jnp.einsum("dn,dnl,dn->dl", Cc, P, dB).real
        L2 = 2 * L
        Kp = jnp.pad(K, ((0, 0), (0, L)))
        up = (lambda x, *d: x.transpose(*d))(u, 0, 2, 1)
        up = jnp.pad(up, ((0, 0), (0, 0), (0, L)))
        Kf = (lambda x, axes=(-2,-1): jnp.fft.rfft2(x.astype(jnp.float32), axes=axes))(Kp[:, None, :], axes=(-2, -1))
        Uf = (lambda x, axes=(-2,-1): jnp.fft.rfft2(x.astype(jnp.float32), axes=axes))(up[:, :, None, :], axes=(-2, -1))
        Yf = Uf * Kf[None, :, :, :]
        y = (lambda x, s, axes=(-2,-1): jnp.fft.irfft2(x, s=s, axes=axes).astype(jnp.bfloat16))(Yf, (1, L2), axes=(-2, -1))[:, :, 0, :L]
        y = (lambda x, *d: x.transpose(*d))(y, 0, 2, 1) + u * Dskip[None, None, :]
        return y

    def _B_ref(x, w_r, w_gate, w_up, w_down):
        B, S, D = x.shape
        C = 8
        r = x @ w_r
        idx = jnp.argsort(-r, axis=-1)[:, :C]
        idx_e = jnp.repeat(idx.reshape(B, C, 1), D, axis=2)
        x_sel = jnp.take_along_axis(x, idx_e, axis=1)
        g = _silu(x_sel @ w_gate)
        u = x_sel @ w_up
        y = (g * u) @ w_down
        r_sel = _sigmoid(jnp.take_along_axis(r, idx, axis=1))
        y = y * r_sel.reshape(B, C, 1)
        b_off = (jnp.arange(B) * S).reshape(B, 1)
        flat_idx = (idx + b_off).reshape(B * C)
        zero = (x * 0.0).reshape(B * S, D)
        upd = _scatter_add(zero, flat_idx, y.reshape(B * C, D), axis=0)
        return x + upd.reshape(B, S, D)

    x = A_u
    xn = _layernorm(x, axis=-1)
    s = _A_ref(xn, A_A_re, A_A_im, A_B_re, A_B_im, A_C_re, A_C_im, A_log_dt, A_Dskip)
    g = _silu(_B_ref(xn, B_w_r, B_w_gate, B_w_up, B_w_down))
    return x + s * g
```

```python
import jax
import jax.numpy as jnp
import numpy as np
import jax.experimental.pallas as pl
import jax.experimental.pallas.tpu as pltpu

F32, BF16, I32, U32 = jnp.float32, jnp.bfloat16, jnp.int32, jnp.uint32

L, D, N, F = 2048, 576, 128, 4608
TOPC = 8
BLK = 512
CB = 64
NCB = D // CB
FB = F // NCB
NT = (((1,), (1,)), ((), ()))
TN = (((0,), (0,)), ((), ()))


def _round_to_bf16(v):
    u = np.asarray(v, np.float32).view(np.uint32)
    return ((u + 0x7FFF + ((u >> 16) & 1)) & 0xFFFF0000).astype(np.uint32).view(np.float32)


def _transform_tables():
    lag_exp = _round_to_bf16(np.arange(L + 1)).astype(np.int64)
    c = np.arange(128)
    kk = np.arange(BLK)

    def root(k, t):
        return np.exp(1j * np.pi * ((4 * k + 1) * t % (4 * BLK)) / (2 * BLK))

    def reim(z):
        z = z.reshape(z.shape[0], -1, 1, 128)
        return np.concatenate([z.real, z.imag], axis=2).reshape(z.shape[0], -1)

    def grp(qs):
        return np.concatenate([q + 8 * np.arange(32) for q in qs])

    def seg(e, m):
        l = np.arange(BLK * m + 1, min(BLK * m + BLK + 1, L))
        l = l[lag_exp[l] == e]
        return root(kk[None, :], (l - BLK * m)[:, None]).sum(0)

    tu = [128 * ((c - ph) % 4) + (c - (c - ph) % 4) % 128 for ph in range(4)]
    g4, g2, go = grp([4, 8, 260, 264]), grp([2, 6, 258, 262]), grp([3, 7, 1, 5])
    gc, gd = grp([516, 520, 772, 776]), grp([1032, 1288, 1544, 1800])
    t1 = np.where((c >= 63) & (c < 127), g4 + 1, np.roll(go, 63))
    t3 = np.where(c < 64, go, g4 - 1)
    tabs = [np.concatenate([reim(root(c[None, :], t[:, None])) for t in ts], axis=1)
            for ts in (tu, (g4, t1, g2, t3))]
    tabs.append(reim(np.stack([seg(e, 1) for e in gc])))
    tabs.append(reim(np.stack([seg(e, 2) for e in np.where(c < 64, gd, gc)])))
    tabs.append(reim(np.stack([seg(e, 3) for e in gd])))
    edge = np.repeat(reim(seg(512, 1)[None, :]), 8, axis=0)
    return np.stack(tabs).astype(np.float32), edge.astype(np.float32)


def _cmul(a, b):
    return a[0] * b[0] - a[1] * b[1], a[0] * b[1] + a[1] * b[0]


def _csq(a):
    return (a[0] + a[1]) * (a[0] - a[1]), (a[0] + a[0]) * a[1]


def _cadd(a, b):
    return a[0] + b[0], a[1] + b[1]


def _csub(a, b):
    return a[0] - b[0], a[1] - b[1]


def _add_i(a, b):
    return a[0] - b[1], a[1] + b[0]


def _sub_i(a, b):
    return a[0] + b[1], a[1] - b[0]


def _radix4(f, inverse=False):
    a, b, c, d = _cadd(f[0], f[2]), _csub(f[0], f[2]), _cadd(f[1], f[3]), _csub(f[1], f[3])
    p, m = (_sub_i, _add_i) if inverse else (_add_i, _sub_i)
    return [_cadd(a, c), p(b, d), _csub(a, c), m(b, d)]


def _lane_exchange(r, bit0, bit1):
    a = [jnp.where(bit0, r[(j + 1) % 4], r[j]) for j in range(4)]
    b = [jnp.where(bit1, a[(j + 2) % 4], a[j]) for j in range(4)]
    return [b[-j % 4] for j in range(4)]


def _rb(v):
    return v.astype(BF16).astype(F32)


def _silu(v):
    h = 0.5 * v
    return h + h * jnp.tanh(h)


def _ssm_values(par, dt):
    a_re, a_im, b_re, b_im, c_re, c_im = par
    sub = jax.lax.broadcasted_iota(I32, (8, 128), 0)
    lane = jax.lax.broadcasted_iota(I32, (8, 128), 1)
    lo = sub < 4
    cls = (lane - sub) & 3
    perm = (4 * (lane & 31) + (sub & 3) + (lane >> 5)) & 127

    def half_roll(v):
        return pltpu.roll(v, 4, 0)

    def dup(z):
        r = [half_roll(v) for v in z]
        return (tuple(jnp.where(lo, v, s) for v, s in zip(z, r)),
                tuple(jnp.where(lo, s, v) for v, s in zip(z, r)))

    def pair(x, y):
        r = [half_roll(v) for v in y]
        return (tuple(jnp.where(lo, v, s) for v, s in zip(x, r)),
                tuple(jnp.where(lo, s, v) for v, s in zip(x, r)))

    mag = jnp.exp(dt * a_re)
    ang = dt * a_im
    pw = {1: (mag * jnp.cos(ang), mag * jnp.sin(ang))}
    for k in range(10):
        pw[2 << k] = _csq(pw[1 << k])
    cb = _cmul((c_re, c_im), (b_re, b_im))
    k0 = jnp.sum(cb[0] * dt, axis=1, keepdims=True)
    sc = dt * (1.0 / BLK)
    w1 = _cmul((cb[0] * sc, cb[1] * sc), pw[1])
    w5 = _cmul(w1, pw[4])
    w1032 = _cmul(_cmul((cb[0] * sc, cb[1] * sc), pw[8]), pw[1024])

    p_seed = [(jnp.where(lo, 1.0, z[0]), jnp.where(lo, 0.0, -z[1])) for z in dup(pw[8])]
    p_step = dup((pw[16][0], -pw[16][1]))
    q_seed = pair(w1, w5)
    q_far = pair(w1032, _cmul(w1032, pw[256]))
    s1, s256, s512 = dup(pw[1]), dup(pw[256]), dup(pw[512])

    def stack(zs):
        return jnp.concatenate(
            [jnp.concatenate([z[j] for z in zs], axis=0).astype(BF16) for j in range(2)], axis=1)

    outs = []
    for h in range(2):
        p = [p_seed[h]]
        for _ in range(15):
            p.append(_cmul(p[-1], p_step[h]))
        q = [q_seed[h]]
        for _ in range(3):
            q.append(_cmul(q[-1], s1[h]))
        q.append(_cmul(q[1], s256[h]))
        q.append(_cmul(q[3], s256[h]))
        q.append(_cmul(q[5], s256[h]))
        q.append(_cmul(q[6], s256[h]))
        q.append(q_far[h])
        q.append(_cmul(q[8], s512[h]))
        outs.append(jax.lax.dot_general(stack(q), stack(p), NT, preferred_element_type=F32))

    def compact(v0, v1):
        o = [[outs[h][8 * v:8 * v + 8] for h in range(2)] for v in (v0, v1)]
        first = [jnp.where(lo, t[0], t[1]) for t in o]
        second = [jnp.where(lo, t[1], t[0]) for t in o]
        e = jnp.where(cls == 0, first[0], pltpu.roll(first[1], 2, 1))
        f = jnp.where(cls == 0, second[0], pltpu.roll(second[1], 2, 1))
        u = jnp.where((cls & 1) == 1, pltpu.roll(half_roll(f), 1, 1), e)
        return jnp.take_along_axis(u, perm, axis=1)

    g4, g2, go, gc, gd = compact(3, 5), compact(1, 4), compact(2, 0), compact(6, 7), compact(8, 9)
    v1 = jnp.where((lane >= 63) & (lane < 127), g4, pltpu.roll(go, 63, 1))
    v3 = jnp.where(lane < 64, go, g4)
    ve = jnp.where(lane < 64, gd, gc)
    k512 = jnp.sum(jnp.where(lane == 127, g4, 0.0), axis=1, keepdims=True)
    return [g4, v1, g2, v3, gc, ve, gd], k0, k512


def _block_conv(kf, k512, edge, uf):
    k = [_radix4(kf[0]),
         [(z[0] + k512 * e[0], z[1] + k512 * e[1]) for z, e in zip(kf[1], edge)],
         kf[2], kf[3]]
    u = [_radix4(f) for f in uf]
    z = [[None] * 4 for _ in range(4)]
    for s in range(4):
        kp = [k[0][s]] + [_sub_i(k[m][s], k[m - 1][s]) for m in (1, 2, 3)]
        kt = [(c, d - c, c + d) for c, d in kp]
        ut = [(u[m][s][0] + u[m][s][1], u[m][s][0], u[m][s][1]) for m in range(4)]
        for i in range(4):
            acc = [kt[0][j] * ut[i][j] for j in range(3)]
            for m in range(1, i + 1):
                acc = [acc[j] + kt[m][j] * ut[i - m][j] for j in range(3)]
            z[i][s] = (acc[0] - acc[2], acc[0] + acc[1])
    return [_radix4(zi, inverse=True) for zi in z]


def _kernel(x_hbm, are_hbm, aim_hbm, bre_hbm, bim_hbm, cre_hbm, cim_hbm, ldt_hbm, dsk_hbm, wr_hbm,
            wg_hbm, wu_hbm, wd_hbm, tab_hbm, edge_hbm, o_hbm,
            x_v, par_v, ldt_v, dsk_v, wr_v, wg_v, wu_v, wd_v, tab_v, edge_v, o_v,
            xn_v, s_v, dt_v, skip_v, k512_v, kvec_v, kf_v, h_v, hot_v,
            sem_in, sem_g, sem_u, sem_d, sem_o):
    small = [(ldt_hbm, ldt_v), (dsk_hbm, dsk_v), (wr_hbm, wr_v)]
    small += [(p, par_v.at[j]) for j, p in
              enumerate((are_hbm, aim_hbm, bre_hbm, bim_hbm, cre_hbm, cim_hbm))]
    small += [(tab_hbm, tab_v), (edge_hbm, edge_v), (x_hbm, x_v)]
    cp_in = [pltpu.make_async_copy(s, d, sem_in.at[j]) for j, (s, d) in enumerate(small)]

    def rows(i):
        return pl.ds(i * CB if isinstance(i, int) else pl.multiple_of(i * CB, CB), CB)

    def cols(i):
        return pl.ds(i * FB if isinstance(i, int) else pl.multiple_of(i * FB, FB), FB)

    def cp_g(i):
        return pltpu.make_async_copy(wg_hbm.at[:, cols(i)], wg_v.at[i], sem_g.at[i])

    def cp_u(i):
        return pltpu.make_async_copy(wu_hbm.at[:, cols(i)], wu_v.at[i], sem_u.at[i])

    def cp_d(i):
        return pltpu.make_async_copy(wd_hbm.at[rows(i)], wd_v.at[rows(i)], sem_d.at[i])

    def cp_o(i):
        return pltpu.make_async_copy(o_v.at[rows(i)], o_hbm.at[rows(i)], sem_o.at[i])

    for c in cp_in:
        c.start()
    for i in range(NCB):
        cp_g(i).start()
        cp_u(i).start()
    for i in range(NCB):
        cp_d(i).start()

    for c in cp_in[:3]:
        c.wait()
    dt_row = _rb(jnp.exp(ldt_v[...].astype(F32).reshape(1, D)))
    dt_v[...] = jnp.broadcast_to(dt_row, (128, D)).T
    skip_v[...] = jnp.broadcast_to(dsk_v[...].astype(F32).reshape(1, D), (128, D)).T
    for c in cp_in[3:11]:
        c.wait()

    @pl.loop(0, NCB)
    def _(i):
        for j in range(CB // 16):
            r = pl.ds(pl.multiple_of(i * CB + 16 * j, 16), 16)
            par = [par_v[t, r, :].astype(F32) for t in range(6)]
            dt = dt_v[r, :]
            res = [_ssm_values([p[8 * g:8 * g + 8] for p in par], dt[8 * g:8 * g + 8])
                   for g in range(2)]
            for t in range(7):
                kvec_v[t, 16 * j:16 * j + 16, :] = jnp.concatenate(
                    [res[0][0][t], res[1][0][t]], axis=0).astype(BF16)
            skip_v[r, :] = skip_v[r, :] + jnp.concatenate([res[0][1], res[1][1]], axis=0)
            k512_v[r, :] = jnp.broadcast_to(
                jnp.concatenate([res[0][2], res[1][2]], axis=0), (16, 128))
        for t in range(4):
            kf_v[rows(i), 256 * t:256 * t + 256] = jnp.dot(
                kvec_v[t], tab_v[1, :, 256 * t:256 * t + 256], preferred_element_type=F32)
        for m in (1, 2, 3):
            kf_v[rows(i), 1024 * m:1024 * m + 1024] = jnp.dot(
                kvec_v[3 + m], tab_v[1 + m], preferred_element_type=F32)

    cp_in[11].wait()
    wr = jnp.broadcast_to(wr_v[...].astype(F32).reshape(1, D), (TOPC, D)).astype(BF16)
    ones = jnp.ones((8, D), BF16)
    eps = float(_round_to_bf16(1e-5))
    mean = jnp.dot(ones, x_v[...], preferred_element_type=F32) / D
    for t in range(L // 128):
        ts = slice(128 * t, 128 * t + 128)
        m = mean[0:1, ts]
        mb = _rb(m)
        d = x_v[:, ts].astype(F32) - mb
        var = jnp.sum(d * d, axis=0, keepdims=True) / D - (m - mb) * (m - mb)
        inv = 1.0 / _rb(jnp.sqrt(_rb(_rb(jnp.maximum(var, 0.0)) + eps)))
        xn_v[:, ts] = (_rb(d) * inv).astype(BF16)
    score = _rb(jnp.dot(wr, xn_v[...], preferred_element_type=F32))

    bits = pltpu.bitcast(jnp.where(score == 0.0, 0.0, score), I32) >> 16
    pos = jax.lax.broadcasted_iota(I32, (TOPC, L), 1)
    key = ((bits ^ ((bits >> 15) & 0x7FFF)) << 11) + (0x38000000 + L - 1 - pos)
    key = pltpu.bitcast(key, F32)
    sub = jax.lax.broadcasted_iota(I32, (TOPC, 128), 0)
    dense = []
    for half in range(2):
        v = key[:, 1024 * half:1024 * half + 128]
        for t in range(1, 8):
            v = jnp.where(sub == t, key[:, 1024 * half + 128 * t:1024 * half + 128 * t + 128], v)
        dense.append(v)
    top = jnp.zeros((TOPC, 128), F32)
    for c in range(TOPC):
        best = jnp.max(jnp.max(jnp.maximum(dense[0], dense[1]), axis=0, keepdims=True),
                       axis=1, keepdims=True)
        top = jnp.where(sub == c, best, top)
        dense = [jnp.where(v == best, 0.0, v) for v in dense]
    hot = jnp.where(key == jnp.tile(top, (1, L // 128)), 1.0, 0.0)
    hot_v[...] = hot
    tb = (pltpu.bitcast(top, I32) - 0x38000000) >> 11
    gate = _rb(jax.nn.sigmoid(pltpu.bitcast((tb ^ ((tb >> 15) & 0x7FFF)) << 16, F32)))
    xs = jax.lax.dot_general(hot.astype(BF16), xn_v[...], NT,
                             preferred_element_type=F32).astype(BF16)

    @pl.loop(0, NCB)
    def _(i):
        cp_g(i).wait()
        cp_u(i).wait()
        g = _rb(jnp.dot(xs, wg_v[i], preferred_element_type=F32))
        u = _rb(jnp.dot(xs, wu_v[i], preferred_element_type=F32))
        h_v[i] = _rb(_silu(g)) * u

        lane = jax.lax.broadcasted_iota(I32, (CB // 2, 128), 1)
        bit0, bit1 = (lane & 1) == 1, (lane & 2) == 2
        ph = []
        for m in range(4):
            r = [pltpu.bitcast(xn_v[rows(i), BLK * m + 128 * q:BLK * m + 128 * q + 128], U32)
                 for q in range(4)]
            r = [v if q == 0 else pltpu.roll(v, q, 1) for q, v in enumerate(r)]
            ph.append(_lane_exchange(r, bit0, bit1))
        uf = [jnp.dot(pltpu.bitcast(jnp.concatenate([ph[m][p] for m in range(4)], axis=0), BF16),
                      tab_v[0, :, 256 * p:256 * p + 256], preferred_element_type=F32)
              for p in range(4)]
        parts = []
        for j in range(CB // 8):
            r = pl.ds(pl.multiple_of(i * CB + 8 * j, 8), 8)
            kf = [[(kf_v[r, 1024 * m + 256 * s:1024 * m + 256 * s + 128],
                    kf_v[r, 1024 * m + 256 * s + 128:1024 * m + 256 * s + 256])
                   for s in range(4)] for m in range(4)]
            edge = [(edge_v[:, 256 * s:256 * s + 128], edge_v[:, 256 * s + 128:256 * s + 256])
                    for s in range(4)]
            u8 = [[(uf[p][CB * m + 8 * j:CB * m + 8 * j + 8, :128],
                    uf[p][CB * m + 8 * j:CB * m + 8 * j + 8, 128:])
                   for p in range(4)] for m in range(4)]
            parts.append(_block_conv(kf, k512_v[r, :], edge, u8))
        yp = []
        for p in range(4):
            z = jnp.concatenate(
                [jnp.concatenate([parts[j][m][p][c] for m in range(4) for j in range(CB // 8)],
                                 axis=0).astype(BF16) for c in range(2)], axis=1)
            y = jax.lax.dot_general(z, tab_v[0, :, 256 * p:256 * p + 256], NT,
                                    preferred_element_type=F32)
            yp.append(pltpu.bitcast(y.astype(BF16), U32))
        skip = skip_v[rows(i), :]
        for m in range(4):
            r = _lane_exchange([y[CB // 2 * m:CB // 2 * (m + 1)] for y in yp], bit0, bit1)
            for q in range(4):
                ts = slice(BLK * m + 128 * q, BLK * m + 128 * q + 128)
                y = r[q] if q == 0 else pltpu.roll(r[q], 128 - q, 1)
                s_v[rows(i), ts] = (pltpu.bitcast(y, BF16).astype(F32)
                                    + xn_v[rows(i), ts].astype(F32) * skip)

    h = jnp.concatenate([h_v[i] for i in range(NCB)], axis=1).astype(BF16)

    @pl.loop(0, NCB)
    def _(i):
        cp_d(i).wait()
        y = jax.lax.dot_general(h, wd_v[rows(i), :], NT, preferred_element_type=F32)
        y = (_rb(y) * gate[:, :CB]).astype(BF16)
        upd = jax.lax.dot_general(y, hot_v[...].astype(BF16), TN, preferred_element_type=F32)
        g = _silu(xn_v[rows(i), :].astype(F32) + upd)
        o_v[rows(i), :] = (x_v[rows(i), :].astype(F32) + s_v[rows(i), :] * g).astype(BF16)
        cp_o(i).start()

    for i in range(NCB):
        cp_o(i).wait()


@jax.jit
def pallas_recurrent_scan__ssm_conv_s4__moe_arch_mod__prompt_kernel(
    A_u: jax.Array,
    A_A_re: jax.Array,
    A_A_im: jax.Array,
    A_B_re: jax.Array,
    A_B_im: jax.Array,
    A_C_re: jax.Array,
    A_C_im: jax.Array,
    A_log_dt: jax.Array,
    A_Dskip: jax.Array,
    B_x: jax.Array,
    B_w_r: jax.Array,
    B_w_gate: jax.Array,
    B_w_up: jax.Array,
    B_w_down: jax.Array,
):
    del B_x
    assert A_u.shape == (1, L, D) and A_A_re.shape == (D, N) and B_w_gate.shape == (D, F)
    tabs, edge = _transform_tables()
    hbm = pl.BlockSpec(memory_space=pl.ANY)
    vmem = pltpu.VMEM
    dma = pltpu.SemaphoreType.DMA
    out = pl.pallas_call(
        _kernel,
        out_shape=jax.ShapeDtypeStruct((D, L), BF16),
        in_specs=[hbm] * 15,
        out_specs=hbm,
        scratch_shapes=[
            vmem((D, L), BF16), vmem((6, D, N), BF16),
            vmem((D,), BF16), vmem((D,), BF16), vmem((D,), BF16),
            vmem((NCB, D, FB), BF16), vmem((NCB, D, FB), BF16), vmem((D, F), BF16),
            vmem((5, 128, 1024), BF16), vmem((8, 1024), F32), vmem((D, L), BF16),
            vmem((D, L), BF16), vmem((D, L), F32),
            vmem((D, 128), F32), vmem((D, 128), F32), vmem((D, 128), F32),
            vmem((7, CB, 128), BF16), vmem((D, 4096), F32),
            vmem((NCB, TOPC, FB), F32), vmem((TOPC, L), F32),
            dma((12,)), dma((NCB,)), dma((NCB,)), dma((NCB,)), dma((NCB,)),
        ],
        compiler_params=pltpu.CompilerParams(vmem_limit_bytes=100 * 1024 * 1024),
    )(A_u[0].T, A_A_re, A_A_im, A_B_re, A_B_im, A_C_re, A_C_im, A_log_dt, A_Dskip, B_w_r,
      B_w_gate, B_w_up, B_w_down.T, tabs.astype(BF16), edge)
    return out.T[None]
```

```python
import jax
import jax.numpy as jnp
import numpy as np
import jax.experimental.pallas as pl
import jax.experimental.pallas.tpu as pltpu

F32, BF16, I32, U32 = jnp.float32, jnp.bfloat16, jnp.int32, jnp.uint32

L, D, N, F = 2048, 576, 128, 4608
TOPC = 8
BLK = 512
CB = 64
NCB = D // CB
FB = F // NCB
DB = 64
NT = (((1,), (1,)), ((), ()))
Q_PAIRS = ((1, 5), (3, 7), (2, 258), (4, 260), (6, 262), (8, 264),
           (516, 772), (520, 776), (1032, 1288), (1544, 1800))
GROUPS = ((6, 7), (8, 9), (3, 5), (0, 1), (2, 4))
RAW = 10 * CB
UF, YP, HP, K512 = 32, 40, 56, 60
K_ORDER = "s vvv p v ss p v ss p v ss p v s v s"
C_ORDER = "MMM I I u I u I u F u F G H"
D_ORDER = "ddd oooo"
PN = 16


def _round_to_bf16(v):
    u = np.asarray(v, np.float32).view(np.uint32)
    return ((u + 0x7FFF + ((u >> 16) & 1)) & 0xFFFF0000).astype(np.uint32).view(np.float32)


def _transform_tables():
    lag_exp = _round_to_bf16(np.arange(L + 1)).astype(np.int64)
    c = np.arange(128)
    kk = np.arange(BLK)

    def root(k, t):
        return np.exp(1j * np.pi * ((4 * k + 1) * t % (4 * BLK)) / (2 * BLK))

    def reim(z):
        z = z.reshape(z.shape[0], -1, 1, 128)
        return np.concatenate([z.real, z.imag], axis=2).reshape(z.shape[0], -1)

    def seg(e, m):
        l = np.arange(BLK * m + 1, min(BLK * m + BLK + 1, L))
        l = l[lag_exp[l] == e]
        return root(kk[None, :], (l - BLK * m)[:, None]).sum(0)

    tu = [128 * ((c - ph) % 4) + (c - (c - ph) % 4) % 128 for ph in range(4)]
    gc, gd, g4, go, g2 = [
        np.concatenate([Q_PAIRS[v][e] + 8 * np.arange(32) for e in range(2) for v in vs])
        for vs in GROUPS]
    t1 = np.where((c >= 63) & (c < 127), g4 + 1,
                  np.where((c >= 31) & (c < 63), np.roll(go, -33), np.roll(go, -1)))
    t3 = np.where(c < 32, np.roll(go, 32), np.where(c < 64, go, g4 - 1))
    tabs = [np.concatenate([reim(root(c[None, :], t[:, None])) for t in ts], axis=1)
            for ts in (tu, (g4, t1, g2, t3))]
    tabs.append(reim(np.stack([seg(e, 1) for e in gc])))
    tabs.append(reim(np.stack([seg(e, 2) for e in np.where(c == 127, gc, gd)])))
    tabs.append(reim(np.stack([seg(e, 3) for e in gd])))
    edge = np.repeat(reim(seg(512, 1)[None, :]), 8, axis=0)
    u = _round_to_bf16(np.stack(tabs)).view(np.uint32)
    return (u[:, 0::2] >> 16) | u[:, 1::2], edge.astype(np.float32)


def _cmul(a, b):
    return a[0] * b[0] - a[1] * b[1], a[0] * b[1] + a[1] * b[0]


def _csq(a):
    return (a[0] + a[1]) * (a[0] - a[1]), (a[0] + a[0]) * a[1]


def _cadd(a, b):
    return a[0] + b[0], a[1] + b[1]


def _csub(a, b):
    return a[0] - b[0], a[1] - b[1]


def _add_i(a, b):
    return a[0] - b[1], a[1] + b[0]


def _sub_i(a, b):
    return a[0] + b[1], a[1] - b[0]


def _lane_exchange(r):
    lane = jax.lax.broadcasted_iota(I32, r[0].shape, 1)
    a = [jnp.where((lane & 1) == 1, r[(j + 1) % 4], r[j]) for j in range(4)]
    b = [jnp.where((lane & 2) == 2, a[(j + 2) % 4], a[j]) for j in range(4)]
    return [b[-j % 4] for j in range(4)]


def _rb(v):
    return v.astype(BF16).astype(F32)


def _silu(v):
    h = 0.5 * v
    return h + h * jnp.tanh(h)


def _pack(even, odd):
    return pltpu.pack_elementwise([even, odd], packed_dtype=BF16)


def _unpack(w):
    return [pltpu.unpack_elementwise(w, index=j, packed_dtype=BF16, unpacked_dtype=F32)
            for j in range(2)]


def _tile(t, n=1):
    return slice(128 * t, 128 * (t + n))


def _ds(start, size, align=None):
    if isinstance(start, int):
        return pl.ds(start, size)
    return pl.ds(pl.multiple_of(start, align or size), size)


def _dot(a, b):
    return jnp.dot(a, b, preferred_element_type=F32)


def _dot_nt(a, b):
    return jax.lax.dot_general(a, b, NT, preferred_element_type=F32)


def _run(order, **stages):
    for step in order.replace(" ", ""):
        next(stages[step])
    for stage in stages.values():
        for _ in stage:
            pass


def _ssm_powers(par, dt):
    a_re, a_im, b_re, b_im, c_re, c_im = par
    mag = jnp.exp(dt * a_re)
    ang = dt * a_im
    pw = {1: (mag * jnp.cos(ang), mag * jnp.sin(ang))}
    for k in range(9):
        pw[2 << k] = _csq(pw[1 << k])
    sc = dt * (1.0 / BLK)
    w = _cmul((c_re, c_im), (b_re * sc, b_im * sc))
    w1, w2 = _cmul(w, pw[1]), _cmul(w, pw[2])
    return [pw[8], pw[16], pw[2], pw[512], w1, _cmul(w1, pw[4]), w2, _cmul(w2, pw[256])], w[0]


def _ssm_products(pw):
    a8, a16, a2, a512, w1, w5, w2, w258 = pw
    sub = jax.lax.broadcasted_iota(I32, (8, 128), 0)
    lane = jax.lax.broadcasted_iota(I32, (8, 128), 1)
    lo = sub < 4

    def pick(z, rows):
        return [jnp.take_along_axis(v, rows, axis=0) for v in z]

    def pair(x, y, h):
        r = [pltpu.roll(v, 4, 0) for v in y]
        return [jnp.where(lo, s, v) if h else jnp.where(lo, v, s) for v, s in zip(x, r)]

    out = []
    for h in range(2):
        p_rows, q_rows = 4 * h + ((sub + 2 * h) & 3), 4 * h + (sub & 3)
        step, s2, s512 = pick(a16, p_rows), pick(a2, q_rows), pick(a512, q_rows)
        p = [[jnp.where(lo, one, v) for one, v in zip((1.0, 0.0), pick(a8, p_rows))]]
        for _ in range(15):
            p.append(_cmul(p[-1], step))
        q = [pair(w1, w5, h)]
        q += [_cmul(q[0], s2), pair(w2, w258, h)]
        for _ in range(3):
            q.append(_cmul(q[-1], s2))
        q += [_cmul(q[3], s512), _cmul(q[5], s512)]
        for _ in range(2):
            q.append(_cmul(q[-1], s512))
        out.append([_dot_nt(*[jnp.concatenate([z[j] for z in zs], axis=0).astype(BF16)
                              for zs in (q, p)]) for j in range(2)])
    first = ((lane - sub) & 3) == 0
    return [jnp.where(first, out[0][0][v:v + 8], out[1][0][v:v + 8])
            - jnp.where(first, out[0][1][v:v + 8], out[1][1][v:v + 8]) for v in range(0, 80, 8)]


def _kernel(x_hbm, are_hbm, aim_hbm, bre_hbm, bim_hbm, cre_hbm, cim_hbm, ldt_hbm, dsk_hbm, wr_hbm,
            wg_hbm, wu_hbm, wd_hbm, tab_hbm, edge_hbm, o_hbm,
            x_v, par_v, ldt_v, dsk_v, wr_v, wg_v, wu_v, wd_v, tab_v, edge_v, o_v,
            xn_v, ph_v, f_v, z_v, pw_v, k0_v, skip_v, raw_v, hot_v, xs_v, yt_v, sem):
    def rows(i):
        return _ds(i * CB, CB)

    cp_vec = [pltpu.make_async_copy(s, d, sem.at[0])
              for s, d in ((ldt_hbm, ldt_v), (dsk_hbm, dsk_v), (wr_hbm, wr_v))]
    cp_par = [pltpu.make_async_copy(p, par_v.at[j], sem.at[1]) for j, p in
              enumerate((are_hbm, aim_hbm, bre_hbm, bim_hbm, cre_hbm, cim_hbm))]
    cp_tab = [pltpu.make_async_copy(s, d, sem.at[4])
              for s, d in ((tab_hbm, tab_v), (edge_hbm, edge_v))]
    cp_x = pltpu.make_async_copy(x_hbm, x_v, sem.at[2])

    def cp_w(i):
        return [pltpu.make_async_copy(s.at[:, _ds(i * FB, FB)], d.at[i], sem.at[5 + i])
                for s, d in ((wg_hbm, wg_v), (wu_hbm, wu_v))]

    def cp_d(i):
        r = _ds(i * DB, DB)
        return pltpu.make_async_copy(wd_hbm.at[r], wd_v.at[r], sem.at[5 + NCB + i])

    for c in cp_vec + cp_par + cp_tab + [cp_x]:
        c.start()
    for i in range(NCB):
        for c in cp_w(i):
            c.start()
    for i in range(D // DB):
        cp_d(i).start()

    def table(t, lo, n):
        return pltpu.bitcast(tab_v[t, :, _tile(lo, n)], BF16)

    raw_v[0:RAW, :] = jnp.zeros((RAW, 128), F32)
    z_v[...] = jnp.zeros(z_v.shape, F32)

    for c in cp_vec:
        c.wait()
    dt_row = _rb(jnp.exp(ldt_v[...].astype(F32).reshape(1, D)))
    raw_v[RAW:RAW + D, :] = jnp.broadcast_to(dt_row, (128, D)).T
    skip_v[...] = jnp.broadcast_to(dsk_v[...].astype(F32).reshape(1, D), (128, D)).T
    for c in cp_par:
        c.wait()

    def kernel_powers(i, n):
        for g in range(0, CB, n):
            r = _ds(i * CB + g, n)
            pw, w = _ssm_powers([par_v[t, r, :].astype(F32) for t in range(6)],
                                raw_v[_ds(RAW + i * CB + g, n), :])
            for t, z in enumerate(pw):
                pw_v[g:g + n, _tile(2 * t)], pw_v[g:g + n, _tile(2 * t + 1)] = z
            k0_v[r, :] = jnp.broadcast_to(jnp.sum(w, axis=1, keepdims=True), (n, 128))
            yield

    def kernel_values(pw):
        for g in range(0, CB, 8):
            out = _ssm_products([(pw[g:g + 8, _tile(2 * t)], pw[g:g + 8, _tile(2 * t + 1)])
                                 for t in range(8)])
            for v in range(10):
                raw_v[pl.ds(CB * v + g, 8), :] = out[v]
            yield

    def kernel_spectrum(i):
        sub = jax.lax.broadcasted_iota(I32, (8, 128), 0)
        lane = jax.lax.broadcasted_iota(I32, (8, 128), 1)
        odd = ((lane - sub) & 1) == 1
        own = ((lane - sub) & 2) == ((sub & 4) >> 1)
        perm = (4 * (lane & 31) + ((sub + ((sub & 4) >> 1)) & 3) + (lane >> 5)) & 127
        u = [jnp.where(odd, pltpu.roll(raw_v[pl.ds(CB * v1 + g, 8), :], 1, 1),
                       raw_v[pl.ds(CB * v0 + g, 8), :])
             for v0, v1 in GROUPS for g in range(0, CB, 8)]
        u = [jnp.where(own, v, pltpu.roll(pltpu.roll(v, 4, 0), 2, 1)) for v in u]
        u = [jnp.take_along_axis(v, perm, axis=1) for v in u]
        gc, gd, g4, go, g2 = [u[t:t + CB // 8] for t in range(0, len(u), CB // 8)]
        mid, low, last = (lane >= 63) & (lane < 127), (lane >= 31) & (lane < 63), lane == 127
        v1 = [jnp.where(mid, a, jnp.where(low, pltpu.roll(b, 95, 1), pltpu.roll(b, 127, 1)))
              for a, b in zip(g4, go)]
        v3 = [jnp.where(lane < 32, pltpu.roll(b, 32, 1), jnp.where(lane < 64, b, a))
              for a, b in zip(g4, go)]
        ve = [jnp.where(last, a, b) for a, b in zip(gc, gd)]
        f_v[rows(i), _tile(K512)] = jnp.broadcast_to(jnp.sum(
            jnp.concatenate([jnp.where(last, a, 0.0) for a in g4], axis=0),
            axis=1, keepdims=True), (CB, 128))
        yield

        def dft(v, t, lo, n):
            return _dot(jnp.concatenate(v, axis=0).astype(BF16), table(t, lo, n))

        for m, v in ((1, gc), (3, gd), (2, ve)):
            for t in (0, 4):
                f_v[rows(i), _tile(8 * m + t, 4)] = dft(v, 1 + m, t, 4)
                yield
        for p, (a, b) in enumerate(((g4, g2), (v1, v3))):
            fa, fb = dft(a, 1, 2 * p, 2), dft(b, 1, 2 * p + 4, 2)
            f_v[rows(i), _tile(4 * p, 2)] = fa + fb
            f_v[rows(i), _tile(4 * p + 2, 2)] = fa - fb
            yield

    _run("", p=kernel_powers(0, 32))
    for c in cp_tab:
        c.wait()

    @pl.loop(0, NCB)
    def _(i):
        _run(K_ORDER, s=kernel_spectrum(jnp.maximum(i - 1, 0)), v=kernel_values(pw_v[...]),
             p=kernel_powers(jnp.minimum(i + 1, NCB - 1), PN))

    cp_x.wait()
    mean = _dot(jnp.ones((8, D), BF16), x_v[...]) * (1.0 / D)
    mean_b = _rb(mean)
    hot_v[...] = mean_b

    def center(i, acc):
        out = []
        for t in range(L // 128):
            w = pltpu.bitcast(x_v[rows(i), _tile(t)], U32)
            sq = acc[t]
            for r in range(0, CB // 2, 8):
                d = [v - hot_v[:, _tile(t)] for v in _unpack(w[r:r + 8])]
                sq = sq + (d[0] * d[0] + d[1] * d[1])
                xn_v[_ds(i * (CB // 2) + r, 8), _tile(t)] = _pack(*d)
            out.append(sq)
        return out

    sq = jax.lax.fori_loop(0, NCB, center, [jnp.zeros((8, 128), F32)] * (L // 128))
    var = (jnp.sum(jnp.concatenate(sq, axis=1), axis=0, keepdims=True) * (1.0 / D)
           - jnp.square(mean - mean_b))
    inv = 1.0 / _rb(jnp.sqrt(_rb(_rb(jnp.maximum(var, 0.0)) + float(_round_to_bf16(1e-5)))))
    wr = jnp.broadcast_to(wr_v[...].astype(F32).reshape(1, D), (TOPC, D)).astype(BF16)
    score = []
    for t in range(L // 128):
        w = jnp.concatenate(
            [_pack(*[v * inv[:, _tile(t)] for v in _unpack(xn_v[r:r + 8, _tile(t)])])
             for r in range(0, D // 2, 8)], axis=0)
        xn_v[:, _tile(t)] = w
        score.append(_dot(wr, pltpu.bitcast(w, BF16)))
    score = _rb(jnp.concatenate(score, axis=1))

    def split_phases(i):
        r = pl.ds(i * CB // 2, CB // 2)
        for m in range(4):
            v = [xn_v[r, _tile(4 * m + q)] for q in range(4)]
            v = _lane_exchange([w if q == 0 else pltpu.roll(w, q, 1) for q, w in enumerate(v)])
            for p in range(4):
                ph_v[r, _tile(4 * m + p)] = v[p]

    def forward(i):
        for h in range(0, CB, 32):
            for p in range(2):
                a, b = [_dot(
                    pltpu.bitcast(jnp.concatenate(
                        [ph_v[_ds(i * (CB // 2) + g // 2, 8), _tile(4 * m + t)]
                         for g in (h, h + 16) for m in range(4)], axis=0), BF16),
                    table(0, 2 * t, 2)) for t in (p, p + 2)]
                yield
                for r in range(0, 128, 8):
                    f_v[4 * h + r:4 * h + r + 8, _tile(UF + 4 * p, 2)] = a[r:r + 8] + b[r:r + 8]
                    f_v[4 * h + r:4 * h + r + 8, _tile(UF + 4 * p + 2, 2)] = a[r:r + 8] - b[r:r + 8]
                    yield

    def multiply(i):
        def load(r, t):
            return f_v[r, _tile(t)], f_v[r, _tile(t + 1)]

        for g in range(0, CB, 8):
            r = _ds(i * CB + g, 8)
            for s, ops in enumerate(((_cadd, _csub), (_add_i, _sub_i))):
                z = []
                for t, op in zip((0, 2), ops):
                    ks, us, acc, prev = [], [], [None] * 4, None
                    for m in range(4):
                        ru = pl.ds(64 * (g // 16) + 16 * m + g % 16, 8)
                        a, b = op(load(ru, UF + 2 * s), load(ru, UF + 2 * s + 4))
                        us.append((a + b, a, b))
                        if m == 0:
                            k = op(load(r, 2 * s), load(r, 2 * s + 4))
                        else:
                            k = load(r, 8 * m + 2 * (s + t))
                        if m == 1:
                            k = [v + f_v[r, _tile(K512)] * edge_v[:, _tile(2 * (s + t) + c)]
                                 for c, v in enumerate(k)]
                        c, d = k if m == 0 else _sub_i(k, prev)
                        ks.append((c, d - c, c + d))
                        prev = k
                        for x, y in [(x, m) for x in range(m + 1)] + [(m, y) for y in range(m)]:
                            if x + y < 4:
                                new = [v * w for v, w in zip(ks[x], us[y])]
                                acc[x + y] = new if acc[x + y] is None else [
                                    v + w for v, w in zip(acc[x + y], new)]
                        if t == 0 or m < 3:
                            yield
                    z.append([(v[0] - v[2], v[0] + v[1]) for v in acc])
                for n in range(4):
                    for t, v in enumerate(_cadd(z[0][n], z[1][n]) + _csub(z[0][n], z[1][n])):
                        z_v[pl.ds(4 * g + 8 * n, 8), _tile(4 * s + t)] = v
                yield

    def inverse(i, z):
        for h in range(0, CB, 32):
            for p, ops in enumerate(((_cadd, _csub), (_sub_i, _add_i))):
                a, c = [[z[4 * h:4 * h + 128, _tile(4 * s + 2 * p + t)] for t in range(2)]
                        for s in range(2)]
                y = [_dot_nt(jnp.concatenate(op(a, c), axis=1).astype(BF16),
                             table(0, 2 * p + 4 * t, 2)) for t, op in enumerate(ops)]
                yield
                for g in range(0, 32, 8):
                    for m in range(4):
                        for t in range(2):
                            f_v[_ds(i * CB + h + g, 8), _tile(YP + 4 * m + p + 2 * t)] = (
                                y[t][4 * g + 8 * m:4 * g + 8 * m + 8])
                        yield

    bits = pltpu.bitcast(jnp.where(score == 0.0, 0.0, score), I32) >> 16
    pos = jax.lax.broadcasted_iota(I32, (TOPC, L), 1)
    key = ((bits ^ ((bits >> 15) & 0x7FFF)) << 11) + (0x38000000 + L - 1 - pos)
    key = pltpu.bitcast(key, F32)
    sub = jax.lax.broadcasted_iota(I32, (TOPC, 128), 0)
    dense = []
    for t0 in (0, 8):
        v = key[:, _tile(t0)]
        for t in range(1, 8):
            v = jnp.where(sub == t, key[:, _tile(t0 + t)], v)
        dense.append(v)
    _run("", s=kernel_spectrum(NCB - 1))
    split_phases(0)
    _run("", f=forward(0))
    top = jnp.zeros((TOPC, 128), F32)
    for c in range(TOPC):
        best = jnp.max(jnp.max(jnp.maximum(dense[0], dense[1]), axis=0, keepdims=True),
                       axis=1, keepdims=True)
        top = jnp.where(sub == c, best, top)
        dense = [jnp.where(v == best, 0.0, v) for v in dense]
        split_phases(c + 1)
    hot = jnp.where(key == jnp.tile(top, (1, L // 128)), 1.0, 0.0)
    hot_v[...] = hot
    tb = (pltpu.bitcast(top, I32) - 0x38000000) >> 11
    gate = _rb(jax.nn.sigmoid(pltpu.bitcast((tb ^ ((tb >> 15) & 0x7FFF)) << 16, F32)))
    xs_v[...] = _dot_nt(hot.astype(BF16), pltpu.bitcast(xn_v[...], BF16))

    def ffn_up(i):
        xs = xs_v[...].astype(BF16)
        for j in range(FB // 128):
            g, u = [_rb(_dot(xs, w[i, :, _tile(j)])) for w in (wg_v, wu_v)]
            f_v[_ds(TOPC * i, TOPC), _tile(HP + j)] = _rb(_silu(g)) * u
            yield

    @pl.loop(0, NCB)
    def _(i):
        for c in cp_w(i):
            c.wait()
        order = C_ORDER
        for k, v in (("M", "m" * 8), ("I", "i" + "im" * 16), ("F", "f" + "fm" * 16),
                     ("G", "f" + "fm" * 8 + "f" * 8), ("H", "f" * 17),
                     ("J", "i" + ("i" * 8 + "m" * 8) * 2), ("E", "f" + ("f" * 8 + "m" * 8) * 2),
                     ("K", "i" + ("i" * 4 + "m" * 4) * 4), ("D", "f" + ("f" * 4 + "m" * 4) * 4)):
            order = order.replace(k, v)
        _run(order, i=inverse(jnp.maximum(i - 1, 0), z_v[...]), m=multiply(i), u=ffn_up(i),
             f=forward(jnp.minimum(i + 1, NCB - 1)))

    def ffn_down(i):
        y = None
        for js in ((0, 1, 2), (3, 4, 5), (6, 7, 8)):
            h = jnp.concatenate([f_v[TOPC * j:TOPC * j + TOPC, _tile(HP, 4)] for j in js], axis=1)
            t = _dot_nt(h.astype(BF16), wd_v[_ds(i * DB, DB), FB * js[0]:FB * (js[-1] + 1)])
            y = t if y is None else y + t
            if js[-1] == 8:
                yt_v[...] = _rb(_rb(y) * gate[:, :DB]).T
            yield

    def finish(i, yt):
        r = _ds(i * DB, DB)
        skip = skip_v[r, :] + BLK * k0_v[r, :]
        for m in range(4):
            upd = _dot(yt.astype(BF16), hot_v[:, _tile(4 * m, 4)].astype(BF16))
            y = _lane_exchange([f_v[r, _tile(YP + 4 * m + p)] for p in range(4)])
            y = [v if q == 0 else pltpu.roll(v, 128 - q, 1) for q, v in enumerate(y)]
            for q in (0, 2):
                sg = []
                for t in (q, q + 1):
                    xn = pltpu.bitcast(xn_v[_ds(i * (DB // 2), DB // 2), _tile(4 * m + t)],
                                       BF16).astype(F32)
                    sg.append((y[t] + xn * skip) * _silu(xn + upd[:, _tile(t)]))
                ts = _tile(4 * m + q, 2)
                o_v[r, ts] = (x_v[r, ts].astype(F32) + jnp.concatenate(sg, axis=1)).astype(BF16)
            yield

    cp_d(0).wait()
    _run("", d=ffn_down(0), i=inverse(NCB - 1, z_v))

    @pl.loop(0, D // DB)
    def _(i):
        @pl.when(i + 1 < D // DB)
        def _():
            cp_d(i + 1).wait()

        _run(D_ORDER, o=finish(i, yt_v[...]), d=ffn_down(jnp.minimum(i + 1, D // DB - 1)))
        r = _ds(i * DB, DB)
        pltpu.make_async_copy(o_v.at[r], o_hbm.at[r], sem.at[3]).start()

    pltpu.make_async_copy(o_v, o_hbm, sem.at[3]).wait()


@jax.jit
def pallas_recurrent_scan__ssm_conv_s4__moe_arch_mod__prompt_kernel(
    A_u: jax.Array,
    A_A_re: jax.Array,
    A_A_im: jax.Array,
    A_B_re: jax.Array,
    A_B_im: jax.Array,
    A_C_re: jax.Array,
    A_C_im: jax.Array,
    A_log_dt: jax.Array,
    A_Dskip: jax.Array,
    B_x: jax.Array,
    B_w_r: jax.Array,
    B_w_gate: jax.Array,
    B_w_up: jax.Array,
    B_w_down: jax.Array,
):
    del B_x
    assert A_u.shape == (1, L, D) and A_A_re.shape == (D, N) and B_w_gate.shape == (D, F)
    tabs, edge = _transform_tables()
    hbm = pl.BlockSpec(memory_space=pl.ANY)
    vmem = pltpu.VMEM
    out = pl.pallas_call(
        _kernel,
        out_shape=jax.ShapeDtypeStruct((D, L), BF16),
        in_specs=[hbm] * 15,
        out_specs=hbm,
        scratch_shapes=[
            vmem((D, L), BF16), vmem((6, D, N), BF16),
            vmem((D,), BF16), vmem((D,), BF16), vmem((D,), BF16),
            vmem((NCB, D, FB), BF16), vmem((NCB, D, FB), BF16), vmem((D, F), BF16),
            vmem((5, 64, 1024), U32), vmem((8, 1024), F32), vmem((D, L), BF16),
            vmem((D // 2, L), U32), vmem((D // 2, L), U32),
            vmem((D, 128 * (K512 + 1)), F32), vmem((4 * CB, 1024), F32),
            vmem((CB, 16 * 128), F32), vmem((D, 128), F32), vmem((D, 128), F32),
            vmem((RAW + D, 128), F32), vmem((TOPC, L), F32), vmem((TOPC, D), F32),
            vmem((DB, TOPC), F32),
            pltpu.SemaphoreType.DMA((5 + NCB + D // DB,)),
        ],
        compiler_params=pltpu.CompilerParams(vmem_limit_bytes=100 * 1024 * 1024),
    )(A_u[0].T, A_A_re, A_A_im, A_B_re, A_B_im, A_C_re, A_C_im, A_log_dt, A_Dskip, B_w_r,
      B_w_gate, B_w_up, B_w_down.T, tabs, edge)
    return out.T[None]
```

```python
import jax
import jax.numpy as jnp
import numpy as np
import jax.experimental.pallas as pl
import jax.experimental.pallas.tpu as pltpu

F32, BF16, I32, U32 = jnp.float32, jnp.bfloat16, jnp.int32, jnp.uint32

L, D, N, F = 2048, 576, 128, 4608
TOPC = 8
BLK = 512
CB = 64
NCB = D // CB
FB = F // NCB
DB = 64
NT = (((1,), (1,)), ((), ()))
Q_PAIRS = ((3, 1), (7, 5), (2, 258), (4, 260), (6, 262), (8, 264),
           (516, 772), (520, 776), (1032, 1288), (1544, 1800))
GROUPS = ((6, 7), (8, 9), (3, 5), (0, 1), (2, 4))
RAW = 10 * CB
UF, YP, HP, K512 = 32, 40, 56, 60
K_ORDER = "s vvv p v ss p v ss p v ss v s p v s"
C_ORDER = "MM K K K K uM D u D u G u H"
D_ORDER = "d o d o d oo"
L_ORDER = "s mm n m n ms n ms n ms n ms n ms n s n ss"
LT = 2
SPLIT = {8: (1, 2), 1: (2, 9)}
PN = 16


def _round_to_bf16(v):
    u = np.asarray(v, np.float32).view(np.uint32)
    return ((u + 0x7FFF + ((u >> 16) & 1)) & 0xFFFF0000).astype(np.uint32).view(np.float32)


def _cmul(a, b):
    return a[0] * b[0] - a[1] * b[1], a[0] * b[1] + a[1] * b[0]


def _csq(a):
    return (a[0] + a[1]) * (a[0] - a[1]), (a[0] + a[0]) * a[1]


def _cadd(a, b):
    return a[0] + b[0], a[1] + b[1]


def _csub(a, b):
    return a[0] - b[0], a[1] - b[1]


def _add_i(a, b):
    return a[0] - b[1], a[1] + b[0]


def _sub_i(a, b):
    return a[0] + b[1], a[1] - b[0]


def _lane_exchange(r):
    lane = jax.lax.broadcasted_iota(I32, r[0].shape, 1)
    a = [jnp.where((lane & 1) == 1, r[(j + 1) % 4], r[j]) for j in range(4)]
    b = [jnp.where((lane & 2) == 2, a[(j + 2) % 4], a[j]) for j in range(4)]
    return [b[-j % 4] for j in range(4)]


def _rb(v):
    return v.astype(BF16).astype(F32)


def _silu(v):
    h = 0.5 * v
    return h + h * jnp.tanh(h)


def _pack(even, odd):
    return pltpu.pack_elementwise([even, odd], packed_dtype=BF16)


def _unpack(w):
    return [pltpu.unpack_elementwise(w, index=j, packed_dtype=BF16, unpacked_dtype=F32)
            for j in range(2)]


def _tile(t, n=1):
    return slice(128 * t, 128 * (t + n))


def _ds(start, size, align=None):
    if isinstance(start, int):
        return pl.ds(start, size)
    return pl.ds(pl.multiple_of(start, align or size), size)


def _dot(a, b):
    return jnp.dot(a, b, preferred_element_type=F32)


def _dot_nt(a, b):
    return jax.lax.dot_general(a, b, NT, preferred_element_type=F32)


def _run(order, **stages):
    for step in order.replace(" ", ""):
        next(stages[step])
    for stage in stages.values():
        for _ in stage:
            pass


def _sort_rows(v, sizes):
    sub = jax.lax.broadcasted_iota(I32, v.shape, 0)
    for k in sizes:
        j = k // 2
        while j:
            w = jnp.take_along_axis(v, sub ^ j, axis=0)
            v = jnp.where(((sub & j) == 0) == ((sub & k) == 0),
                          jnp.maximum(v, w), jnp.minimum(v, w))
            j //= 2
    return v


def _merge_top(a, b):
    sub = jax.lax.broadcasted_iota(I32, a.shape, 0)
    return _sort_rows(jnp.maximum(a, jnp.take_along_axis(b, 7 - sub, axis=0)), (8,))


def _write_tables(tab_v, edge_v):
    sub = jax.lax.broadcasted_iota(I32, (8, 128), 0)
    lane = jax.lax.broadcasted_iota(I32, (8, 128), 1)
    ang = (((4 * lane + 1) << sub) & (4 * BLK - 1)).astype(F32) * (np.pi / (2 * BLK))
    bits = jnp.cos(ang), jnp.sin(ang)
    known = {1 << s: [jnp.broadcast_to(v[s:s + 1], (8, 128)) for v in bits] for s in range(8)}
    known[0] = [jnp.ones((8, 128), F32), jnp.zeros((8, 128), F32)]

    def times_i(z, n):
        for _ in range(n % 4):
            z = (-z[1], z[0])
        return z

    def power(t):
        if t >= BLK:
            return times_i(power(t - BLK), 1)
        if t not in known:
            low = t & -t if t & (t - 1) else t // 2
            known[t] = _cmul(power(t - low), power(low))
        return known[t]

    def put(cond, z, base):
        return [jnp.where(cond, v, w) for v, w in zip(z, base)]

    def lag_sum(ts, s):
        terms = [times_i(power(t), s * t) for t in ts]
        return [sum(z[c] for z in terms) for c in range(2)]

    def ramp(step):
        z = put((sub & 1) == 1, power(step), known[0])
        for b in (2, 4):
            z = _cmul(z, put((sub & b) == b, power(b * step), known[0]))
        return z

    def store(t, j, col, even, odd):
        for c in range(2):
            tab_v[t, 8 * j:8 * j + 8, _tile(col + c)] = _pack(even[c], odd[c])

    ramp2, ramp16 = ramp(2), ramp(16)
    for p in range(4):
        col = []
        for e in range(2):
            q0, q1 = (e - p) % 4, (e + 2 - p) % 4
            z = [_cmul(ramp2, put((sub & 1) == 1, power(127 * q1 + e), power(127 * q0 + e)))]
            for _ in range(8):
                z.append(_cmul(z[-1], power(16)))
            z[0] = put(2 * sub + e < ((2 * sub + e - p) & 3), z[8], z[0])
            col.append(z)
        for j in range(8):
            store(0, j, 2 * p, col[0][j], col[1][j])

    lag_exp = _round_to_bf16(np.arange(L)).astype(np.int64)
    c = np.arange(128)
    gc, gd, g4, go, g2 = [
        np.concatenate([Q_PAIRS[v][e] + 8 * np.arange(32) for e in range(2) for v in vs])
        for vs in GROUPS]
    g1 = np.where((c >= 63) & (c < 127), g4, np.roll(go, 63))
    g3, ge = np.where(c < 64, go, g4), np.where(c == 127, gc, gd)
    rows16 = {}

    def ramp_from(t):
        if t not in rows16:
            back = [d for d in (8, 128) if t - d in rows16]
            rows16[t] = (_cmul(rows16[t - back[0]], power(back[0])) if back
                         else _cmul(ramp16, power(t)))
        return rows16[t]

    def lags(e, m, phase=None):
        ts = [int(l) - BLK * m for l in np.nonzero(lag_exp == e)[0] if 0 < l - BLK * m <= BLK]
        return [t for t in ts if phase is None or t % 4 == phase]

    def rows(tss, s):
        z = [known[0][1]] * 2
        if tss[0]:
            half = len(tss[0]) // 2
            z = ramp_from(tss[0][half])
            if half:
                assert tss[0][half] % 4 == 0 and len(tss[0]) % 2 == 1
                box = 1.0 + 2.0 * lag_sum(range(1, half + 1), s)[0]
                z = [v * box for v in z]
        for r, ts in enumerate(tss):
            if ts != [t + 16 * r for t in tss[0]]:
                z = put(sub == r, lag_sum(ts, s), z)
        return z

    for j in range(8):
        for p, g in enumerate((g4, g1, g2, g3)):
            store(1, j, 2 * p, *[rows([lags(v, 0, p) for v in g[16 * j + e:16 * j + 16:2]], 0)
                                 for e in range(2)])
        for m, g in ((1, gc), (2, ge), (3, gd)):
            for s in range(4):
                store(1 + m, j, 2 * s, *[rows([lags(v, m) for v in g[16 * j + e:16 * j + 16:2]], s)
                                         for e in range(2)])
    for s in range(4):
        edge_v[:, _tile(2 * s)], edge_v[:, _tile(2 * s + 1)] = lag_sum(lags(BLK, 1), s)


def _ssm_powers(par, dt):
    a_re, a_im, b_re, b_im, c_re, c_im = par
    mag = jnp.exp(dt * a_re)
    ang = dt * a_im
    pw = {1: (mag * jnp.cos(ang), mag * jnp.sin(ang))}
    for k in range(9):
        pw[2 << k] = _csq(pw[1 << k])
    sc = dt * (2.0 / BLK)
    w = _cmul((c_re, c_im), (b_re * sc, b_im * sc))
    w1, w2 = _cmul(w, pw[1]), _cmul(w, pw[2])
    return [pw[8], pw[16], pw[2], pw[4], pw[512],
            w1, _cmul(w1, pw[2]), w2, _cmul(w2, pw[256])], w[0]


def _ssm_products(pw):
    a8, a16, a2, a4, a512, w1, w3, w2, w258 = pw
    sub = jax.lax.broadcasted_iota(I32, (8, 128), 0)
    lane = jax.lax.broadcasted_iota(I32, (8, 128), 1)
    lo = sub < 4

    def pick(z, rows):
        return [jnp.take_along_axis(v, rows, axis=0) for v in z]

    def pair(x, y, h):
        r = [pltpu.roll(v, 4, 0) for v in y]
        return [jnp.where(lo, s, v) if h else jnp.where(lo, v, s) for v, s in zip(x, r)]

    out = []
    for h in range(2):
        p_rows, q_rows = 4 * h + ((sub + 2 * h) & 3), 4 * h + (sub & 3)
        step, s2, s512 = pick(a16, p_rows), pick(a2, q_rows), pick(a512, q_rows)
        p = [[jnp.where(lo, one, v) for one, v in zip((1.0, 0.0), pick(a8, p_rows))]]
        for _ in range(15):
            p.append(_cmul(p[-1], step))
        q = [pair(w3, w1, h)]
        q += [_cmul(q[0], pick(a4, q_rows)), pair(w2, w258, h)]
        for _ in range(3):
            q.append(_cmul(q[-1], s2))
        q += [_cmul(q[3], s512), _cmul(q[5], s512)]
        for _ in range(2):
            q.append(_cmul(q[-1], s512))
        out.append([_dot_nt(*[jnp.concatenate([z[j] for z in zs], axis=0).astype(BF16)
                              for zs in (q, p)]) for j in range(2)])
    first = ((lane - sub) & 3) == 0
    return [jnp.where(first, out[0][0][v:v + 8], out[1][0][v:v + 8])
            - jnp.where(first, out[0][1][v:v + 8], out[1][1][v:v + 8]) for v in range(0, 80, 8)]


def _kernel(x_hbm, are_hbm, aim_hbm, bre_hbm, bim_hbm, cre_hbm, cim_hbm, ldt_hbm, dsk_hbm, wr_hbm,
            wg_hbm, wu_hbm, wd_hbm, o_hbm,
            x_v, par_v, ldt_v, dsk_v, wr_v, wg_v, wu_v, wd_v, tab_v, edge_v, o_v,
            xn_v, ph_v, f_v, z_v, pw_v, k0_v, skip_v, raw_v, hot_v, xs_v, yt_v, sem):
    def rows(i):
        return _ds(i * CB, CB)

    def words(i, n):
        return _ds(i * (n // 2), n // 2)

    pars = (are_hbm, aim_hbm, bre_hbm, bim_hbm, cre_hbm, cim_hbm)
    cp_dt = pltpu.make_async_copy(ldt_hbm, ldt_v, sem.at[0])
    cp_head, cp_rest = [
        [pltpu.make_async_copy(p.at[r], par_v.at[j, r], sem.at[k]) for j, p in enumerate(pars)]
        for k, r in ((1, pl.ds(0, 2 * CB)), (4, pl.ds(2 * CB, D - 2 * CB)))]
    cp_x = [pltpu.make_async_copy(s, d, sem.at[2])
            for s, d in ((x_hbm.bitcast(U32), x_v), (dsk_hbm, dsk_v), (wr_hbm, wr_v))]

    def cp_w(i):
        return [pltpu.make_async_copy(s.bitcast(U32).at[:, _ds(i * FB, FB)], d.at[i], sem.at[5 + i])
                for s, d in ((wg_hbm, wg_v), (wu_hbm, wu_v))]

    def cp_d(i):
        return pltpu.make_async_copy(wd_hbm.bitcast(U32).at[words(i, DB)], wd_v.at[words(i, DB)],
                                     sem.at[5 + NCB + i])

    for c in [cp_dt] + cp_head + cp_rest + cp_x:
        c.start()

    def table(t, lo, n):
        return pltpu.bitcast(tab_v[t, :, _tile(lo, n)], BF16)

    raw_v[0:RAW, :] = jnp.zeros((RAW, 128), F32)
    _write_tables(tab_v, edge_v)

    cp_dt.wait()
    dt_row = _rb(jnp.exp(ldt_v[...].astype(F32).reshape(1, D)))
    raw_v[RAW:RAW + D, :] = jnp.broadcast_to(dt_row, (128, D)).T
    for c in cp_head:
        c.wait()
    z_v[...] = jnp.zeros(z_v.shape, F32)

    def kernel_powers(i, n):
        for g in range(0, CB, n):
            r = _ds(i * CB + g, n)
            pw, w = _ssm_powers([par_v[t, r, :].astype(F32) for t in range(6)],
                                raw_v[_ds(RAW + i * CB + g, n), :])
            for t, z in enumerate(pw):
                pw_v[g:g + n, _tile(2 * t)], pw_v[g:g + n, _tile(2 * t + 1)] = z
            k0_v[r, :] = jnp.broadcast_to(jnp.sum(w, axis=1, keepdims=True), (n, 128))
            yield

    def kernel_values(pw):
        for g in range(0, CB, 8):
            out = _ssm_products([(pw[g:g + 8, _tile(2 * t)], pw[g:g + 8, _tile(2 * t + 1)])
                                 for t in range(9)])
            for v in range(10):
                raw_v[pl.ds(CB * v + g, 8), :] = out[v]
            yield

    def kernel_spectrum(i):
        sub = jax.lax.broadcasted_iota(I32, (8, 128), 0)
        lane = jax.lax.broadcasted_iota(I32, (8, 128), 1)
        odd = ((lane - sub) & 1) == 1
        own = ((lane - sub) & 2) == ((sub & 4) >> 1)
        perm = (4 * (lane & 31) + ((sub + ((sub & 4) >> 1)) & 3) + (lane >> 5)) & 127
        u = [jnp.where(odd, pltpu.roll(raw_v[pl.ds(CB * v1 + g, 8), :], 1, 1),
                       raw_v[pl.ds(CB * v0 + g, 8), :])
             for v0, v1 in GROUPS for g in range(0, CB, 8)]
        u = [jnp.where(own, v, pltpu.roll(pltpu.roll(v, 4, 0), 2, 1)) for v in u]
        u = [jnp.take_along_axis(v, perm, axis=1) for v in u]
        gc, gd, g4, go, g2 = [u[t:t + CB // 8] for t in range(0, len(u), CB // 8)]
        mid, last = (lane >= 63) & (lane < 127), lane == 127
        v1 = [jnp.where(mid, a, pltpu.roll(b, 63, 1)) for a, b in zip(g4, go)]
        v3 = [jnp.where(lane < 64, b, a) for a, b in zip(g4, go)]
        ve = [jnp.where(last, a, b) for a, b in zip(gc, gd)]
        f_v[rows(i), _tile(K512)] = jnp.broadcast_to(jnp.sum(
            jnp.concatenate([jnp.where(last, a, 0.0) for a in g4], axis=0),
            axis=1, keepdims=True), (CB, 128))
        yield

        def dft(v, t, lo, n):
            return _dot(jnp.concatenate(v, axis=0).astype(BF16), table(t, lo, n))

        for m, v in ((1, gc), (3, gd), (2, ve)):
            for t in (0, 4):
                f_v[rows(i), _tile(8 * m + t, 4)] = dft(v, 1 + m, t, 4)
                yield
        for p, (a, b) in enumerate(((g4, g2), (v1, v3))):
            fa, fb = dft(a, 1, 2 * p, 2), dft(b, 1, 2 * p + 4, 2)
            f_v[rows(i), _tile(4 * p, 2)] = fa + fb
            f_v[rows(i), _tile(4 * p + 2, 2)] = fa - fb
            yield

    _run("", p=kernel_powers(0, 32))

    @pl.loop(0, NCB)
    def _(i):
        @pl.when(i == 1)
        def _():
            for c in cp_rest:
                c.wait()

        for c in cp_w(i):
            c.start()
        _run(K_ORDER, s=kernel_spectrum(jnp.maximum(i - 1, 0)), v=kernel_values(pw_v[...]),
             p=kernel_powers(jnp.minimum(i + 1, NCB - 1), PN))

    for c in cp_x:
        c.wait()
    for i in range(D // DB):
        cp_d(i).start()
    skip_v[...] = jnp.broadcast_to(dsk_v[...].astype(F32).reshape(1, D), (128, D)).T
    wr = jnp.broadcast_to(wr_v[...].astype(F32).reshape(1, D), (TOPC, D)).astype(BF16)
    eps = float(_round_to_bf16(1e-5))
    mean, score = [], []

    def token_mean():
        for t in range(0, L // 128, LT):
            m = _dot(jnp.ones((8, D), BF16), pltpu.bitcast(x_v[:, _tile(t, LT)], BF16)) * (1.0 / D)
            mean.extend(m[:, _tile(j)] for j in range(LT))
            yield

    def normalize():
        for t0 in range(0, L // 128, LT):
            out = []
            for t in range(t0, t0 + LT):
                mb, sq, cen = _rb(mean[t]), [0.0, 0.0], []
                for r in range(0, D // 2, 8):
                    d = [v - mb for v in _unpack(x_v[r:r + 8, _tile(t)])]
                    sq = [a + v * v for a, v in zip(sq, d)]
                    cen.append(_pack(*d))
                var = (jnp.sum(sq[0] + sq[1], axis=0, keepdims=True) * (1.0 / D)
                       - jnp.square(mean[t] - mb))
                inv = 0.5 / _rb(jnp.sqrt(_rb(_rb(jnp.maximum(var, 0.0)) + eps)))
                out.append(jnp.concatenate(
                    [_pack(*[v * inv for v in _unpack(w)]) for w in cen], axis=0))
            out = jnp.concatenate(out, axis=1)
            xn_v[:, _tile(t0, LT)] = out
            score.append(_rb(2.0 * _dot(wr, pltpu.bitcast(out, BF16))))
            yield

    _run(L_ORDER, s=kernel_spectrum(NCB - 1), m=token_mean(), n=normalize())
    score = jnp.concatenate(score, axis=1)

    def split_phases(i):
        r = pl.ds(i * CB // 2, CB // 2)
        for m in range(4):
            v = [xn_v[r, _tile(4 * m + q)] for q in range(4)]
            v = _lane_exchange([w if q == 0 else pltpu.roll(w, q, 1) for q, w in enumerate(v)])
            for p in range(4):
                ph_v[r, _tile(4 * m + p)] = v[p]

    def forward(i):
        for h in range(0, CB, 32):
            for p in range(2):
                a, b = [_dot(
                    pltpu.bitcast(jnp.concatenate(
                        [ph_v[_ds(i * (CB // 2) + g // 2, 8), _tile(4 * m + t)]
                         for g in (h, h + 16) for m in range(4)], axis=0), BF16),
                    table(0, 2 * t, 2)) for t in (p, p + 2)]
                yield
                for r in range(0, 128, 8):
                    f_v[4 * h + r:4 * h + r + 8, _tile(UF + 4 * p, 2)] = a[r:r + 8] + b[r:r + 8]
                    f_v[4 * h + r:4 * h + r + 8, _tile(UF + 4 * p + 2, 2)] = a[r:r + 8] - b[r:r + 8]
                    yield

    def multiply(i):
        def load(r, t):
            return f_v[r, _tile(t)], f_v[r, _tile(t + 1)]

        for g in range(0, CB, 8):
            r = _ds(i * CB + g, 8)
            for s, ops in enumerate(((_cadd, _csub), (_add_i, _sub_i))):
                z = []
                for t, op in zip((0, 2), ops):
                    ks, us, acc, prev = [], [], [None] * 4, None
                    for m in range(4):
                        ru = pl.ds(64 * (g // 16) + 16 * m + g % 16, 8)
                        a, b = op(load(ru, UF + 2 * s), load(ru, UF + 2 * s + 4))
                        us.append((a + b, a, b))
                        if m == 0:
                            k = op(load(r, 2 * s), load(r, 2 * s + 4))
                        else:
                            k = load(r, 8 * m + 2 * (s + t))
                        if m == 1:
                            k = [v + f_v[r, _tile(K512)] * edge_v[:, _tile(2 * (s + t) + c)]
                                 for c, v in enumerate(k)]
                        c, d = k if m == 0 else _sub_i(k, prev)
                        ks.append((c, d - c, c + d))
                        prev = k
                        for x, y in [(x, m) for x in range(m + 1)] + [(m, y) for y in range(m)]:
                            if x + y < 4:
                                new = [v * w for v, w in zip(ks[x], us[y])]
                                acc[x + y] = new if acc[x + y] is None else [
                                    v + w for v, w in zip(acc[x + y], new)]
                        if t == 0 or m < 3:
                            yield
                    z.append([(v[0] - v[2], v[0] + v[1]) for v in acc])
                for n in range(4):
                    for t, v in enumerate(_cadd(z[0][n], z[1][n]) + _csub(z[0][n], z[1][n])):
                        z_v[pl.ds(4 * g + 8 * n, 8), _tile(4 * s + t)] = v
                yield

    def inverse(i, z):
        for h in range(0, CB, 32):
            for p, ops in enumerate(((_cadd, _csub), (_sub_i, _add_i))):
                a, c = [[z[4 * h:4 * h + 128, _tile(4 * s + 2 * p + t)] for t in range(2)]
                        for s in range(2)]
                y = [_dot_nt(jnp.concatenate(op(a, c), axis=1).astype(BF16),
                             table(0, 2 * p + 4 * t, 2)) for t, op in enumerate(ops)]
                yield
                for g in range(0, 32, 8):
                    for m in range(4):
                        for t in range(2):
                            f_v[_ds(i * CB + h + g, 8), _tile(YP + 4 * m + p + 2 * t)] = (
                                y[t][4 * g + 8 * m:4 * g + 8 * m + 8])
                        yield

    bits = pltpu.bitcast(jnp.where(score == 0.0, 0.0, score), I32) >> 16
    pos = jax.lax.broadcasted_iota(I32, (TOPC, L), 1)
    key = ((bits ^ ((bits >> 15) & 0x7FFF)) << 11) + (0x38000000 + L - 1 - pos)
    key = pltpu.bitcast(key, F32)
    sub = jax.lax.broadcasted_iota(I32, (TOPC, 128), 0)
    dense = []
    for t0 in (0, 8):
        v = key[:, _tile(t0)]
        for t in range(1, 8):
            v = jnp.where(sub == t, key[:, _tile(t0 + t)], v)
        dense.append(v)
    split_phases(0)
    _run("", f=forward(0))
    top = _merge_top(*[_sort_rows(v, (2, 4, 8)) for v in dense])
    for step, count in ((8, 16), (1, 8)):
        top = [top] + [pltpu.roll(top, step * k, 1) for k in range(1, count)]
        while len(top) > 1:
            top = [_merge_top(a, b) for a, b in zip(top[0::2], top[1::2])]
        top = top[0]
        for i in range(*SPLIT[step]):
            split_phases(i)
    hot_v[...] = jnp.where(key == jnp.tile(top, (1, L // 128)), 1.0, 0.0)
    top = pltpu.bitcast(top, I32) - 0x38000000
    tb = top >> 11
    gate = _rb(jax.nn.sigmoid(pltpu.bitcast((tb ^ ((tb >> 15) & 0x7FFF)) << 16, F32)))
    tok = (L - 1) - (top & (L - 1))
    pick = (tok & 127) == jax.lax.broadcasted_iota(I32, (TOPC, 128), 1)
    xs_v[...] = _dot_nt(
        jnp.concatenate([jnp.where(pick & (sub == c), 2.0, 0.0) for c in range(TOPC)],
                        axis=1).astype(BF16),
        pltpu.bitcast(jnp.concatenate(
            [xn_v[:, _ds(tok[c, 0] & (L - 128), 128)] for c in range(TOPC)], axis=1), BF16))

    def ffn_up(i):
        xs = xs_v[...].astype(BF16)
        for j in range(FB // 128):
            g, u = [_rb(_dot(xs, pltpu.bitcast(w[i, :, _tile(j)], BF16))) for w in (wg_v, wu_v)]
            f_v[_ds(TOPC * i, TOPC), _tile(HP + j)] = _rb(_silu(g)) * u
            yield

    @pl.loop(0, NCB)
    def _(i):
        for c in cp_w(i):
            c.wait()
        order = C_ORDER
        for k, v in (("M", "m" * 8), ("I", "i" + "im" * 16), ("F", "f" + "fm" * 16),
                     ("G", "f" + "fm" * 8 + "f" * 8), ("H", "f" * 17),
                     ("J", "i" + ("i" * 8 + "m" * 8) * 2), ("E", "f" + ("f" * 8 + "m" * 8) * 2),
                     ("K", "i" + ("i" * 4 + "m" * 4) * 4), ("D", "f" + ("f" * 4 + "m" * 4) * 4)):
            order = order.replace(k, v)
        _run(order, i=inverse(jnp.maximum(i - 1, 0), z_v[...]), m=multiply(i), u=ffn_up(i),
             f=forward(jnp.minimum(i + 1, NCB - 1)))

    def ffn_down(i):
        y = None
        for js in ((0, 1, 2), (3, 4, 5), (6, 7, 8)):
            h = jnp.concatenate([f_v[TOPC * j:TOPC * j + TOPC, _tile(HP, 4)] for j in js], axis=1)
            t = _dot_nt(h.astype(BF16), pltpu.bitcast(
                wd_v[words(i, DB), FB * js[0]:FB * (js[-1] + 1)], BF16))
            y = t if y is None else y + t
            if js[-1] == 8:
                yt_v[...] = (0.5 * _rb(_rb(y) * gate[:, :DB])).T
            yield

    def finish(i, yt):
        r = _ds(i * DB, DB)
        skip = 2.0 * skip_v[r, :] + BLK * k0_v[r, :]
        for m in range(4):
            upd = _dot(yt.astype(BF16), hot_v[:, _tile(4 * m, 4)].astype(BF16))
            y = _lane_exchange([f_v[r, _tile(YP + 4 * m + p)] for p in range(4)])
            y = [v if q == 0 else pltpu.roll(v, 128 - q, 1) for q, v in enumerate(y)]
            for q in (0, 2):
                out = []
                for t in (q, q + 1):
                    x, xn = [pltpu.bitcast(w[words(i, DB), _tile(4 * m + t)], BF16).astype(F32)
                             for w in (x_v, xn_v)]
                    h = xn + upd[:, _tile(t)]
                    out.append(x + (y[t] + xn * skip) * (h + h * jnp.tanh(h)))
                o_v[r, _tile(4 * m + q, 2)] = jnp.concatenate(out, axis=1).astype(BF16)
            yield

    cp_d(0).wait()
    _run("", d=ffn_down(0), i=inverse(NCB - 1, z_v))

    @pl.loop(0, D // DB)
    def _(i):
        @pl.when(i + 1 < D // DB)
        def _():
            cp_d(i + 1).wait()

        _run(D_ORDER, o=finish(i, yt_v[...]), d=ffn_down(jnp.minimum(i + 1, D // DB - 1)))
        r = _ds(i * DB, DB)
        pltpu.make_async_copy(o_v.at[r], o_hbm.at[r], sem.at[3]).start()

    pltpu.make_async_copy(o_v, o_hbm, sem.at[3]).wait()


@jax.jit
def pallas_recurrent_scan__ssm_conv_s4__moe_arch_mod__prompt_kernel(
    A_u: jax.Array,
    A_A_re: jax.Array,
    A_A_im: jax.Array,
    A_B_re: jax.Array,
    A_B_im: jax.Array,
    A_C_re: jax.Array,
    A_C_im: jax.Array,
    A_log_dt: jax.Array,
    A_Dskip: jax.Array,
    B_x: jax.Array,
    B_w_r: jax.Array,
    B_w_gate: jax.Array,
    B_w_up: jax.Array,
    B_w_down: jax.Array,
):
    del B_x
    assert A_u.shape == (1, L, D) and A_A_re.shape == (D, N) and B_w_gate.shape == (D, F)
    hbm = pl.BlockSpec(memory_space=pl.ANY)
    vmem = pltpu.VMEM
    out = pl.pallas_call(
        _kernel,
        out_shape=jax.ShapeDtypeStruct((D, L), BF16),
        in_specs=[hbm] * 13,
        out_specs=hbm,
        scratch_shapes=[
            vmem((D // 2, L), U32), vmem((6, D, N), BF16),
            vmem((D,), BF16), vmem((D,), BF16), vmem((D,), BF16),
            vmem((NCB, D // 2, FB), U32), vmem((NCB, D // 2, FB), U32), vmem((D // 2, F), U32),
            vmem((5, 64, 1024), U32), vmem((8, 1024), F32), vmem((D, L), BF16),
            vmem((D // 2, L), U32), vmem((D // 2, L), U32),
            vmem((D, 128 * (K512 + 1)), F32), vmem((4 * CB, 1024), F32),
            vmem((CB, 18 * 128), F32), vmem((D, 128), F32), vmem((D, 128), F32),
            vmem((RAW + D, 128), F32), vmem((TOPC, L), F32), vmem((TOPC, D), F32),
            vmem((DB, TOPC), F32),
            pltpu.SemaphoreType.DMA((5 + NCB + D // DB,)),
        ],
        compiler_params=pltpu.CompilerParams(vmem_limit_bytes=100 * 1024 * 1024),
    )(A_u[0].T, A_A_re, A_A_im, A_B_re, A_B_im, A_C_re, A_C_im, A_log_dt, A_Dskip, B_w_r,
      B_w_gate, B_w_up, B_w_down.T)
    return out.T[None]
```

```python
import jax
import jax.numpy as jnp
import numpy as np
import jax.experimental.pallas as pl
import jax.experimental.pallas.tpu as pltpu

F32, BF16, I32, U32 = jnp.float32, jnp.bfloat16, jnp.int32, jnp.uint32

L, D, N, F = 2048, 576, 128, 4608
TOPC = 8
BLK = 512
CB = 64
NCB = D // CB
FB = F // NCB
DB = 64
NT = (((1,), (1,)), ((), ()))
Q_PAIRS = ((3, 1), (7, 5), (2, 258), (4, 260), (6, 262), (8, 264),
           (516, 772), (520, 776), (1032, 1288), (1544, 1800))
GROUPS = ((6, 7), (8, 9), (3, 5), (0, 1), (2, 4))
K_ORDER = "c ss v v p s p v s p v s p v s p v p s v p s p v"
C_ORDER = "I u I u I u I u G uu G uu F uu H"
D_ORDER = "o d o d o dd o d o d o d o dd o"
L_ORDER = "c m ss m n ssss m n sstt m n tttt n tt"
LT = 4
SPLIT = {8: (1, 2), 1: (2, 9)}
PN = 8
M3 = True
VT = 'float32'
WG = 3


def _round_to_bf16(v):
    u = np.asarray(v, np.float32).view(np.uint32)
    return ((u + 0x7FFF + ((u >> 16) & 1)) & 0xFFFF0000).astype(np.uint32).view(np.float32)


def _cmul(a, b):
    return a[0] * b[0] - a[1] * b[1], a[0] * b[1] + a[1] * b[0]


def _csq(a):
    return (a[0] + a[1]) * (a[0] - a[1]), (a[0] + a[0]) * a[1]


def _cadd(a, b):
    return a[0] + b[0], a[1] + b[1]


def _csub(a, b):
    return a[0] - b[0], a[1] - b[1]


def _add_i(a, b):
    return a[0] - b[1], a[1] + b[0]


def _sub_i(a, b):
    return a[0] + b[1], a[1] - b[0]


def _lane_exchange(r):
    lane = jax.lax.broadcasted_iota(I32, r[0].shape, 1)
    a = [jnp.where((lane & 1) == 1, r[(j + 1) % 4], r[j]) for j in range(4)]
    b = [jnp.where((lane & 2) == 2, a[(j + 2) % 4], a[j]) for j in range(4)]
    return [b[-j % 4] for j in range(4)]


def _rb(v):
    return v.astype(BF16).astype(F32)


def _silu(v):
    h = 0.5 * v
    return h + h * jnp.tanh(h)


def _pack(even, odd):
    return pltpu.pack_elementwise([even, odd], packed_dtype=BF16)


def _unpack(w):
    return [pltpu.unpack_elementwise(w, index=j, packed_dtype=BF16, unpacked_dtype=F32)
            for j in range(2)]


def _tile(t, n=1):
    return slice(128 * t, 128 * (t + n))


def _ds(start, size, align=None):
    if isinstance(start, int):
        return pl.ds(start, size)
    return pl.ds(pl.multiple_of(start, align or size), size)


def _dot(a, b):
    return jnp.dot(a, b, preferred_element_type=F32)


def _dot_nt(a, b):
    return jax.lax.dot_general(a, b, NT, preferred_element_type=F32)


def _run(order, **stages):
    for step in order.replace(" ", ""):
        next(stages[step])
    for stage in stages.values():
        for _ in stage:
            pass


def _pacer(step):
    clock = []

    def after(v):
        if not clock:
            return v
        always = jax.lax.broadcasted_iota(I32, v.shape, 1) < step + 128
        return jnp.where(always, v, jnp.tile(clock[-1], (v.shape[0] // 8, 1)))

    return clock, after


def _sort_rows(v, sizes):
    sub = jax.lax.broadcasted_iota(I32, v.shape, 0)
    for k in sizes:
        j = k // 2
        while j:
            w = jnp.take_along_axis(v, sub ^ j, axis=0)
            v = jnp.where(((sub & j) == 0) == ((sub & k) == 0),
                          jnp.maximum(v, w), jnp.minimum(v, w))
            j //= 2
    return v


def _merge_top(a, b):
    sub = jax.lax.broadcasted_iota(I32, a.shape, 0)
    return _sort_rows(jnp.maximum(a, jnp.take_along_axis(b, 7 - sub, axis=0)), (8,))


def _write_tables(tab_v, edge_v):
    sub = jax.lax.broadcasted_iota(I32, (8, 128), 0)
    lane = jax.lax.broadcasted_iota(I32, (8, 128), 1)
    ang = (((4 * lane + 1) << sub) & (4 * BLK - 1)).astype(F32) * (np.pi / (2 * BLK))
    bits = jnp.cos(ang), jnp.sin(ang)
    known = {1 << s: [jnp.broadcast_to(v[s:s + 1], (8, 128)) for v in bits] for s in range(8)}
    known[0] = [jnp.ones((8, 128), F32), jnp.zeros((8, 128), F32)]

    def times_i(z, n):
        for _ in range(n % 4):
            z = (-z[1], z[0])
        return z

    def power(t):
        if t >= BLK:
            return times_i(power(t - BLK), 1)
        if t not in known:
            low = t & -t if t & (t - 1) else t // 2
            known[t] = _cmul(power(t - low), power(low))
        return known[t]

    def put(cond, z, base):
        return [jnp.where(cond, v, w) for v, w in zip(z, base)]

    def lag_sum(ts, s):
        terms = [times_i(power(t), s * t) for t in ts]
        return [sum(z[c] for z in terms) for c in range(2)]

    def ramp(step):
        z = put((sub & 1) == 1, power(step), known[0])
        for b in (2, 4):
            z = _cmul(z, put((sub & b) == b, power(b * step), known[0]))
        return z

    def store(t, j, col, even, odd):
        for c in range(2):
            tab_v[t, 8 * j:8 * j + 8, _tile(col + c)] = _pack(even[c], odd[c])

    ramp2, ramp16 = ramp(2), ramp(16)
    for p in range(4):
        col = []
        for e in range(2):
            q0, q1 = (e - p) % 4, (e + 2 - p) % 4
            z = [_cmul(ramp2, put((sub & 1) == 1, power(127 * q1 + e), power(127 * q0 + e)))]
            for _ in range(8):
                z.append(_cmul(z[-1], power(16)))
            z[0] = put(2 * sub + e < ((2 * sub + e - p) & 3), z[8], z[0])
            col.append(z)
        for j in range(8):
            store(0, j, 2 * p, col[0][j], col[1][j])

    lag_exp = _round_to_bf16(np.arange(L)).astype(np.int64)
    c = np.arange(128)
    gc, gd, g4, go, g2 = [
        np.concatenate([Q_PAIRS[v][e] + 8 * np.arange(32) for e in range(2) for v in vs])
        for vs in GROUPS]
    g1 = np.where((c >= 63) & (c < 127), g4, np.roll(go, 63))
    g3, ge = np.where(c < 64, go, g4), np.where(c == 127, gc, gd)
    rows16 = {}

    def ramp_from(t):
        if t not in rows16:
            back = [d for d in (8, 128) if t - d in rows16]
            rows16[t] = (_cmul(rows16[t - back[0]], power(back[0])) if back
                         else _cmul(ramp16, power(t)))
        return rows16[t]

    def lags(e, m, phase=None):
        ts = [int(l) - BLK * m for l in np.nonzero(lag_exp == e)[0] if 0 < l - BLK * m <= BLK]
        return [t for t in ts if phase is None or t % 4 == phase]

    def rows(tss, s):
        z = [known[0][1]] * 2
        if tss[0]:
            half = len(tss[0]) // 2
            z = ramp_from(tss[0][half])
            if half:
                assert tss[0][half] % 4 == 0 and len(tss[0]) % 2 == 1
                box = 1.0 + 2.0 * lag_sum(range(1, half + 1), s)[0]
                z = [v * box for v in z]
        for r, ts in enumerate(tss):
            if ts != [t + 16 * r for t in tss[0]]:
                z = put(sub == r, lag_sum(ts, s), z)
        return z

    for j in range(8):
        for p, g in enumerate((g4, g1, g2, g3)):
            store(1, j, 2 * p, *[rows([lags(v, 0, p) for v in g[16 * j + e:16 * j + 16:2]], 0)
                                 for e in range(2)])
        for m, g in ((1, gc), (2, ge), (3, gd)):
            for s in range(4):
                store(1 + m, j, 2 * s, *[rows([lags(v, m) for v in g[16 * j + e:16 * j + 16:2]], s)
                                         for e in range(2)])
    for s in range(4):
        edge_v[:, _tile(2 * s, 2)] = jnp.tile(
            jnp.concatenate(lag_sum(lags(BLK, 1), s), axis=1), (CB // 8, 1))


def _ssm_powers(par, dt):
    a_re, a_im, b_re, b_im, c_re, c_im = par
    mag = jnp.exp(dt * a_re)
    ang = dt * a_im
    pw = {1: (mag * jnp.cos(ang), mag * jnp.sin(ang))}
    for k in range(9):
        pw[2 << k] = _csq(pw[1 << k])
    sc = dt * (2.0 / BLK)
    w = _cmul((c_re, c_im), (b_re * sc, b_im * sc))
    w1, w2 = _cmul(w, pw[1]), _cmul(w, pw[2])
    return [pw[8], pw[16], pw[2], pw[4], pw[512],
            w1, _cmul(w1, pw[2]), w2, _cmul(w2, pw[256])], w[0]


def _ssm_products(pw):
    a8, a16, a2, a4, a512, w1, w3, w2, w258 = pw
    sub = jax.lax.broadcasted_iota(I32, (8, 128), 0)
    lane = jax.lax.broadcasted_iota(I32, (8, 128), 1)
    lo = sub < 4

    def pick(z, rows):
        return [jnp.take_along_axis(v, rows, axis=0) for v in z]

    def pair(x, y, h):
        r = [pltpu.roll(v, 4, 0) for v in y]
        return [jnp.where(lo, s, v) if h else jnp.where(lo, v, s) for v, s in zip(x, r)]

    out = []
    for h in range(2):
        p_rows, q_rows = 4 * h + ((sub + 2 * h) & 3), 4 * h + (sub & 3)
        step, s2, s512 = pick(a16, p_rows), pick(a2, q_rows), pick(a512, q_rows)
        p = [[jnp.where(lo, one, v) for one, v in zip((1.0, 0.0), pick(a8, p_rows))]]
        for _ in range(15):
            p.append(_cmul(p[-1], step))
        q = [pair(w3, w1, h)]
        q += [_cmul(q[0], pick(a4, q_rows)), pair(w2, w258, h)]
        for _ in range(3):
            q.append(_cmul(q[-1], s2))
        q += [_cmul(q[3], s512), _cmul(q[5], s512)]
        for _ in range(2):
            q.append(_cmul(q[-1], s512))
        out.append([_dot_nt(*[jnp.concatenate([z[j] for z in zs], axis=0).astype(BF16)
                              for zs in (q, p)]) for j in range(2)])
    first = ((lane - sub) & 3) == 0
    return [jnp.where(first, out[0][0][v:v + 8], out[1][0][v:v + 8])
            - jnp.where(first, out[0][1][v:v + 8], out[1][1][v:v + 8]) for v in range(0, 80, 8)]


def _kernel(x_hbm, are_hbm, aim_hbm, bre_hbm, bim_hbm, cre_hbm, cim_hbm, ldt_hbm, dsk_hbm, wr_hbm,
            wg_hbm, wu_hbm, wd_hbm, o_hbm,
            x_v, par_v, ldt_v, dsk_v, wr_v, wg_v, wu_v, wd_v, tab_v, edge_v, o_v,
            xn_v, ph_v, kf_v, uf_v, z_v, y_v, pw_v, dt_v, k0_v, skip_v, raw_v, vec_v,
            hot_v, xs_v, h_v, yr_v, yt_v, sem):
    def rows(i):
        return _ds(i * CB, CB)

    def words(i, n):
        return _ds(i * (n // 2), n // 2)

    pars = (are_hbm, aim_hbm, bre_hbm, bim_hbm, cre_hbm, cim_hbm)
    cp_dt = pltpu.make_async_copy(ldt_hbm, ldt_v, sem.at[0])
    cp_head, cp_rest = [
        [pltpu.make_async_copy(p.at[r], par_v.at[j, r], sem.at[k]) for j, p in enumerate(pars)]
        for k, r in ((1, pl.ds(0, 2 * CB)), (4, pl.ds(2 * CB, D - 2 * CB)))]
    cp_x = [pltpu.make_async_copy(s, d, sem.at[2])
            for s, d in ((x_hbm.bitcast(U32), x_v), (dsk_hbm, dsk_v), (wr_hbm, wr_v))]

    def cp_w(i):
        c = _ds(i * WG * FB, WG * FB)
        return [pltpu.make_async_copy(s.bitcast(U32).at[:, c], d.at[:, c], sem.at[5 + i])
                for s, d in ((wg_hbm, wg_v), (wu_hbm, wu_v))]

    def cp_d(i):
        return pltpu.make_async_copy(wd_hbm.bitcast(U32).at[words(i, DB)], wd_v.at[words(i, DB)],
                                     sem.at[5 + NCB // WG + i])

    for c in [cp_dt] + cp_head + cp_rest + cp_x:
        c.start()

    def table(t, lo, n):
        return pltpu.bitcast(tab_v[t, :, _tile(lo, n)], BF16)

    raw_v[...] = jnp.zeros(raw_v.shape, F32)
    vec_v[...] = jnp.zeros(vec_v.shape, VT)
    _write_tables(tab_v, edge_v)

    cp_dt.wait()
    dt_row = _rb(jnp.exp(ldt_v[...].astype(F32).reshape(1, D)))
    dt_v[...] = jnp.broadcast_to(dt_row, (128, D)).T
    for c in cp_head:
        c.wait()
    z_v[...] = jnp.zeros(z_v.shape, F32)

    def kernel_powers(i, after):
        par = [par_v[t, rows(i), :].astype(F32) for t in range(6)]
        k0 = []
        for g in range(0, CB, PN):
            pw, w = _ssm_powers([v[g:g + PN] for v in par], after(dt_v[_ds(i * CB + g, PN), :]))
            pw_v[g:g + PN, :] = jnp.concatenate([v for z in pw for v in z], axis=1)
            k0_v[_ds(i * CB + g, PN), :] = jnp.broadcast_to(
                jnp.sum(w, axis=1, keepdims=True), (PN, 128))
            yield

    def kernel_values(pw, clock):
        for g in range(0, CB, 8):
            out = _ssm_products([(pw[g:g + 8, _tile(2 * t)], pw[g:g + 8, _tile(2 * t + 1)])
                                 for t in range(9)])
            for v in range(10):
                raw_v[v, g:g + 8, :] = out[v]
            clock.append(out[0])
            yield

    def kernel_vectors(i, raw):
        sub = jax.lax.broadcasted_iota(I32, (8, 128), 0)
        lane = jax.lax.broadcasted_iota(I32, (8, 128), 1)
        odd = ((lane - sub) & 1) == 1
        own = ((lane - sub) & 2) == ((sub & 4) >> 1)
        perm = (4 * (lane & 31) + ((sub + ((sub & 4) >> 1)) & 3) + (lane >> 5)) & 127
        u = [jnp.where(odd, pltpu.roll(raw[v1, g:g + 8], 1, 1), raw[v0, g:g + 8])
             for v0, v1 in GROUPS for g in range(0, CB, 8)]
        u = [jnp.where(own, v, pltpu.roll(pltpu.roll(v, 4, 0), 2, 1)) for v in u]
        u = [jnp.take_along_axis(v, perm, axis=1) for v in u]
        gc, gd, g4, go, g2 = [u[t:t + CB // 8] for t in range(0, len(u), CB // 8)]
        mid, last = (lane >= 63) & (lane < 127), lane == 127
        g1 = [jnp.where(mid, a, pltpu.roll(b, 63, 1)) for a, b in zip(g4, go)]
        g3 = [jnp.where(lane < 64, b, a) for a, b in zip(g4, go)]
        ge = [jnp.where(last, a, b) for a, b in zip(gc, gd)]
        for t, v in enumerate((g4, g1, g2, g3, gc, ge, gd)):
            vec_v[t] = jnp.concatenate(v, axis=0).astype(VT)
        kf_v[rows(i), _tile(32)] = jnp.broadcast_to(jnp.sum(
            jnp.concatenate([jnp.where(last, a, 0.0) for a in g4], axis=0),
            axis=1, keepdims=True), (CB, 128))
        yield

    def kernel_spectrum(i, vec, clock):
        for m in (1, 3, 2):
            for t in (0, 4):
                f = _dot(vec[3 + m].astype(BF16), table(1 + m, t, 4))
                kf_v[rows(i), _tile(8 * m + t, 4)] = f
                clock.append(f[0:8, 0:128])
                yield
        for p in range(2):
            a, b = [_dot(vec[t].astype(BF16), table(1, 2 * t, 2)) for t in (p, p + 2)]
            kf_v[rows(i), _tile(4 * p, 2)] = a + b
            kf_v[rows(i), _tile(4 * p + 2, 2)] = a - b
            clock.append(a[0:8, 0:128])
            yield

    _run("", p=kernel_powers(0, lambda v: v))
    for j in range(NCB // WG):
        for c in cp_w(j):
            c.start()

    @pl.loop(0, NCB)
    def _(i):
        @pl.when(i == 1)
        def _():
            for c in cp_rest:
                c.wait()

        clock, after = _pacer(i)
        _run(K_ORDER, s=kernel_spectrum(jnp.maximum(i - 2, 0), vec_v[...], clock),
             c=kernel_vectors(jnp.maximum(i - 1, 0), raw_v[...]),
             v=kernel_values(pw_v[...], clock),
             p=kernel_powers(jnp.minimum(i + 1, NCB - 1), after))

    for c in cp_x:
        c.wait()
    skip_v[...] = jnp.broadcast_to(dsk_v[...].astype(F32).reshape(1, D), (128, D)).T
    wr = jnp.broadcast_to(wr_v[...].astype(F32).reshape(1, D), (TOPC, D)).astype(BF16)
    eps = float(_round_to_bf16(1e-5))
    mean, score = [], []

    def token_mean():
        for t in range(0, L // 128, LT):
            m = _dot(jnp.ones((8, D), BF16), pltpu.bitcast(x_v[:, _tile(t, LT)], BF16)) * (1.0 / D)
            mean.extend(m[:, _tile(j)] for j in range(LT))
            yield

    def normalize():
        for t0 in range(0, L // 128, LT):
            out = []
            for t in range(t0, t0 + LT):
                mb, sq, cen = _rb(mean[t]), [0.0, 0.0], []
                for r in range(0, D // 2, 8):
                    d = [v - mb for v in _unpack(x_v[r:r + 8, _tile(t)])]
                    sq = [a + v * v for a, v in zip(sq, d)]
                    cen.append(_pack(*d))
                var = (jnp.sum(sq[0] + sq[1], axis=0, keepdims=True) * (1.0 / D)
                       - jnp.square(mean[t] - mb))
                inv = 0.5 / _rb(jnp.sqrt(_rb(_rb(jnp.maximum(var, 0.0)) + eps)))
                out.append(jnp.concatenate(
                    [_pack(*[v * inv for v in _unpack(w)]) for w in cen], axis=0))
            out = jnp.concatenate(out, axis=1)
            xn_v[:, _tile(t0, LT)] = out
            score.append(_rb(2.0 * _dot(wr, pltpu.bitcast(out, BF16))))
            yield

    _run(L_ORDER, s=kernel_spectrum(NCB - 2, vec_v[...], []), c=kernel_vectors(NCB - 1, raw_v),
         t=kernel_spectrum(NCB - 1, vec_v, []), m=token_mean(), n=normalize())
    score = jnp.concatenate(score, axis=1)
    for i in range(D // DB):
        cp_d(i).start()

    def split_phases(i):
        r = pl.ds(i * CB // 2, CB // 2)
        for m in range(4):
            v = [xn_v[r, _tile(4 * m + q)] for q in range(4)]
            v = _lane_exchange([w if q == 0 else pltpu.roll(w, q, 1) for q, w in enumerate(v)])
            for p in range(4):
                ph_v[r, _tile(4 * m + p)] = v[p]

    def forward(i, clock):
        for h in range(0, CB, 32):
            for p in range(2):
                a, b = [_dot(
                    pltpu.bitcast(jnp.concatenate(
                        [ph_v[_ds(i * (CB // 2) + g // 2, 8), _tile(4 * m + t)]
                         for g in (h, h + 16) for m in range(4)], axis=0), BF16),
                    table(0, 2 * t, 2)) for t in (p, p + 2)]
                uf_v[4 * h:4 * h + 128, _tile(4 * p, 2)] = a + b
                uf_v[4 * h:4 * h + 128, _tile(4 * p + 2, 2)] = a - b
                for r in range(0, 128, 16):
                    clock.append(a[r:r + 8, 0:128])
                    yield

    def multiply(i, uf, after):
        def pair(src, r, t):
            return src[r, _tile(t)], src[r, _tile(t + 1)]

        for g in range(0, CB, 8):
            r = _ds(i * CB + g, 8)
            ru = [slice(64 * (g // 16) + 16 * m + g % 16, 64 * (g // 16) + 16 * m + g % 16 + 8)
                  for m in range(4)]
            for s, ops in enumerate(((_cadd, _csub), (_add_i, _sub_i))):
                ks, us = [], []
                for t, op in zip((s, s + 2), ops):
                    k = [op(pair(kf_v, r, 2 * s), pair(kf_v, r, 2 * s + 4))]
                    k += [pair(kf_v, r, 8 * m + 2 * t) for m in (1, 2, 3)]
                    k[1] = [v + kf_v[r, _tile(32)] * edge_v[g:g + 8, _tile(2 * t + c)]
                            for c, v in enumerate(k[1])]
                    k = [k[0]] + [_sub_i(k[m], k[m - 1]) for m in (1, 2, 3)]
                    ks.append([(c, d - c, c + d) if M3 else (c, d) for c, d in k])
                    u = [op(pair(uf, v, 2 * s), pair(uf, v, 2 * s + 4)) for v in ru]
                    us.append([(a + b, a, b) if M3 else (a, b) for a, b in u])
                for n in range(4):
                    z = []
                    for k, u in zip(ks, us):
                        if not M3:
                            acc = _cmul(k[0], u[n] if z else (after(u[n][0]), u[n][1]))
                            for m in range(1, n + 1):
                                acc = _cadd(acc, _cmul(k[m], u[n - m]))
                            z.append(acc)
                            continue
                        acc = [v * w for v, w in zip(k[0], u[n])]
                        if not z:
                            acc[0] = after(acc[0])
                        for m in range(1, n + 1):
                            acc = [a + v * w for a, v, w in zip(acc, k[m], u[n - m])]
                        z.append((acc[0] - acc[2], acc[0] + acc[1]))
                    for t, v in enumerate(_cadd(*z) + _csub(*z)):
                        z_v[pl.ds(4 * g + 8 * n, 8), _tile(4 * s + t)] = v
                    yield

    def inverse(i, z, clock):
        for h in range(0, CB, 32):
            for p, ops in enumerate(((_cadd, _csub), (_sub_i, _add_i))):
                a, c = [[z[4 * h:4 * h + 128, _tile(4 * s + 2 * p + t)] for t in range(2)]
                        for s in range(2)]
                y = [_dot_nt(jnp.concatenate(op(a, c), axis=1).astype(BF16),
                             table(0, 2 * p + 4 * t, 2)) for t, op in enumerate(ops)]
                for g in range(0, 32, 8):
                    for m in range(4):
                        for t in range(2):
                            y_v[_ds(i * CB + h + g, 8), _tile(4 * m + p + 2 * t)] = (
                                y[t][4 * g + 8 * m:4 * g + 8 * m + 8])
                for r in range(0, 128, 16):
                    clock.append(y[0][r:r + 8])
                    yield

    bits = pltpu.bitcast(jnp.where(score == 0.0, 0.0, score), I32) >> 16
    pos = jax.lax.broadcasted_iota(I32, (TOPC, L), 1)
    key = ((bits ^ ((bits >> 15) & 0x7FFF)) << 11) + (0x38000000 + L - 1 - pos)
    key = pltpu.bitcast(key, F32)
    sub = jax.lax.broadcasted_iota(I32, (TOPC, 128), 0)
    dense = []
    for t0 in (0, 8):
        v = key[:, _tile(t0)]
        for t in range(1, 8):
            v = jnp.where(sub == t, key[:, _tile(t0 + t)], v)
        dense.append(v)
    split_phases(0)
    _run("", f=forward(0, []))
    top = _merge_top(*[_sort_rows(v, (2, 4, 8)) for v in dense])
    for step, count in ((8, 16), (1, 8)):
        top = [top] + [pltpu.roll(top, step * k, 1) for k in range(1, count)]
        while len(top) > 1:
            top = [_merge_top(a, b) for a, b in zip(top[0::2], top[1::2])]
        top = top[0]
        for i in range(*SPLIT[step]):
            split_phases(i)
    hot_v[...] = jnp.where(key == jnp.tile(top, (1, L // 128)), 1.0, 0.0)
    top = pltpu.bitcast(top, I32) - 0x38000000
    tb = top >> 11
    gate = _rb(jax.nn.sigmoid(pltpu.bitcast((tb ^ ((tb >> 15) & 0x7FFF)) << 16, F32)))
    tok = (L - 1) - (top & (L - 1))
    pick = (tok & 127) == jax.lax.broadcasted_iota(I32, (TOPC, 128), 1)
    xs_v[...] = _dot_nt(
        jnp.concatenate([jnp.where(pick & (sub == c), 2.0, 0.0) for c in range(TOPC)],
                        axis=1).astype(BF16),
        pltpu.bitcast(jnp.concatenate(
            [xn_v[:, _ds(tok[c, 0] & (L - 128), 128)] for c in range(TOPC)], axis=1), BF16))

    def ffn_up(i):
        acc = [0.0, 0.0]
        for j in range(0, D, 128):
            n = min(128, D - j)
            for t, w in enumerate((wg_v, wu_v)):
                acc[t] = acc[t] + _dot(
                    xs_v[:, j:j + n].astype(BF16),
                    pltpu.bitcast(w[j // 2:(j + n) // 2, _ds(i * FB, FB)], BF16))
                yield
        h_v[:, _ds(i * FB, FB)] = _rb(_silu(_rb(acc[0]))) * _rb(acc[1])

    @pl.loop(0, NCB)
    def _(i):
        for j in range(NCB // WG):
            @pl.when(i == j * WG)
            def _():
                for c in cp_w(j):
                    c.wait()

        clock, after = _pacer(i)
        _run(C_ORDER.replace('I', 'im' * 8).replace('F', 'fm' * 8).replace('J', 'imimimim' * 2 + 'm').replace('G', 'fmfmmfmfmm' * 2).replace('E', 'fmfmmfmm' * 2 + 'fmfm').replace('H', 'f' * 8), i=inverse(jnp.maximum(i - 1, 0), z_v[...], clock),
             m=multiply(i, uf_v[...], after), u=ffn_up(i),
             f=forward(jnp.minimum(i + 1, NCB - 1), clock))

    def ffn_down(i):
        y = 0.0
        for j in range(0, F, FB):
            y = y + _dot_nt(h_v[:, j:j + FB].astype(BF16),
                            pltpu.bitcast(wd_v[words(i, DB), j:j + FB], BF16))
            if j + FB == F:
                yr_v[...] = 0.5 * _rb(_rb(y) * gate[:, :DB])
            yield

    def finish(i, yt):
        for g in range(0, DB, 32):
            r, rw = _ds(i * DB + g, 32), _ds(i * (DB // 2) + g // 2, 16)
            skip = 2.0 * skip_v[r, :] + BLK * k0_v[r, :]
            for m in range(4):
                upd = _dot(yt[g:g + 32].astype(BF16), hot_v[:, _tile(4 * m, 4)].astype(BF16))
                y = _lane_exchange([y_v[r, _tile(4 * m + p)] for p in range(4)])
                y = [v if q == 0 else pltpu.roll(v, 128 - q, 1) for q, v in enumerate(y)]
                for q in (0, 2):
                    out = []
                    for t in (q, q + 1):
                        x, xn = [pltpu.bitcast(w[rw, _tile(4 * m + t)], BF16).astype(F32)
                                 for w in (x_v, xn_v)]
                        h = xn + upd[:, _tile(t)]
                        out.append(x + (y[t] + xn * skip) * (h + h * jnp.tanh(h)))
                    o_v[r, _tile(4 * m + q, 2)] = jnp.concatenate(out, axis=1).astype(BF16)
                yield

    cp_d(0).wait()
    cp_d(1).wait()
    _run("", d=ffn_down(0))
    yt_v[...] = yr_v[...].T
    _run("", d=ffn_down(1), i=inverse(NCB - 1, z_v, []))

    @pl.loop(0, D // DB)
    def _(i):
        @pl.when(i + 2 < D // DB)
        def _():
            cp_d(i + 2).wait()

        yt = yt_v[...]
        yt_v[...] = yr_v[...].T
        _run(D_ORDER, o=finish(i, yt), d=ffn_down(jnp.minimum(i + 2, D // DB - 1)))
        r = _ds(i * DB, DB)
        pltpu.make_async_copy(o_v.at[r], o_hbm.at[r], sem.at[3]).start()

    pltpu.make_async_copy(o_v, o_hbm, sem.at[3]).wait()


@jax.jit
def pallas_recurrent_scan__ssm_conv_s4__moe_arch_mod__prompt_kernel(
    A_u: jax.Array,
    A_A_re: jax.Array,
    A_A_im: jax.Array,
    A_B_re: jax.Array,
    A_B_im: jax.Array,
    A_C_re: jax.Array,
    A_C_im: jax.Array,
    A_log_dt: jax.Array,
    A_Dskip: jax.Array,
    B_x: jax.Array,
    B_w_r: jax.Array,
    B_w_gate: jax.Array,
    B_w_up: jax.Array,
    B_w_down: jax.Array,
):
    del B_x
    assert A_u.shape == (1, L, D) and A_A_re.shape == (D, N) and B_w_gate.shape == (D, F)
    hbm = pl.BlockSpec(memory_space=pl.ANY)
    vmem = pltpu.VMEM
    out = pl.pallas_call(
        _kernel,
        out_shape=jax.ShapeDtypeStruct((D, L), BF16),
        in_specs=[hbm] * 13,
        out_specs=hbm,
        scratch_shapes=[
            vmem((D // 2, L), U32), vmem((6, D, N), BF16),
            vmem((D,), BF16), vmem((D,), BF16), vmem((D,), BF16),
            vmem((D // 2, F), U32), vmem((D // 2, F), U32), vmem((D // 2, F), U32),
            vmem((5, 64, 1024), U32), vmem((CB, 1024), F32), vmem((D, L), BF16),
            vmem((D // 2, L), U32), vmem((D // 2, L), U32),
            vmem((D, 33 * 128), F32), vmem((4 * CB, 1024), F32), vmem((4 * CB, 1024), F32),
            vmem((D, L), F32), vmem((CB, 18 * 128), F32),
            vmem((D, 128), F32), vmem((D, 128), F32), vmem((D, 128), F32),
            vmem((10, CB, 128), F32), vmem((7, CB, 128), VT),
            vmem((TOPC, L), F32), vmem((TOPC, D), F32), vmem((TOPC, F), F32),
            vmem((TOPC, DB), F32), vmem((DB, TOPC), F32),
            pltpu.SemaphoreType.DMA((5 + NCB // WG + D // DB,)),
        ],
        compiler_params=pltpu.CompilerParams(vmem_limit_bytes=100 * 1024 * 1024),
    )(A_u[0].T, A_A_re, A_A_im, A_B_re, A_B_im, A_C_re, A_C_im, A_log_dt, A_Dskip, B_w_r,
      B_w_gate, B_w_up, B_w_down.T)
    return out.T[None]
```

```python
import jax
import jax.numpy as jnp
import numpy as np
import jax.experimental.pallas as pl
import jax.experimental.pallas.tpu as pltpu

F32, BF16, I32, U32 = jnp.float32, jnp.bfloat16, jnp.int32, jnp.uint32

L, D, N, F = 2048, 576, 128, 4608
TOPC = 8
BLK = 512
CB = 64
NCB = D // CB
FB = F // NCB
DB = 64
NT = (((1,), (1,)), ((), ()))
Q_PAIRS = ((3, 1), (7, 5), (2, 258), (4, 260), (6, 262), (8, 264),
           (516, 772), (520, 776), (1032, 1288), (1544, 1800))
GROUPS = ((6, 7), (8, 9), (3, 5), (0, 1), (2, 4))
K_ORDER = "c ss v v p s p v s p v s p v s p v p s v p s p v"
C_ORDER = "I u I u I u I u G uu G uu F uu H"
D_ORDER = "o d o d o dd o d o d o d o dd o"
L_ORDER = "c m ss m n ssss m n sstt m n tttt n tt"
LT = 4
NT_ = 4
EARLY = 4
MID = 5
PN = 8
PI = 32
P_ORDER = "oo I oo I oo I o I o"
M3 = True
VT = 'float32'
WG = 3


def _round_to_bf16(v):
    u = np.asarray(v, np.float32).view(np.uint32)
    return ((u + 0x7FFF + ((u >> 16) & 1)) & 0xFFFF0000).astype(np.uint32).view(np.float32)


def _cmul(a, b):
    return a[0] * b[0] - a[1] * b[1], a[0] * b[1] + a[1] * b[0]


def _csq(a):
    return (a[0] + a[1]) * (a[0] - a[1]), (a[0] + a[0]) * a[1]


def _cadd(a, b):
    return a[0] + b[0], a[1] + b[1]


def _csub(a, b):
    return a[0] - b[0], a[1] - b[1]


def _add_i(a, b):
    return a[0] - b[1], a[1] + b[0]


def _sub_i(a, b):
    return a[0] + b[1], a[1] - b[0]


def _lane_exchange(r):
    lane = jax.lax.broadcasted_iota(I32, r[0].shape, 1)
    a = [jnp.where((lane & 1) == 1, r[(j + 1) % 4], r[j]) for j in range(4)]
    b = [jnp.where((lane & 2) == 2, a[(j + 2) % 4], a[j]) for j in range(4)]
    return [b[-j % 4] for j in range(4)]


def _rb(v):
    return v.astype(BF16).astype(F32)


def _silu(v):
    h = 0.5 * v
    return h + h * jnp.tanh(h)


def _pack(even, odd):
    return pltpu.pack_elementwise([even, odd], packed_dtype=BF16)


def _unpack(w):
    return [pltpu.unpack_elementwise(w, index=j, packed_dtype=BF16, unpacked_dtype=F32)
            for j in range(2)]


def _tile(t, n=1):
    return slice(128 * t, 128 * (t + n))


def _ds(start, size, align=None):
    if isinstance(start, int):
        return pl.ds(start, size)
    return pl.ds(pl.multiple_of(start, align or size), size)


def _dot(a, b):
    return jnp.dot(a, b, preferred_element_type=F32)


def _dot_nt(a, b):
    return jax.lax.dot_general(a, b, NT, preferred_element_type=F32)


def _run(order, **stages):
    for step in order.replace(" ", ""):
        next(stages[step])
    for stage in stages.values():
        for _ in stage:
            pass


def _pacer(step):
    clock = []

    def after(v):
        if not clock:
            return v
        always = jax.lax.broadcasted_iota(I32, v.shape, 1) < step + 128
        return jnp.where(always, v, jnp.tile(clock[-1], (v.shape[0] // 8, 1)))

    return clock, after


def _sort_rows(v, sizes):
    sub = jax.lax.broadcasted_iota(I32, v.shape, 0)
    for k in sizes:
        j = k // 2
        while j:
            w = jnp.take_along_axis(v, sub ^ j, axis=0)
            v = jnp.where(((sub & j) == 0) == ((sub & k) == 0),
                          jnp.maximum(v, w), jnp.minimum(v, w))
            j //= 2
    return v


def _merge_top(a, b):
    sub = jax.lax.broadcasted_iota(I32, a.shape, 0)
    return _sort_rows(jnp.maximum(a, jnp.take_along_axis(b, 7 - sub, axis=0)), (8,))


def _write_tables(tab_v, edge_v):
    sub = jax.lax.broadcasted_iota(I32, (8, 128), 0)
    lane = jax.lax.broadcasted_iota(I32, (8, 128), 1)
    ang = (((4 * lane + 1) << sub) & (4 * BLK - 1)).astype(F32) * (np.pi / (2 * BLK))
    bits = jnp.cos(ang), jnp.sin(ang)
    known = {1 << s: [jnp.broadcast_to(v[s:s + 1], (8, 128)) for v in bits] for s in range(8)}
    known[0] = [jnp.ones((8, 128), F32), jnp.zeros((8, 128), F32)]

    def times_i(z, n):
        for _ in range(n % 4):
            z = (-z[1], z[0])
        return z

    def power(t):
        if t >= BLK:
            return times_i(power(t - BLK), 1)
        if t not in known:
            low = t & -t if t & (t - 1) else t // 2
            known[t] = _cmul(power(t - low), power(low))
        return known[t]

    def put(cond, z, base):
        return [jnp.where(cond, v, w) for v, w in zip(z, base)]

    def lag_sum(ts, s):
        terms = [times_i(power(t), s * t) for t in ts]
        return [sum(z[c] for z in terms) for c in range(2)]

    def ramp(step):
        z = put((sub & 1) == 1, power(step), known[0])
        for b in (2, 4):
            z = _cmul(z, put((sub & b) == b, power(b * step), known[0]))
        return z

    def store(t, j, col, even, odd):
        for c in range(2):
            tab_v[t, 8 * j:8 * j + 8, _tile(col + c)] = _pack(even[c], odd[c])

    ramp2, ramp16 = ramp(2), ramp(16)
    for p in range(4):
        col = []
        for e in range(2):
            q0, q1 = (e - p) % 4, (e + 2 - p) % 4
            z = [_cmul(ramp2, put((sub & 1) == 1, power(127 * q1 + e), power(127 * q0 + e)))]
            for _ in range(8):
                z.append(_cmul(z[-1], power(16)))
            z[0] = put(2 * sub + e < ((2 * sub + e - p) & 3), z[8], z[0])
            col.append(z)
        for j in range(8):
            store(0, j, 2 * p, col[0][j], col[1][j])

    lag_exp = _round_to_bf16(np.arange(L)).astype(np.int64)
    c = np.arange(128)
    gc, gd, g4, go, g2 = [
        np.concatenate([Q_PAIRS[v][e] + 8 * np.arange(32) for e in range(2) for v in vs])
        for vs in GROUPS]
    g1 = np.where((c >= 63) & (c < 127), g4, np.roll(go, 63))
    g3, ge = np.where(c < 64, go, g4), np.where(c == 127, gc, gd)
    rows16 = {}

    def ramp_from(t):
        if t not in rows16:
            back = [d for d in (8, 128) if t - d in rows16]
            rows16[t] = (_cmul(rows16[t - back[0]], power(back[0])) if back
                         else _cmul(ramp16, power(t)))
        return rows16[t]

    def lags(e, m, phase=None):
        ts = [int(l) - BLK * m for l in np.nonzero(lag_exp == e)[0] if 0 < l - BLK * m <= BLK]
        return [t for t in ts if phase is None or t % 4 == phase]

    def rows(tss, s):
        z = [known[0][1]] * 2
        if tss[0]:
            half = len(tss[0]) // 2
            z = ramp_from(tss[0][half])
            if half:
                assert tss[0][half] % 4 == 0 and len(tss[0]) % 2 == 1
                box = 1.0 + 2.0 * lag_sum(range(1, half + 1), s)[0]
                z = [v * box for v in z]
        for r, ts in enumerate(tss):
            if ts != [t + 16 * r for t in tss[0]]:
                z = put(sub == r, lag_sum(ts, s), z)
        return z

    for j in range(8):
        for p, g in enumerate((g4, g1, g2, g3)):
            store(1, j, 2 * p, *[rows([lags(v, 0, p) for v in g[16 * j + e:16 * j + 16:2]], 0)
                                 for e in range(2)])
        for m, g in ((1, gc), (2, ge), (3, gd)):
            for s in range(4):
                store(1 + m, j, 2 * s, *[rows([lags(v, m) for v in g[16 * j + e:16 * j + 16:2]], s)
                                         for e in range(2)])
    for s in range(4):
        edge_v[:, _tile(2 * s, 2)] = jnp.tile(
            jnp.concatenate(lag_sum(lags(BLK, 1), s), axis=1), (CB // 8, 1))


def _ssm_powers(par, dt):
    a_re, a_im, b_re, b_im, c_re, c_im = par
    mag = jnp.exp(dt * a_re)
    ang = dt * a_im
    pw = {1: (mag * jnp.cos(ang), mag * jnp.sin(ang))}
    for k in range(9):
        pw[2 << k] = _csq(pw[1 << k])
    sc = dt * (2.0 / BLK)
    w = _cmul((c_re, c_im), (b_re * sc, b_im * sc))
    w1, w2 = _cmul(w, pw[1]), _cmul(w, pw[2])
    return [pw[8], pw[16], pw[2], pw[4], pw[512],
            w1, _cmul(w1, pw[2]), w2, _cmul(w2, pw[256])], w[0]


def _ssm_products(pw):
    a8, a16, a2, a4, a512, w1, w3, w2, w258 = pw
    sub = jax.lax.broadcasted_iota(I32, (8, 128), 0)
    lane = jax.lax.broadcasted_iota(I32, (8, 128), 1)
    lo = sub < 4

    def pick(z, rows):
        return [jnp.take_along_axis(v, rows, axis=0) for v in z]

    def pair(x, y, h):
        r = [pltpu.roll(v, 4, 0) for v in y]
        return [jnp.where(lo, s, v) if h else jnp.where(lo, v, s) for v, s in zip(x, r)]

    out = []
    for h in range(2):
        p_rows, q_rows = 4 * h + ((sub + 2 * h) & 3), 4 * h + (sub & 3)
        step, s2, s512 = pick(a16, p_rows), pick(a2, q_rows), pick(a512, q_rows)
        p = [[jnp.where(lo, one, v) for one, v in zip((1.0, 0.0), pick(a8, p_rows))]]
        for _ in range(15):
            p.append(_cmul(p[-1], step))
        q = [pair(w3, w1, h)]
        q += [_cmul(q[0], pick(a4, q_rows)), pair(w2, w258, h)]
        for _ in range(3):
            q.append(_cmul(q[-1], s2))
        q += [_cmul(q[3], s512), _cmul(q[5], s512)]
        for _ in range(2):
            q.append(_cmul(q[-1], s512))
        out.append([_dot_nt(*[jnp.concatenate([z[j] for z in zs], axis=0).astype(BF16)
                              for zs in (q, p)]) for j in range(2)])
    first = ((lane - sub) & 3) == 0
    return [jnp.where(first, out[0][0][v:v + 8], out[1][0][v:v + 8])
            - jnp.where(first, out[0][1][v:v + 8], out[1][1][v:v + 8]) for v in range(0, 80, 8)]


def _kernel(x_hbm, are_hbm, aim_hbm, bre_hbm, bim_hbm, cre_hbm, cim_hbm, ldt_hbm, dsk_hbm, wr_hbm,
            wg_hbm, wu_hbm, wd_hbm, o_hbm,
            x_v, par_v, ldt_v, dsk_v, wr_v, wg_v, wu_v, wd_v, tab_v, edge_v, o_v,
            xn_v, ph_v, kf_v, uf_v, z_v, y_v, pw_v, dt_v, k0_v, k512_v, skip_v, raw_v, vec_v,
            hot_v, xs_v, h_v, yr_v, yt_v, sem):
    def rows(i):
        return _ds(i * CB, CB)

    def words(i, n):
        return _ds(i * (n // 2), n // 2)

    pars = (are_hbm, aim_hbm, bre_hbm, bim_hbm, cre_hbm, cim_hbm)
    cp_dt = pltpu.make_async_copy(ldt_hbm, ldt_v, sem.at[0])
    cp_head, cp_rest = [
        [pltpu.make_async_copy(p.at[r], par_v.at[j, r], sem.at[k]) for j, p in enumerate(pars)]
        for k, r in ((1, pl.ds(0, 2 * CB)), (4, pl.ds(2 * CB, D - 2 * CB)))]
    cp_x = [pltpu.make_async_copy(s, d, sem.at[2])
            for s, d in ((x_hbm.bitcast(U32), x_v), (dsk_hbm, dsk_v), (wr_hbm, wr_v))]

    def cp_w(i):
        c = _ds(i * WG * FB, WG * FB)
        return [pltpu.make_async_copy(s.bitcast(U32).at[:, c], d.at[:, c], sem.at[5 + i])
                for s, d in ((wg_hbm, wg_v), (wu_hbm, wu_v))]

    def cp_d(i):
        r = words(i, WG * CB)
        return pltpu.make_async_copy(wd_hbm.bitcast(U32).at[r], wd_v.at[r],
                                     sem.at[5 + NCB // WG + i])

    for c in [cp_dt] + cp_head + cp_rest + cp_x:
        c.start()

    def table(t, lo, n):
        return pltpu.bitcast(tab_v[t, :, _tile(lo, n)], BF16)

    raw_v[...] = jnp.zeros(raw_v.shape, F32)
    vec_v[...] = jnp.zeros(vec_v.shape, VT)
    _write_tables(tab_v, edge_v)

    cp_dt.wait()
    dt_row = _rb(jnp.exp(ldt_v[...].astype(F32).reshape(1, D)))
    dt_v[...] = jnp.broadcast_to(dt_row, (128, D)).T
    for c in cp_head:
        c.wait()

    def kernel_powers(i, after):
        par = [par_v[t, rows(i), :].astype(F32) for t in range(6)]
        k0 = []
        for g in range(0, CB, PN):
            pw, w = _ssm_powers([v[g:g + PN] for v in par], after(dt_v[_ds(i * CB + g, PN), :]))
            pw_v[g:g + PN, :] = jnp.concatenate([v for z in pw for v in z], axis=1)
            k0_v[_ds(i * CB + g, PN), :] = jnp.broadcast_to(
                jnp.sum(w, axis=1, keepdims=True), (PN, 128))
            yield

    def kernel_values(pw, clock):
        for g in range(0, CB, 8):
            out = _ssm_products([(pw[g:g + 8, _tile(2 * t)], pw[g:g + 8, _tile(2 * t + 1)])
                                 for t in range(9)])
            for v in range(10):
                raw_v[v, g:g + 8, :] = out[v]
            clock.append(out[0])
            yield

    def kernel_vectors(i, raw):
        sub = jax.lax.broadcasted_iota(I32, (8, 128), 0)
        lane = jax.lax.broadcasted_iota(I32, (8, 128), 1)
        odd = ((lane - sub) & 1) == 1
        own = ((lane - sub) & 2) == ((sub & 4) >> 1)
        perm = (4 * (lane & 31) + ((sub + ((sub & 4) >> 1)) & 3) + (lane >> 5)) & 127
        u = [jnp.where(odd, pltpu.roll(raw[v1, g:g + 8], 1, 1), raw[v0, g:g + 8])
             for v0, v1 in GROUPS for g in range(0, CB, 8)]
        u = [jnp.where(own, v, pltpu.roll(pltpu.roll(v, 4, 0), 2, 1)) for v in u]
        u = [jnp.take_along_axis(v, perm, axis=1) for v in u]
        gc, gd, g4, go, g2 = [u[t:t + CB // 8] for t in range(0, len(u), CB // 8)]
        mid, last = (lane >= 63) & (lane < 127), lane == 127
        g1 = [jnp.where(mid, a, pltpu.roll(b, 63, 1)) for a, b in zip(g4, go)]
        g3 = [jnp.where(lane < 64, b, a) for a, b in zip(g4, go)]
        ge = [jnp.where(last, a, b) for a, b in zip(gc, gd)]
        for t, v in enumerate((g4, g1, g2, g3, gc, ge, gd)):
            vec_v[t] = jnp.concatenate(v, axis=0).astype(VT)
        k512_v[rows(i), :] = jnp.broadcast_to(jnp.sum(
            jnp.concatenate([jnp.where(last, a, 0.0) for a in g4], axis=0),
            axis=1, keepdims=True), (CB, 128))
        yield

    def kernel_spectrum(i, vec, clock):
        for m in (1, 3, 2):
            for t in (0, 4):
                f = _dot(vec[3 + m].astype(BF16), table(1 + m, t, 4))
                kf_v[rows(i), _tile(8 * m + t, 4)] = f
                clock.append(f[0:8, 0:128])
                yield
        for p in range(2):
            a, b = [_dot(vec[t].astype(BF16), table(1, 2 * t, 2)) for t in (p, p + 2)]
            kf_v[rows(i), _tile(4 * p, 2)] = a + b
            kf_v[rows(i), _tile(4 * p + 2, 2)] = a - b
            clock.append(a[0:8, 0:128])
            yield

    _run("", p=kernel_powers(0, lambda v: v))
    for j in range(NCB // WG):
        for c in cp_w(j):
            c.start()
    for j in range(NCB // WG):
        cp_d(j).start()

    @pl.loop(0, NCB)
    def _(i):
        @pl.when(i == 1)
        def _():
            for c in cp_rest:
                c.wait()

        clock, after = _pacer(i)
        _run(K_ORDER, s=kernel_spectrum(jnp.maximum(i - 2, 0), vec_v[...], clock),
             c=kernel_vectors(jnp.maximum(i - 1, 0), raw_v[...]),
             v=kernel_values(pw_v[...], clock),
             p=kernel_powers(jnp.minimum(i + 1, NCB - 1), after))

    for c in cp_x:
        c.wait()
    skip_v[...] = jnp.broadcast_to(dsk_v[...].astype(F32).reshape(1, D), (128, D)).T
    wr = jnp.broadcast_to(wr_v[...].astype(F32).reshape(1, D), (TOPC, D)).astype(BF16)
    eps = float(_round_to_bf16(1e-5))
    mean, score = [], []

    def token_mean():
        for t in range(0, L // 128, LT):
            m = _dot(jnp.ones((8, D), BF16), pltpu.bitcast(x_v[:, _tile(t, LT)], BF16)) * (1.0 / D)
            mean.extend(m[:, _tile(j)] for j in range(LT))
            yield

    def split_phases(i, ms=range(4)):
        r = pl.ds(i * CB // 2, CB // 2)
        for m in ms:
            v = [xn_v[r, _tile(4 * m + q)] for q in range(4)]
            v = _lane_exchange([w if q == 0 else pltpu.roll(w, q, 1) for q, w in enumerate(v)])
            for p in range(4):
                ph_v[r, _tile(4 * m + p)] = v[p]

    def center():
        for t in range(L // 128):
            mb, sq, cen = _rb(mean[t]), [0.0, 0.0], []
            for r in range(0, D // 2, 8):
                d = [v - mb for v in _unpack(x_v[r:r + 8, _tile(t)])]
                sq = [a + v * v for a, v in zip(sq, d)]
                cen.append(_pack(*d))
            var = (jnp.sum(sq[0] + sq[1], axis=0, keepdims=True) * (1.0 / D)
                   - jnp.square(mean[t] - mb))
            yield cen, 0.5 / _rb(jnp.sqrt(_rb(_rb(jnp.maximum(var, 0.0)) + eps)))

    def normalize():
        tiles = center()
        for t in range(0, L // 128, NT_):
            out = jnp.concatenate([
                jnp.concatenate([_pack(*[v * inv for v in _unpack(w)]) for w in cen], axis=0)
                for cen, inv in [next(tiles) for _ in range(NT_)]], axis=1)
            xn_v[:, _tile(t, NT_)] = out
            for i in range(EARLY):
                split_phases(i, [t // 4])
            score.append(_rb(2.0 * _dot(wr, pltpu.bitcast(out, BF16))))
            yield

    _run(L_ORDER, s=kernel_spectrum(NCB - 2, vec_v[...], []), c=kernel_vectors(NCB - 1, raw_v),
         t=kernel_spectrum(NCB - 1, vec_v, []), m=token_mean(), n=normalize())
    score = jnp.concatenate(score, axis=1)

    def forward(i, clock):
        for h in range(0, CB, 32):
            for p in range(2):
                a, b = [_dot(
                    pltpu.bitcast(jnp.concatenate(
                        [ph_v[_ds(i * (CB // 2) + g // 2, 8), _tile(4 * m + t)]
                         for g in (h, h + 16) for m in range(4)], axis=0), BF16),
                    table(0, 2 * t, 2)) for t in (p, p + 2)]
                uf_v[4 * h:4 * h + 128, _tile(4 * p, 2)] = a + b
                uf_v[4 * h:4 * h + 128, _tile(4 * p + 2, 2)] = a - b
                for r in range(0, 128, 16):
                    clock.append(a[r:r + 8, 0:128])
                    yield

    def multiply(i, uf, after):
        def pair(src, r, t):
            return src[r, _tile(t)], src[r, _tile(t + 1)]

        for g in range(0, CB, 8):
            r = _ds(i * CB + g, 8)
            ru = [slice(64 * (g // 16) + 16 * m + g % 16, 64 * (g // 16) + 16 * m + g % 16 + 8)
                  for m in range(4)]
            for s, ops in enumerate(((_cadd, _csub), (_add_i, _sub_i))):
                ks, us = [], []
                for t, op in zip((s, s + 2), ops):
                    k = [op(pair(kf_v, r, 2 * s), pair(kf_v, r, 2 * s + 4))]
                    k += [pair(kf_v, r, 8 * m + 2 * t) for m in (1, 2, 3)]
                    k[1] = [v + k512_v[r, :] * edge_v[g:g + 8, _tile(2 * t + c)]
                            for c, v in enumerate(k[1])]
                    k = [k[0]] + [_sub_i(k[m], k[m - 1]) for m in (1, 2, 3)]
                    ks.append([(c, d - c, c + d) if M3 else (c, d) for c, d in k])
                    u = [op(pair(uf, v, 2 * s), pair(uf, v, 2 * s + 4)) for v in ru]
                    us.append([(a + b, a, b) if M3 else (a, b) for a, b in u])
                for n in range(4):
                    z = []
                    for k, u in zip(ks, us):
                        if not M3:
                            acc = _cmul(k[0], u[n] if z else (after(u[n][0]), u[n][1]))
                            for m in range(1, n + 1):
                                acc = _cadd(acc, _cmul(k[m], u[n - m]))
                            z.append(acc)
                            continue
                        acc = [v * w for v, w in zip(k[0], u[n])]
                        if not z:
                            acc[0] = after(acc[0])
                        for m in range(1, n + 1):
                            acc = [a + v * w for a, v, w in zip(acc, k[m], u[n - m])]
                        z.append((acc[0] - acc[2], acc[0] + acc[1]))
                    for t, v in enumerate(_cadd(*z) + _csub(*z)):
                        z_v[pl.ds(4 * g + 8 * n, 8), _tile(4 * s + t)] = v
                    yield

    def inverse(i, z, clock, n=32):
        for h in range(0, CB, n):
            for p, ops in enumerate(((_cadd, _csub), (_sub_i, _add_i))):
                a, c = [[z[4 * h:4 * h + 4 * n, _tile(4 * s + 2 * p + t)] for t in range(2)]
                        for s in range(2)]
                y = [_dot_nt(jnp.concatenate(op(a, c), axis=1).astype(BF16),
                             table(0, 2 * p + 4 * t, 2)) for t, op in enumerate(ops)]
                for g in range(0, n, 8):
                    for m in range(4):
                        for t in range(2):
                            y_v[_ds(i * CB + h + g, 8), _tile(4 * m + p + 2 * t)] = (
                                y[t][4 * g + 8 * m:4 * g + 8 * m + 8])
                for r in range(0, 4 * n, 16):
                    clock.append(y[0][r:r + 8])
                    yield

    bits = pltpu.bitcast(jnp.where(score == 0.0, 0.0, score), I32) >> 16
    pos = jax.lax.broadcasted_iota(I32, (TOPC, L), 1)
    key = ((bits ^ ((bits >> 15) & 0x7FFF)) << 11) + (0x38000000 + L - 1 - pos)
    key = pltpu.bitcast(key, F32)
    sub = jax.lax.broadcasted_iota(I32, (TOPC, 128), 0)
    dense = []
    for t0 in (0, 8):
        v = key[:, _tile(t0)]
        for t in range(1, 8):
            v = jnp.where(sub == t, key[:, _tile(t0 + t)], v)
        dense.append(v)
    _run("", f=forward(0, []))
    top = _merge_top(*[_sort_rows(v, (2, 4, 8)) for v in dense])
    for step, count in ((8, 16), (1, 8)):
        top = [top] + [pltpu.roll(top, step * k, 1) for k in range(1, count)]
        while len(top) > 1:
            top = [_merge_top(a, b) for a, b in zip(top[0::2], top[1::2])]
        top = top[0]
        for i in range(*{8: (EARLY, MID), 1: (MID, NCB)}[step]):
            split_phases(i)
    hot_v[...] = jnp.where(key == jnp.tile(top, (1, L // 128)), 1.0, 0.0)
    top = pltpu.bitcast(top, I32) - 0x38000000
    tb = top >> 11
    gate = _rb(jax.nn.sigmoid(pltpu.bitcast((tb ^ ((tb >> 15) & 0x7FFF)) << 16, F32)))
    tok = (L - 1) - (top & (L - 1))
    pick = (tok & 127) == jax.lax.broadcasted_iota(I32, (TOPC, 128), 1)
    xs_v[...] = xs = _dot_nt(
        jnp.concatenate([jnp.where(pick & (sub == c), 2.0, 0.0) for c in range(TOPC)],
                        axis=1).astype(BF16),
        pltpu.bitcast(jnp.concatenate(
            [xn_v[:, _ds(tok[c, 0] & (L - 128), 128)] for c in range(TOPC)], axis=1), BF16))

    z_v[...] = jnp.tile(xs[:, 0:128], (4 * CB // TOPC, 8))

    def ffn_up(i):
        acc = [0.0, 0.0]
        for j in range(0, D, 128):
            n = min(128, D - j)
            for t, w in enumerate((wg_v, wu_v)):
                acc[t] = acc[t] + _dot(
                    xs_v[:, j:j + n].astype(BF16),
                    pltpu.bitcast(w[j // 2:(j + n) // 2, _ds(i * FB, FB)], BF16))
                yield
        h_v[:, _ds(i * FB, FB)] = _rb(_silu(_rb(acc[0]))) * _rb(acc[1])

    @pl.loop(0, NCB)
    def _(i):
        for j in range(NCB // WG):
            @pl.when(i == j * WG)
            def _():
                for c in cp_w(j):
                    c.wait()

        clock, after = _pacer(i)
        _run(C_ORDER.replace('I', 'im' * 8).replace('F', 'fm' * 8).replace('J', 'imimimim' * 2 + 'm').replace('G', 'fmfmmfmfmm' * 2).replace('E', 'fmfmmfmm' * 2 + 'fmfm').replace('H', 'f' * 8), i=inverse(jnp.maximum(i - 1, 0), z_v[...], clock),
             m=multiply(i, uf_v[...], after), u=ffn_up(i),
             f=forward(jnp.minimum(i + 1, NCB - 1), clock))

    def ffn_down(i):
        y = 0.0
        for j in range(0, F, FB):
            y = y + _dot_nt(h_v[:, j:j + FB].astype(BF16),
                            pltpu.bitcast(wd_v[words(i, DB), j:j + FB], BF16))
            if j + FB == F:
                yr_v[...] = 0.5 * _rb(_rb(y) * gate[:, :DB])
            yield

    def finish(i, yt):
        for g in range(0, DB, 32):
            r, rw = _ds(i * DB + g, 32), _ds(i * (DB // 2) + g // 2, 16)
            skip = 2.0 * skip_v[r, :] + BLK * k0_v[r, :]
            for m in range(4):
                upd = _dot(yt[g:g + 32].astype(BF16), hot_v[:, _tile(4 * m, 4)].astype(BF16))
                y = _lane_exchange([y_v[r, _tile(4 * m + p)] for p in range(4)])
                y = [v if q == 0 else pltpu.roll(v, 128 - q, 1) for q, v in enumerate(y)]
                for q in (0, 2):
                    out = []
                    for t in (q, q + 1):
                        x, xn = [pltpu.bitcast(w[rw, _tile(4 * m + t)], BF16).astype(F32)
                                 for w in (x_v, xn_v)]
                        h = xn + upd[:, _tile(t)]
                        out.append(x + (y[t] + xn * skip) * (h + h * jnp.tanh(h)))
                    o_v[r, _tile(4 * m + q, 2)] = jnp.concatenate(out, axis=1).astype(BF16)
                yield

    cp_d(0).wait()
    def first_down():
        yield from ffn_down(0)
        yt_v[...] = yr_v[...].T
        yield from ffn_down(1)

    def send(row, n):
        r = _ds(row, n)
        pltpu.make_async_copy(o_v.at[r], o_hbm.at[r], sem.at[3]).start()

    _run("", d=first_down())

    @pl.loop(0, NCB - 2)
    def _(i):
        for j in range(1, NCB // WG):
            @pl.when(i + 2 == j * WG)
            def _():
                cp_d(j).wait()

        yt = yt_v[...]
        yt_v[...] = yr_v[...].T
        _run(D_ORDER, o=finish(i, yt), d=ffn_down(i + 2))
        send(i * CB, CB)

    _run(P_ORDER.replace("I", "i" * (PI // 4)), o=finish(NCB - 2, yt_v[...]),
         i=inverse(NCB - 1, z_v, [], PI))
    send(D - 2 * CB, CB)
    last = finish(NCB - 1, yr_v[...].T)
    for row in (D - CB, D - CB // 2):
        for _ in range(4):
            next(last)
        send(row, CB // 2)
    pltpu.make_async_copy(o_v, o_hbm, sem.at[3]).wait()


@jax.jit
def pallas_recurrent_scan__ssm_conv_s4__moe_arch_mod__prompt_kernel(
    A_u: jax.Array,
    A_A_re: jax.Array,
    A_A_im: jax.Array,
    A_B_re: jax.Array,
    A_B_im: jax.Array,
    A_C_re: jax.Array,
    A_C_im: jax.Array,
    A_log_dt: jax.Array,
    A_Dskip: jax.Array,
    B_x: jax.Array,
    B_w_r: jax.Array,
    B_w_gate: jax.Array,
    B_w_up: jax.Array,
    B_w_down: jax.Array,
):
    del B_x
    assert A_u.shape == (1, L, D) and A_A_re.shape == (D, N) and B_w_gate.shape == (D, F)
    hbm = pl.BlockSpec(memory_space=pl.ANY)
    vmem = pltpu.VMEM
    out = pl.pallas_call(
        _kernel,
        out_shape=jax.ShapeDtypeStruct((D, L), BF16),
        in_specs=[hbm] * 13,
        out_specs=hbm,
        scratch_shapes=[
            vmem((D // 2, L), U32), vmem((6, D, N), BF16),
            vmem((D,), BF16), vmem((D,), BF16), vmem((D,), BF16),
            vmem((D // 2, F), U32), vmem((D // 2, F), U32), vmem((D // 2, F), U32),
            vmem((5, 64, 1024), U32), vmem((CB, 1024), F32), vmem((D, L), BF16),
            vmem((D // 2, L), U32), vmem((D // 2, L), U32),
            vmem((D, 4096), F32), vmem((4 * CB, 1024), F32), vmem((4 * CB, 1024), F32),
            vmem((D, L), F32), vmem((CB, 18 * 128), F32),
            *[vmem((D, 128), F32)] * 4,
            vmem((10, CB, 128), F32), vmem((7, CB, 128), VT),
            vmem((TOPC, L), F32), vmem((TOPC, D), F32), vmem((TOPC, F), F32),
            vmem((TOPC, DB), F32), vmem((DB, TOPC), F32),
            pltpu.SemaphoreType.DMA((5 + 2 * (NCB // WG),)),
        ],
        compiler_params=pltpu.CompilerParams(vmem_limit_bytes=100 * 1024 * 1024),
    )(A_u[0].T, A_A_re, A_A_im, A_B_re, A_B_im, A_C_re, A_C_im, A_log_dt, A_Dskip, B_w_r,
      B_w_gate, B_w_up, B_w_down.T)
    return out.T[None]
```

```python
import jax
import jax.numpy as jnp
import numpy as np
import jax.experimental.pallas as pl
import jax.experimental.pallas.tpu as pltpu

F32, BF16, I32, U32 = jnp.float32, jnp.bfloat16, jnp.int32, jnp.uint32

L, D, N, F = 2048, 576, 128, 4608
TOPC = 8
BLK = 512
CB = 64
NCB = D // CB
FB = F // NCB
DB = 64
NT = (((1,), (1,)), ((), ()))
Q_PAIRS = ((3, 1), (7, 5), (2, 258), (4, 260), (6, 262), (8, 264),
           (516, 772), (520, 776), (1032, 1288), (1544, 1800))
GROUPS = ((6, 7), (8, 9), (3, 5), (0, 1), (2, 4))
K_ORDER = "cssvspvpvsspvppvvpssvpspv"
C_ORDER = "mimimiimiimmimimuimimimiimimimimimumimiimimimmimimuimimimimimimimmimufmfmmffmmmfmmfmfmfmuufmfmfmfmmfmmfmmfmfmufmfmfmffmffmmfmfmuuuffffffmf"
D_ORDER = "ododododododododd"
L_ORDER = "cmssmnsssmsstsntmnttntttt"
LT = 4
NT_ = 4
EARLY = 4
MID = 5
PN = 8
PI = 32
P_ORDER = "oo I oo I oo I o I o"
M3 = True
VT = 'float32'
WG = 3
LAST = 48
HOLD = 2


def _round_to_bf16(v):
    u = np.asarray(v, np.float32).view(np.uint32)
    return ((u + 0x7FFF + ((u >> 16) & 1)) & 0xFFFF0000).astype(np.uint32).view(np.float32)


def _cmul(a, b):
    return a[0] * b[0] - a[1] * b[1], a[0] * b[1] + a[1] * b[0]


def _csq(a):
    return (a[0] + a[1]) * (a[0] - a[1]), (a[0] + a[0]) * a[1]


def _cadd(a, b):
    return a[0] + b[0], a[1] + b[1]


def _csub(a, b):
    return a[0] - b[0], a[1] - b[1]


def _add_i(a, b):
    return a[0] - b[1], a[1] + b[0]


def _sub_i(a, b):
    return a[0] + b[1], a[1] - b[0]


def _lane_exchange(r):
    lane = jax.lax.broadcasted_iota(I32, r[0].shape, 1)
    a = [jnp.where((lane & 1) == 1, r[(j + 1) % 4], r[j]) for j in range(4)]
    b = [jnp.where((lane & 2) == 2, a[(j + 2) % 4], a[j]) for j in range(4)]
    return [b[-j % 4] for j in range(4)]


def _rb(v):
    return v.astype(BF16).astype(F32)


def _silu(v):
    h = 0.5 * v
    return h + h * jnp.tanh(h)


def _pack(even, odd):
    return pltpu.pack_elementwise([even, odd], packed_dtype=BF16)


def _unpack(w):
    return [pltpu.unpack_elementwise(w, index=j, packed_dtype=BF16, unpacked_dtype=F32)
            for j in range(2)]


def _tile(t, n=1):
    return slice(128 * t, 128 * (t + n))


def _ds(start, size, align=None):
    if isinstance(start, int):
        return pl.ds(start, size)
    return pl.ds(pl.multiple_of(start, align or size), size)


def _dot(a, b):
    return jnp.dot(a, b, preferred_element_type=F32)


def _dot_nt(a, b):
    return jax.lax.dot_general(a, b, NT, preferred_element_type=F32)


def _run(order, **stages):
    for step in order.replace(" ", ""):
        next(stages[step])
    for stage in stages.values():
        for _ in stage:
            pass


def _pacer(step):
    clock = []

    def after(v):
        if not clock:
            return v
        always = jax.lax.broadcasted_iota(I32, v.shape, 1) < step + 128
        return jnp.where(always, v, jnp.tile(clock[-1], (v.shape[0] // 8, 1)))

    return clock, after


def _sort_rows(v, sizes):
    sub = jax.lax.broadcasted_iota(I32, v.shape, 0)
    for k in sizes:
        j = k // 2
        while j:
            w = jnp.take_along_axis(v, sub ^ j, axis=0)
            v = jnp.where(((sub & j) == 0) == ((sub & k) == 0),
                          jnp.maximum(v, w), jnp.minimum(v, w))
            j //= 2
    return v


def _merge_top(a, b):
    sub = jax.lax.broadcasted_iota(I32, a.shape, 0)
    return _sort_rows(jnp.maximum(a, jnp.take_along_axis(b, 7 - sub, axis=0)), (8,))


def _write_tables(tab_v, edge_v):
    sub = jax.lax.broadcasted_iota(I32, (8, 128), 0)
    lane = jax.lax.broadcasted_iota(I32, (8, 128), 1)
    ang = (((4 * lane + 1) << sub) & (4 * BLK - 1)).astype(F32) * (np.pi / (2 * BLK))
    bits = jnp.cos(ang), jnp.sin(ang)
    known = {1 << s: [jnp.broadcast_to(v[s:s + 1], (8, 128)) for v in bits] for s in range(8)}
    known[0] = [jnp.ones((8, 128), F32), jnp.zeros((8, 128), F32)]

    def times_i(z, n):
        for _ in range(n % 4):
            z = (-z[1], z[0])
        return z

    def power(t):
        if t >= BLK:
            return times_i(power(t - BLK), 1)
        if t not in known:
            low = t & -t if t & (t - 1) else t // 2
            known[t] = _cmul(power(t - low), power(low))
        return known[t]

    def put(cond, z, base):
        return [jnp.where(cond, v, w) for v, w in zip(z, base)]

    def lag_sum(ts, s):
        terms = [times_i(power(t), s * t) for t in ts]
        return [sum(z[c] for z in terms) for c in range(2)]

    def ramp(step):
        z = put((sub & 1) == 1, power(step), known[0])
        for b in (2, 4):
            z = _cmul(z, put((sub & b) == b, power(b * step), known[0]))
        return z

    def store(t, j, col, even, odd):
        for c in range(2):
            tab_v[t, 8 * j:8 * j + 8, _tile(col + c)] = _pack(even[c], odd[c])

    ramp2, ramp16 = ramp(2), ramp(16)
    for p in range(4):
        col = []
        for e in range(2):
            q0, q1 = (e - p) % 4, (e + 2 - p) % 4
            z = [_cmul(ramp2, put((sub & 1) == 1, power(127 * q1 + e), power(127 * q0 + e)))]
            for _ in range(8):
                z.append(_cmul(z[-1], power(16)))
            z[0] = put(2 * sub + e < ((2 * sub + e - p) & 3), z[8], z[0])
            col.append(z)
        for j in range(8):
            store(0, j, 2 * p, col[0][j], col[1][j])

    lag_exp = _round_to_bf16(np.arange(L)).astype(np.int64)
    c = np.arange(128)
    gc, gd, g4, go, g2 = [
        np.concatenate([Q_PAIRS[v][e] + 8 * np.arange(32) for e in range(2) for v in vs])
        for vs in GROUPS]
    g1 = np.where((c >= 63) & (c < 127), g4, np.roll(go, 63))
    g3, ge = np.where(c < 64, go, g4), np.where(c == 127, gc, gd)
    rows16 = {}

    def ramp_from(t):
        if t not in rows16:
            back = [d for d in (8, 128) if t - d in rows16]
            rows16[t] = (_cmul(rows16[t - back[0]], power(back[0])) if back
                         else _cmul(ramp16, power(t)))
        return rows16[t]

    def lags(e, m, phase=None):
        ts = [int(l) - BLK * m for l in np.nonzero(lag_exp == e)[0] if 0 < l - BLK * m <= BLK]
        return [t for t in ts if phase is None or t % 4 == phase]

    def rows(tss, s):
        z = [known[0][1]] * 2
        if tss[0]:
            half = len(tss[0]) // 2
            z = ramp_from(tss[0][half])
            if half:
                assert tss[0][half] % 4 == 0 and len(tss[0]) % 2 == 1
                box = 1.0 + 2.0 * lag_sum(range(1, half + 1), s)[0]
                z = [v * box for v in z]
        for r, ts in enumerate(tss):
            if ts != [t + 16 * r for t in tss[0]]:
                z = put(sub == r, lag_sum(ts, s), z)
        return z

    for j in range(8):
        for p, g in enumerate((g4, g1, g2, g3)):
            store(1, j, 2 * p, *[rows([lags(v, 0, p) for v in g[16 * j + e:16 * j + 16:2]], 0)
                                 for e in range(2)])
        for m, g in ((1, gc), (2, ge), (3, gd)):
            for s in range(4):
                store(1 + m, j, 2 * s, *[rows([lags(v, m) for v in g[16 * j + e:16 * j + 16:2]], s)
                                         for e in range(2)])
    for s in range(4):
        edge_v[:, _tile(2 * s, 2)] = jnp.tile(
            jnp.concatenate(lag_sum(lags(BLK, 1), s), axis=1), (CB // 8, 1))


def _ssm_powers(par, dt):
    a_re, a_im, b_re, b_im, c_re, c_im = par
    mag = jnp.exp(dt * a_re)
    ang = dt * a_im
    pw = {1: (mag * jnp.cos(ang), mag * jnp.sin(ang))}
    for k in range(9):
        pw[2 << k] = _csq(pw[1 << k])
    sc = dt * (2.0 / BLK)
    w = _cmul((c_re, c_im), (b_re * sc, b_im * sc))
    w1, w2 = _cmul(w, pw[1]), _cmul(w, pw[2])
    return [pw[8], pw[16], pw[2], pw[4], pw[512],
            w1, _cmul(w1, pw[2]), w2, _cmul(w2, pw[256])], w[0]


def _ssm_products(pw):
    a8, a16, a2, a4, a512, w1, w3, w2, w258 = pw
    sub = jax.lax.broadcasted_iota(I32, (8, 128), 0)
    lane = jax.lax.broadcasted_iota(I32, (8, 128), 1)
    lo = sub < 4

    def pick(z, rows):
        return [jnp.take_along_axis(v, rows, axis=0) for v in z]

    def pair(x, y, h):
        r = [pltpu.roll(v, 4, 0) for v in y]
        return [jnp.where(lo, s, v) if h else jnp.where(lo, v, s) for v, s in zip(x, r)]

    out = []
    for h in range(2):
        p_rows, q_rows = 4 * h + ((sub + 2 * h) & 3), 4 * h + (sub & 3)
        step, s2, s512 = pick(a16, p_rows), pick(a2, q_rows), pick(a512, q_rows)
        p = [[jnp.where(lo, one, v) for one, v in zip((1.0, 0.0), pick(a8, p_rows))]]
        for _ in range(15):
            p.append(_cmul(p[-1], step))
        q = [pair(w3, w1, h)]
        q += [_cmul(q[0], pick(a4, q_rows)), pair(w2, w258, h)]
        for _ in range(3):
            q.append(_cmul(q[-1], s2))
        q += [_cmul(q[3], s512), _cmul(q[5], s512)]
        for _ in range(2):
            q.append(_cmul(q[-1], s512))
        out.append([_dot_nt(*[jnp.concatenate([z[j] for z in zs], axis=0).astype(BF16)
                              for zs in (q, p)]) for j in range(2)])
    first = ((lane - sub) & 3) == 0
    return [jnp.where(first, out[0][0][v:v + 8], out[1][0][v:v + 8])
            - jnp.where(first, out[0][1][v:v + 8], out[1][1][v:v + 8]) for v in range(0, 80, 8)]


def _kernel(x_hbm, are_hbm, aim_hbm, bre_hbm, bim_hbm, cre_hbm, cim_hbm, ldt_hbm, dsk_hbm, wr_hbm,
            wg_hbm, wu_hbm, wd_hbm, o_hbm,
            x_v, par_v, ldt_v, dsk_v, wr_v, wg_v, wu_v, wd_v, tab_v, edge_v, o_v,
            xn_v, ph_v, kf_v, uf_v, z_v, y_v, pw_v, dt_v, k0_v, k512_v, skip_v, raw_v, vec_v,
            hot_v, xs_v, h_v, yr_v, yt_v, sem):
    def rows(i):
        return _ds(i * CB, CB)

    def words(i, n):
        return _ds(i * (n // 2), n // 2)

    pars = (are_hbm, aim_hbm, bre_hbm, bim_hbm, cre_hbm, cim_hbm)
    cp_dt = pltpu.make_async_copy(ldt_hbm, ldt_v, sem.at[0])
    cp_head, cp_rest = [
        [pltpu.make_async_copy(p.at[r], par_v.at[j, r], sem.at[k]) for j, p in enumerate(pars)]
        for k, r in ((1, pl.ds(0, 2 * CB)), (4, pl.ds(2 * CB, D - 2 * CB)))]
    cp_x = [pltpu.make_async_copy(s, d, sem.at[2])
            for s, d in ((x_hbm.bitcast(U32), x_v), (dsk_hbm, dsk_v), (wr_hbm, wr_v))]

    def cp_w(i):
        c = _ds(i * WG * FB, WG * FB)
        return [pltpu.make_async_copy(s.bitcast(U32).at[:, c], d.at[:, c], sem.at[5 + i])
                for s, d in ((wg_hbm, wg_v), (wu_hbm, wu_v))]

    def cp_d(i):
        cuts = (0, (HOLD + 2) * CB, D - LAST, D)
        r = pl.ds(cuts[i] // 2, (cuts[i + 1] - cuts[i]) // 2)
        return pltpu.make_async_copy(wd_hbm.bitcast(U32).at[r], wd_v.at[r],
                                     sem.at[5 + NCB // WG + i])

    for c in [cp_dt] + cp_head + cp_rest + cp_x:
        c.start()

    def table(t, lo, n):
        return pltpu.bitcast(tab_v[t, :, _tile(lo, n)], BF16)

    raw_v[...] = jnp.zeros(raw_v.shape, F32)
    vec_v[...] = jnp.zeros(vec_v.shape, VT)
    _write_tables(tab_v, edge_v)

    cp_dt.wait()
    dt_row = _rb(jnp.exp(ldt_v[...].astype(F32).reshape(1, D)))
    dt_v[...] = jnp.broadcast_to(dt_row, (128, D)).T
    for c in cp_head:
        c.wait()

    def kernel_powers(i, after):
        par = [par_v[t, rows(i), :].astype(F32) for t in range(6)]
        k0 = []
        for g in range(0, CB, PN):
            pw, w = _ssm_powers([v[g:g + PN] for v in par], after(dt_v[_ds(i * CB + g, PN), :]))
            pw_v[g:g + PN, :] = jnp.concatenate([v for z in pw for v in z], axis=1)
            k0_v[_ds(i * CB + g, PN), :] = jnp.broadcast_to(
                jnp.sum(w, axis=1, keepdims=True), (PN, 128))
            yield

    def kernel_values(pw, clock):
        for g in range(0, CB, 8):
            out = _ssm_products([(pw[g:g + 8, _tile(2 * t)], pw[g:g + 8, _tile(2 * t + 1)])
                                 for t in range(9)])
            for v in range(10):
                raw_v[v, g:g + 8, :] = out[v]
            clock.append(out[0])
            yield

    def kernel_vectors(i, raw):
        sub = jax.lax.broadcasted_iota(I32, (8, 128), 0)
        lane = jax.lax.broadcasted_iota(I32, (8, 128), 1)
        odd = ((lane - sub) & 1) == 1
        own = ((lane - sub) & 2) == ((sub & 4) >> 1)
        perm = (4 * (lane & 31) + ((sub + ((sub & 4) >> 1)) & 3) + (lane >> 5)) & 127
        u = [jnp.where(odd, pltpu.roll(raw[v1, g:g + 8], 1, 1), raw[v0, g:g + 8])
             for v0, v1 in GROUPS for g in range(0, CB, 8)]
        u = [jnp.where(own, v, pltpu.roll(pltpu.roll(v, 4, 0), 2, 1)) for v in u]
        u = [jnp.take_along_axis(v, perm, axis=1) for v in u]
        gc, gd, g4, go, g2 = [u[t:t + CB // 8] for t in range(0, len(u), CB // 8)]
        mid, last = (lane >= 63) & (lane < 127), lane == 127
        g1 = [jnp.where(mid, a, pltpu.roll(b, 63, 1)) for a, b in zip(g4, go)]
        g3 = [jnp.where(lane < 64, b, a) for a, b in zip(g4, go)]
        ge = [jnp.where(last, a, b) for a, b in zip(gc, gd)]
        for t, v in enumerate((g4, g1, g2, g3, gc, ge, gd)):
            vec_v[t] = jnp.concatenate(v, axis=0).astype(VT)
        k512_v[rows(i), :] = jnp.broadcast_to(jnp.sum(
            jnp.concatenate([jnp.where(last, a, 0.0) for a in g4], axis=0),
            axis=1, keepdims=True), (CB, 128))
        yield

    def kernel_spectrum(i, vec, clock):
        for m in (1, 3, 2):
            for t in (0, 4):
                f = _dot(vec[3 + m].astype(BF16), table(1 + m, t, 4))
                kf_v[rows(i), _tile(8 * m + t, 4)] = f
                clock.append(f[0:8, 0:128])
                yield
        for p in range(2):
            a, b = [_dot(vec[t].astype(BF16), table(1, 2 * t, 2)) for t in (p, p + 2)]
            kf_v[rows(i), _tile(4 * p, 2)] = a + b
            kf_v[rows(i), _tile(4 * p + 2, 2)] = a - b
            clock.append(a[0:8, 0:128])
            yield

    _run("", p=kernel_powers(0, lambda v: v))
    for j in range(NCB // WG):
        for c in cp_w(j):
            c.start()
    for j in range(3):
        cp_d(j).start()

    @pl.loop(0, NCB)
    def _(i):
        @pl.when(i == 1)
        def _():
            for c in cp_rest:
                c.wait()

        clock, after = _pacer(i)
        _run(K_ORDER, s=kernel_spectrum(jnp.maximum(i - 2, 0), vec_v[...], clock),
             c=kernel_vectors(jnp.maximum(i - 1, 0), raw_v[...]),
             v=kernel_values(pw_v[...], clock),
             p=kernel_powers(jnp.minimum(i + 1, NCB - 1), after))

    for c in cp_x:
        c.wait()
    skip_v[...] = jnp.broadcast_to(dsk_v[...].astype(F32).reshape(1, D), (128, D)).T
    wr = jnp.broadcast_to(wr_v[...].astype(F32).reshape(1, D), (TOPC, D)).astype(BF16)
    eps = float(_round_to_bf16(1e-5))
    mean, score = [], []

    def token_mean():
        for t in range(0, L // 128, LT):
            m = _dot(jnp.ones((8, D), BF16), pltpu.bitcast(x_v[:, _tile(t, LT)], BF16)) * (1.0 / D)
            mean.extend(m[:, _tile(j)] for j in range(LT))
            yield

    def split_phases(i, ms=range(4)):
        r = pl.ds(i * CB // 2, CB // 2)
        for m in ms:
            v = [xn_v[r, _tile(4 * m + q)] for q in range(4)]
            v = _lane_exchange([w if q == 0 else pltpu.roll(w, q, 1) for q, w in enumerate(v)])
            for p in range(4):
                ph_v[r, _tile(4 * m + p)] = v[p]

    def center():
        for t in range(L // 128):
            mb, sq, cen = _rb(mean[t]), [0.0, 0.0], []
            for r in range(0, D // 2, 8):
                d = [v - mb for v in _unpack(x_v[r:r + 8, _tile(t)])]
                sq = [a + v * v for a, v in zip(sq, d)]
                cen.append(_pack(*d))
            var = (jnp.sum(sq[0] + sq[1], axis=0, keepdims=True) * (1.0 / D)
                   - jnp.square(mean[t] - mb))
            yield cen, 0.5 / _rb(jnp.sqrt(_rb(_rb(jnp.maximum(var, 0.0)) + eps)))

    def normalize():
        tiles = center()
        for t in range(0, L // 128, NT_):
            out = jnp.concatenate([
                jnp.concatenate([_pack(*[v * inv for v in _unpack(w)]) for w in cen], axis=0)
                for cen, inv in [next(tiles) for _ in range(NT_)]], axis=1)
            xn_v[:, _tile(t, NT_)] = out
            for i in range(EARLY):
                split_phases(i, [t // 4])
            score.append(_rb(2.0 * _dot(wr, pltpu.bitcast(out, BF16))))
            yield

    _run(L_ORDER, s=kernel_spectrum(NCB - 2, vec_v[...], []), c=kernel_vectors(NCB - 1, raw_v),
         t=kernel_spectrum(NCB - 1, vec_v, []), m=token_mean(), n=normalize())
    score = jnp.concatenate(score, axis=1)

    def forward(i, clock):
        for h in range(0, CB, 32):
            for p in range(2):
                a, b = [_dot(
                    pltpu.bitcast(jnp.concatenate(
                        [ph_v[_ds(i * (CB // 2) + g // 2, 8), _tile(4 * m + t)]
                         for g in (h, h + 16) for m in range(4)], axis=0), BF16),
                    table(0, 2 * t, 2)) for t in (p, p + 2)]
                uf_v[4 * h:4 * h + 128, _tile(4 * p, 2)] = a + b
                uf_v[4 * h:4 * h + 128, _tile(4 * p + 2, 2)] = a - b
                for r in range(0, 128, 16):
                    clock.append(a[r:r + 8, 0:128])
                    yield

    def multiply(i, uf, after):
        def pair(src, r, t):
            return src[r, _tile(t)], src[r, _tile(t + 1)]

        for g in range(0, CB, 8):
            r = _ds(i * CB + g, 8)
            ru = [slice(64 * (g // 16) + 16 * m + g % 16, 64 * (g // 16) + 16 * m + g % 16 + 8)
                  for m in range(4)]
            for s, ops in enumerate(((_cadd, _csub), (_add_i, _sub_i))):
                ks, us = [], []
                for t, op in zip((s, s + 2), ops):
                    k = [op(pair(kf_v, r, 2 * s), pair(kf_v, r, 2 * s + 4))]
                    k += [pair(kf_v, r, 8 * m + 2 * t) for m in (1, 2, 3)]
                    k[1] = [v + k512_v[r, :] * edge_v[g:g + 8, _tile(2 * t + c)]
                            for c, v in enumerate(k[1])]
                    k = [k[0]] + [_sub_i(k[m], k[m - 1]) for m in (1, 2, 3)]
                    ks.append([(c, d - c, c + d) if M3 else (c, d) for c, d in k])
                    u = [op(pair(uf, v, 2 * s), pair(uf, v, 2 * s + 4)) for v in ru]
                    us.append([(a + b, a, b) if M3 else (a, b) for a, b in u])
                for n in range(4):
                    z = []
                    for k, u in zip(ks, us):
                        if not M3:
                            acc = _cmul(k[0], u[n] if z else (after(u[n][0]), u[n][1]))
                            for m in range(1, n + 1):
                                acc = _cadd(acc, _cmul(k[m], u[n - m]))
                            z.append(acc)
                            continue
                        acc = [v * w for v, w in zip(k[0], u[n])]
                        if not z:
                            acc[0] = after(acc[0])
                        for m in range(1, n + 1):
                            acc = [a + v * w for a, v, w in zip(acc, k[m], u[n - m])]
                        z.append((acc[0] - acc[2], acc[0] + acc[1]))
                    for t, v in enumerate(_cadd(*z) + _csub(*z)):
                        z_v[pl.ds(4 * g + 8 * n, 8), _tile(4 * s + t)] = v
                    yield

    def inverse(i, z, clock, n=32):
        for h in range(0, CB, n):
            for p, ops in enumerate(((_cadd, _csub), (_sub_i, _add_i))):
                a, c = [[z[4 * h:4 * h + 4 * n, _tile(4 * s + 2 * p + t)] for t in range(2)]
                        for s in range(2)]
                y = [_dot_nt(jnp.concatenate(op(a, c), axis=1).astype(BF16),
                             table(0, 2 * p + 4 * t, 2)) for t, op in enumerate(ops)]
                for g in range(0, n, 8):
                    for m in range(4):
                        for t in range(2):
                            y_v[_ds(i * CB + h + g, 8), _tile(4 * m + p + 2 * t)] = (
                                y[t][4 * g + 8 * m:4 * g + 8 * m + 8])
                for r in range(0, 4 * n, 16):
                    clock.append(y[0][r:r + 8])
                    yield

    bits = pltpu.bitcast(jnp.where(score == 0.0, 0.0, score), I32) >> 16
    pos = jax.lax.broadcasted_iota(I32, (TOPC, L), 1)
    key = ((bits ^ ((bits >> 15) & 0x7FFF)) << 11) + (0x38000000 + L - 1 - pos)
    key = pltpu.bitcast(key, F32)
    sub = jax.lax.broadcasted_iota(I32, (TOPC, 128), 0)
    dense = []
    for t0 in (0, 8):
        v = key[:, _tile(t0)]
        for t in range(1, 8):
            v = jnp.where(sub == t, key[:, _tile(t0 + t)], v)
        dense.append(v)
    _run("", f=forward(0, []))
    top = _merge_top(*[_sort_rows(v, (2, 4, 8)) for v in dense])
    for step, count in ((8, 16), (1, 8)):
        top = [top] + [pltpu.roll(top, step * k, 1) for k in range(1, count)]
        while len(top) > 1:
            top = [_merge_top(a, b) for a, b in zip(top[0::2], top[1::2])]
        top = top[0]
        for i in range(*{8: (EARLY, MID), 1: (MID, NCB)}[step]):
            split_phases(i)
    hot_v[...] = jnp.where(key == jnp.tile(top, (1, L // 128)), 1.0, 0.0)
    top = pltpu.bitcast(top, I32) - 0x38000000
    tb = top >> 11
    gate = _rb(jax.nn.sigmoid(pltpu.bitcast((tb ^ ((tb >> 15) & 0x7FFF)) << 16, F32)))
    tok = (L - 1) - (top & (L - 1))
    pick = (tok & 127) == jax.lax.broadcasted_iota(I32, (TOPC, 128), 1)
    xs_v[...] = xs = _dot_nt(
        jnp.concatenate([jnp.where(pick & (sub == c), 2.0, 0.0) for c in range(TOPC)],
                        axis=1).astype(BF16),
        pltpu.bitcast(jnp.concatenate(
            [xn_v[:, _ds(tok[c, 0] & (L - 128), 128)] for c in range(TOPC)], axis=1), BF16))

    z_v[...] = jnp.tile(xs[:, 0:128], (4 * CB // TOPC, 8))

    def ffn_up(i):
        acc = [0.0, 0.0]
        for j in range(0, D, 128):
            n = min(128, D - j)
            for t, w in enumerate((wg_v, wu_v)):
                acc[t] = acc[t] + _dot(
                    xs_v[:, j:j + n].astype(BF16),
                    pltpu.bitcast(w[j // 2:(j + n) // 2, _ds(i * FB, FB)], BF16))
                yield
        h_v[:, _ds(i * FB, FB)] = _rb(_silu(_rb(acc[0]))) * _rb(acc[1])

    @pl.loop(0, NCB)
    def _(i):
        for j in range(NCB // WG):
            @pl.when(i == j * WG)
            def _():
                for c in cp_w(j):
                    c.wait()

        clock, after = _pacer(i)
        _run(C_ORDER.replace('I', 'im' * 8).replace('F', 'fm' * 8).replace('J', 'imimimim' * 2 + 'm').replace('G', 'fmfmmfmfmm' * 2).replace('E', 'fmfmmfmm' * 2 + 'fmfm').replace('H', 'f' * 8), i=inverse(jnp.maximum(i - 1, 0), z_v[...], clock),
             m=multiply(i, uf_v[...], after), u=ffn_up(i),
             f=forward(jnp.minimum(i + 1, NCB - 1), clock))

    def ffn_down(i):
        y = 0.0
        for j in range(0, F, FB):
            y = y + _dot_nt(h_v[:, j:j + FB].astype(BF16),
                            pltpu.bitcast(wd_v[words(i, DB), j:j + FB], BF16))
            if j + FB == F:
                yr_v[...] = 0.5 * _rb(_rb(y) * gate[:, :DB])
            yield

    def finish(i, yt):
        for g in range(0, DB, 32):
            r, rw = _ds(i * DB + g, 32), _ds(i * (DB // 2) + g // 2, 16)
            skip = 2.0 * skip_v[r, :] + BLK * k0_v[r, :]
            for m in range(4):
                upd = _dot(yt[g:g + 32].astype(BF16), hot_v[:, _tile(4 * m, 4)].astype(BF16))
                y = _lane_exchange([y_v[r, _tile(4 * m + p)] for p in range(4)])
                y = [v if q == 0 else pltpu.roll(v, 128 - q, 1) for q, v in enumerate(y)]
                for q in (0, 2):
                    out = []
                    for t in (q, q + 1):
                        x, xn = [pltpu.bitcast(w[rw, _tile(4 * m + t)], BF16).astype(F32)
                                 for w in (x_v, xn_v)]
                        h = xn + upd[:, _tile(t)]
                        out.append(x + (y[t] + xn * skip) * (h + h * jnp.tanh(h)))
                    o_v[r, _tile(4 * m + q, 2)] = jnp.concatenate(out, axis=1).astype(BF16)
                yield

    cp_d(0).wait()
    def first_down():
        yield from ffn_down(0)
        yt_v[...] = yr_v[...].T
        yield from ffn_down(1)

    def send(row, n):
        r = _ds(row, n)
        pltpu.make_async_copy(o_v.at[r], o_hbm.at[r], sem.at[3]).start()

    _run("", d=first_down())

    @pl.loop(0, NCB - 2)
    def _(i):
        @pl.when(i == HOLD)
        def _():
            cp_d(1).wait()
            send(0, HOLD * CB)

        pl.when(i + 2 == (D - LAST) // CB)(cp_d(2).wait)
        yt = yt_v[...]
        yt_v[...] = yr_v[...].T
        _run(D_ORDER, o=finish(i, yt), d=ffn_down(i + 2))
        pl.when(i >= HOLD)(lambda: send(i * CB, CB))

    _run(P_ORDER.replace("I", "i" * (PI // 4)), o=finish(NCB - 2, yt_v[...]),
         i=inverse(NCB - 1, z_v, [], PI))
    send(D - 2 * CB, CB)
    last = finish(NCB - 1, yr_v[...].T)
    for row in (D - CB, D - CB // 2):
        for _ in range(4):
            next(last)
        send(row, CB // 2)
    pltpu.make_async_copy(o_v, o_hbm, sem.at[3]).wait()


@jax.jit
def pallas_recurrent_scan__ssm_conv_s4__moe_arch_mod__prompt_kernel(
    A_u: jax.Array,
    A_A_re: jax.Array,
    A_A_im: jax.Array,
    A_B_re: jax.Array,
    A_B_im: jax.Array,
    A_C_re: jax.Array,
    A_C_im: jax.Array,
    A_log_dt: jax.Array,
    A_Dskip: jax.Array,
    B_x: jax.Array,
    B_w_r: jax.Array,
    B_w_gate: jax.Array,
    B_w_up: jax.Array,
    B_w_down: jax.Array,
):
    del B_x
    assert A_u.shape == (1, L, D) and A_A_re.shape == (D, N) and B_w_gate.shape == (D, F)
    hbm = pl.BlockSpec(memory_space=pl.ANY)
    vmem = pltpu.VMEM
    out = pl.pallas_call(
        _kernel,
        out_shape=jax.ShapeDtypeStruct((D, L), BF16),
        in_specs=[hbm] * 13,
        out_specs=hbm,
        scratch_shapes=[
            vmem((D // 2, L), U32), vmem((6, D, N), BF16),
            vmem((D,), BF16), vmem((D,), BF16), vmem((D,), BF16),
            vmem((D // 2, F), U32), vmem((D // 2, F), U32), vmem((D // 2, F), U32),
            vmem((5, 64, 1024), U32), vmem((CB, 1024), F32), vmem((D, L), BF16),
            vmem((D // 2, L), U32), vmem((D // 2, L), U32),
            vmem((D, 4096), F32), vmem((4 * CB, 1024), F32), vmem((4 * CB, 1024), F32),
            vmem((D, L), F32), vmem((CB, 18 * 128), F32),
            *[vmem((D, 128), F32)] * 4,
            vmem((10, CB, 128), F32), vmem((7, CB, 128), VT),
            vmem((TOPC, L), F32), vmem((TOPC, D), F32), vmem((TOPC, F), F32),
            vmem((TOPC, DB), F32), vmem((DB, TOPC), F32),
            pltpu.SemaphoreType.DMA((8 + NCB // WG,)),
        ],
        compiler_params=pltpu.CompilerParams(vmem_limit_bytes=100 * 1024 * 1024),
    )(A_u[0].T, A_A_re, A_A_im, A_B_re, A_B_im, A_C_re, A_C_im, A_log_dt, A_Dskip, B_w_r,
      B_w_gate, B_w_up, B_w_down.T)
    return out.T[None]
```

```python
import jax
import jax.numpy as jnp
import numpy as np
import jax.experimental.pallas as pl
import jax.experimental.pallas.tpu as pltpu

F32, BF16, I32, U32 = jnp.float32, jnp.bfloat16, jnp.int32, jnp.uint32

L, D, N, F = 2048, 576, 128, 4608
TOPC = 8
BLK = 512
CB = 64
NCB = D // CB
FB = F // NCB
DB = 64
NT = (((1,), (1,)), ((), ()))
Q_PAIRS = ((3, 1), (7, 5), (2, 258), (4, 260), (6, 262), (8, 264),
           (516, 772), (520, 776), (1032, 1288), (1544, 1800))
GROUPS = ((6, 7), (8, 9), (3, 5), (0, 1), (2, 4))
K_ORDER = "cssvspvpvsspvppvvpssvpspv"
C_ORDER = "mimimiimiimmimimuimimimiimimimimimumimiimimimmimimuimimimimimimimmimufmfmmffmmmfmmfmfmfmuufmfmfmfmmfmmfmmfmfmufmfmfmffmffmmfmfmuuuffffffmf"
D_ORDER = "ododododododododd"
L_ORDER = "cmssmnsssmsstsntmnttntttt"
LT = 4
NT_ = 4
EARLY = 4
MID = 5
PN = 8
PI = 32
P_ORDER = "oo I oo I oo I o I o"
M3 = True
VT = 'float32'
WG = 3
LAST = 48
HOLD = 2


def _round_to_bf16(v):
    u = np.asarray(v, np.float32).view(np.uint32)
    return ((u + 0x7FFF + ((u >> 16) & 1)) & 0xFFFF0000).astype(np.uint32).view(np.float32)


def _cmul(a, b):
    return a[0] * b[0] - a[1] * b[1], a[0] * b[1] + a[1] * b[0]


def _csq(a):
    return (a[0] + a[1]) * (a[0] - a[1]), (a[0] + a[0]) * a[1]


def _cadd(a, b):
    return a[0] + b[0], a[1] + b[1]


def _csub(a, b):
    return a[0] - b[0], a[1] - b[1]


def _add_i(a, b):
    return a[0] - b[1], a[1] + b[0]


def _sub_i(a, b):
    return a[0] + b[1], a[1] - b[0]


def _lane_exchange(r):
    lane = jax.lax.broadcasted_iota(I32, r[0].shape, 1)
    a = [jnp.where((lane & 1) == 1, r[(j + 1) % 4], r[j]) for j in range(4)]
    b = [jnp.where((lane & 2) == 2, a[(j + 2) % 4], a[j]) for j in range(4)]
    return [b[-j % 4] for j in range(4)]


def _rb(v):
    return v.astype(BF16).astype(F32)


def _silu(v):
    h = 0.5 * v
    return h + h * jnp.tanh(h)


def _tile(t, n=1):
    return slice(128 * t, 128 * (t + n))


def _ds(start, size, align=None):
    if isinstance(start, int):
        return pl.ds(start, size)
    return pl.ds(pl.multiple_of(start, align or size), size)


def _dot(a, b):
    return jnp.dot(a, b, preferred_element_type=F32)


def _dot_nt(a, b):
    return jax.lax.dot_general(a, b, NT, preferred_element_type=F32)


def _run(order, **stages):
    for step in order.replace(" ", ""):
        next(stages[step])
    for stage in stages.values():
        for _ in stage:
            pass


def _pacer(step):
    clock = []

    def after(v):
        if not clock:
            return v
        always = jax.lax.broadcasted_iota(I32, v.shape, 1) < step + 128
        return jnp.where(always, v, jnp.tile(clock[-1], (v.shape[0] // 8, 1)))

    return clock, after


def _sort_rows(v, sizes):
    sub = jax.lax.broadcasted_iota(I32, v.shape, 0)
    for k in sizes:
        j = k // 2
        while j:
            w = jnp.take_along_axis(v, sub ^ j, axis=0)
            v = jnp.where(((sub & j) == 0) == ((sub & k) == 0),
                          jnp.maximum(v, w), jnp.minimum(v, w))
            j //= 2
    return v


def _merge_top(a, b):
    sub = jax.lax.broadcasted_iota(I32, a.shape, 0)
    return _sort_rows(jnp.maximum(a, jnp.take_along_axis(b, 7 - sub, axis=0)), (8,))


def _write_tables(tab_v, edge_v):
    sub = jax.lax.broadcasted_iota(I32, (8, 128), 0)
    lane = jax.lax.broadcasted_iota(I32, (8, 128), 1)
    ang = (((4 * lane + 1) << sub) & (4 * BLK - 1)).astype(F32) * (np.pi / (2 * BLK))
    bits = jnp.cos(ang), jnp.sin(ang)
    known = {1 << s: [jnp.broadcast_to(v[s:s + 1], (8, 128)) for v in bits] for s in range(8)}
    known[0] = [jnp.ones((8, 128), F32), jnp.zeros((8, 128), F32)]

    def times_i(z, n):
        for _ in range(n % 4):
            z = (-z[1], z[0])
        return z

    def power(t):
        if t >= BLK:
            return times_i(power(t - BLK), 1)
        if t not in known:
            low = t & -t if t & (t - 1) else t // 2
            known[t] = _cmul(power(t - low), power(low))
        return known[t]

    def put(cond, z, base):
        return [jnp.where(cond, v, w) for v, w in zip(z, base)]

    def lag_sum(ts, s):
        terms = [times_i(power(t), s * t) for t in ts]
        return [sum(z[c] for z in terms) for c in range(2)]

    def ramp(step):
        z = put((sub & 1) == 1, power(step), known[0])
        for b in (2, 4):
            z = _cmul(z, put((sub & b) == b, power(b * step), known[0]))
        return z

    def store(t, col, tiles):
        for c in range(2):
            tab_v[t, :, _tile(col + c)] = jnp.concatenate(
                [z[c] for z in tiles], axis=0).astype(BF16)

    ramp1, ramp8 = ramp(1), ramp(8)
    for p in range(4):
        q, z = (sub - p) & 3, known[0]
        for n in (1, 2, 3):
            z = put(q == n, power(127 * n), z)
        z = [_cmul(ramp1, z)]
        for _ in range(16):
            z.append(_cmul(z[-1], power(8)))
        store(0, 2 * p, [put(sub < q, z[16], z[0])] + z[1:16])

    lag_exp = _round_to_bf16(np.arange(L)).astype(np.int64)
    c = np.arange(128)
    gc, gd, g4, go, g2 = [
        np.concatenate([Q_PAIRS[v][e] + 8 * np.arange(32) for e in range(2) for v in vs])
        for vs in GROUPS]
    g1 = np.where((c >= 63) & (c < 127), g4, np.roll(go, 63))
    g3, ge = np.where(c < 64, go, g4), np.where(c == 127, gc, gd)
    ramps = {}

    def ramp_from(t):
        if t not in ramps:
            ramps[t] = (_cmul(ramps[t - 64], power(64)) if t - 64 in ramps
                        else _cmul(ramp8, power(t)))
        return ramps[t]

    def lags(e, m, phase=None):
        ts = [int(l) - BLK * m for l in np.nonzero(lag_exp == e)[0] if 0 < l - BLK * m <= BLK]
        return [t for t in ts if phase is None or t % 4 == phase]

    def rows(tss, s):
        z, runs = [known[0][1]] * 2, [[]] * 8
        if tss[0]:
            half = [len(ts) // 2 for ts in tss[:2]]
            t = tss[0][half[0]]
            runs = [list(range(t + 8 * r - half[r % 2], t + 8 * r + half[r % 2] + 1))
                    for r in range(8)]
            z = ramp_from(t)
            if any(half):
                assert t % 4 == 0
                even, odd = [1.0 + 2.0 * lag_sum(range(1, h + 1), s)[0] for h in half]
                z = [v * jnp.where((sub & 1) == 1, odd, even) for v in z]
        for r, ts in enumerate(tss):
            if ts != runs[r]:
                z = put(sub == r, lag_sum(ts, s), z)
        return z

    for p, g in enumerate((g4, g1, g2, g3)):
        store(1, 2 * p, [rows([lags(e, 0, p) for e in es], 0) for es in g.reshape(16, 8)])
    for m, g in ((1, gc), (2, ge), (3, gd)):
        for s in range(4):
            store(1 + m, 2 * s, [rows([lags(e, m) for e in es], s) for es in g.reshape(16, 8)])
    for s in range(4):
        edge_v[:, _tile(2 * s, 2)] = jnp.tile(
            jnp.concatenate(lag_sum(lags(BLK, 1), s), axis=1), (CB // 8, 1))


def _ssm_powers(par, dt):
    a_re, a_im, b_re, b_im, c_re, c_im = par
    mag = jnp.exp(dt * a_re)
    ang = dt * a_im
    pw = {1: (mag * jnp.cos(ang), mag * jnp.sin(ang))}
    for k in range(9):
        pw[2 << k] = _csq(pw[1 << k])
    sc = dt * (2.0 / BLK)
    w = _cmul((c_re, c_im), (b_re * sc, b_im * sc))
    w1, w2 = _cmul(w, pw[1]), _cmul(w, pw[2])
    return [pw[8], pw[16], pw[2], pw[4], pw[512],
            w1, _cmul(w1, pw[2]), w2, _cmul(w2, pw[256])], w[0]


def _ssm_products(pw):
    a8, a16, a2, a4, a512, w1, w3, w2, w258 = pw
    sub = jax.lax.broadcasted_iota(I32, (8, 128), 0)
    lane = jax.lax.broadcasted_iota(I32, (8, 128), 1)
    lo = sub < 4

    def pick(z, rows):
        return [jnp.take_along_axis(v, rows, axis=0) for v in z]

    def pair(x, y, h):
        r = [pltpu.roll(v, 4, 0) for v in y]
        return [jnp.where(lo, s, v) if h else jnp.where(lo, v, s) for v, s in zip(x, r)]

    out = []
    for h in range(2):
        p_rows, q_rows = 4 * h + ((sub + 2 * h) & 3), 4 * h + (sub & 3)
        step, s2, s512 = pick(a16, p_rows), pick(a2, q_rows), pick(a512, q_rows)
        p = [[jnp.where(lo, one, v) for one, v in zip((1.0, 0.0), pick(a8, p_rows))]]
        for _ in range(15):
            p.append(_cmul(p[-1], step))
        q = [pair(w3, w1, h)]
        q += [_cmul(q[0], pick(a4, q_rows)), pair(w2, w258, h)]
        for _ in range(3):
            q.append(_cmul(q[-1], s2))
        q += [_cmul(q[3], s512), _cmul(q[5], s512)]
        for _ in range(2):
            q.append(_cmul(q[-1], s512))
        out.append([_dot_nt(*[jnp.concatenate([z[j] for z in zs], axis=0).astype(BF16)
                              for zs in (q, p)]) for j in range(2)])
    first = ((lane - sub) & 3) == 0
    return [jnp.where(first, out[0][0][v:v + 8], out[1][0][v:v + 8])
            - jnp.where(first, out[0][1][v:v + 8], out[1][1][v:v + 8]) for v in range(0, 80, 8)]


def _kernel(x_hbm, are_hbm, aim_hbm, bre_hbm, bim_hbm, cre_hbm, cim_hbm, ldt_hbm, dsk_hbm, wr_hbm,
            wg_hbm, wu_hbm, wd_hbm, o_hbm,
            x_v, par_v, ldt_v, dsk_v, wr_v, wg_v, wu_v, wd_v, tab_v, edge_v, o_v,
            xn_v, ph_v, kf_v, uf_v, z_v, y_v, pw_v, dt_v, k0_v, k512_v, skip_v, raw_v, vec_v,
            hot_v, xs_v, h_v, yr_v, yt_v, sem):
    def rows(i):
        return _ds(i * CB, CB)

    x_v, wg_v, wu_v, wd_v, tab_v, xn_v, ph_v = [
        v.bitcast(BF16) for v in (x_v, wg_v, wu_v, wd_v, tab_v, xn_v, ph_v)]

    pars = (are_hbm, aim_hbm, bre_hbm, bim_hbm, cre_hbm, cim_hbm)
    cp_dt = pltpu.make_async_copy(ldt_hbm, ldt_v, sem.at[0])
    cp_head, cp_rest = [
        [pltpu.make_async_copy(p.at[r], par_v.at[j, r], sem.at[k]) for j, p in enumerate(pars)]
        for k, r in ((1, pl.ds(0, 2 * CB)), (4, pl.ds(2 * CB, D - 2 * CB)))]
    cp_x = [pltpu.make_async_copy(s, d, sem.at[2])
            for s, d in ((x_hbm, x_v), (dsk_hbm, dsk_v), (wr_hbm, wr_v))]

    def cp_w(i):
        c = _ds(i * WG * FB, WG * FB)
        return [pltpu.make_async_copy(s.at[:, c], d.at[:, c], sem.at[5 + i])
                for s, d in ((wg_hbm, wg_v), (wu_hbm, wu_v))]

    def cp_d(i):
        cuts = (0, (HOLD + 2) * CB, D - LAST, D)
        r = pl.ds(cuts[i], cuts[i + 1] - cuts[i])
        return pltpu.make_async_copy(wd_hbm.at[r], wd_v.at[r],
                                     sem.at[5 + NCB // WG + i])

    for c in [cp_dt] + cp_head + cp_rest + cp_x:
        c.start()

    def table(t, lo, n):
        return tab_v[t, :, _tile(lo, n)]

    raw_v[...] = jnp.zeros(raw_v.shape, F32)
    vec_v[...] = jnp.zeros(vec_v.shape, VT)
    _write_tables(tab_v, edge_v)

    cp_dt.wait()
    dt_row = _rb(jnp.exp(ldt_v[...].astype(F32).reshape(1, D)))
    dt_v[...] = jnp.broadcast_to(dt_row, (128, D)).T
    for c in cp_head:
        c.wait()

    def kernel_powers(i, after):
        par = [par_v[t, rows(i), :].astype(F32) for t in range(6)]
        k0 = []
        for g in range(0, CB, PN):
            pw, w = _ssm_powers([v[g:g + PN] for v in par], after(dt_v[_ds(i * CB + g, PN), :]))
            pw_v[g:g + PN, :] = jnp.concatenate([v for z in pw for v in z], axis=1)
            k0_v[_ds(i * CB + g, PN), :] = jnp.broadcast_to(
                jnp.sum(w, axis=1, keepdims=True), (PN, 128))
            yield

    def kernel_values(pw, clock):
        for g in range(0, CB, 8):
            out = _ssm_products([(pw[g:g + 8, _tile(2 * t)], pw[g:g + 8, _tile(2 * t + 1)])
                                 for t in range(9)])
            for v in range(10):
                raw_v[v, g:g + 8, :] = out[v]
            clock.append(out[0])
            yield

    def kernel_vectors(i, raw):
        sub = jax.lax.broadcasted_iota(I32, (8, 128), 0)
        lane = jax.lax.broadcasted_iota(I32, (8, 128), 1)
        odd = ((lane - sub) & 1) == 1
        own = ((lane - sub) & 2) == ((sub & 4) >> 1)
        perm = (4 * (lane & 31) + ((sub + ((sub & 4) >> 1)) & 3) + (lane >> 5)) & 127
        u = [jnp.where(odd, pltpu.roll(raw[v1, g:g + 8], 1, 1), raw[v0, g:g + 8])
             for v0, v1 in GROUPS for g in range(0, CB, 8)]
        u = [jnp.where(own, v, pltpu.roll(pltpu.roll(v, 4, 0), 2, 1)) for v in u]
        u = [jnp.take_along_axis(v, perm, axis=1) for v in u]
        gc, gd, g4, go, g2 = [u[t:t + CB // 8] for t in range(0, len(u), CB // 8)]
        mid, last = (lane >= 63) & (lane < 127), lane == 127
        g1 = [jnp.where(mid, a, pltpu.roll(b, 63, 1)) for a, b in zip(g4, go)]
        g3 = [jnp.where(lane < 64, b, a) for a, b in zip(g4, go)]
        ge = [jnp.where(last, a, b) for a, b in zip(gc, gd)]
        for t, v in enumerate((g4, g1, g2, g3, gc, ge, gd)):
            vec_v[t] = jnp.concatenate(v, axis=0).astype(VT)
        k512_v[rows(i), :] = jnp.broadcast_to(jnp.sum(
            jnp.concatenate([jnp.where(last, a, 0.0) for a in g4], axis=0),
            axis=1, keepdims=True), (CB, 128))
        yield

    def kernel_spectrum(i, vec, clock):
        for m in (1, 3, 2):
            for t in (0, 4):
                f = _dot(vec[3 + m].astype(BF16), table(1 + m, t, 4))
                kf_v[rows(i), _tile(8 * m + t, 4)] = f
                clock.append(f[0:8, 0:128])
                yield
        for p in range(2):
            a, b = [_dot(vec[t].astype(BF16), table(1, 2 * t, 2)) for t in (p, p + 2)]
            kf_v[rows(i), _tile(4 * p, 2)] = a + b
            kf_v[rows(i), _tile(4 * p + 2, 2)] = a - b
            clock.append(a[0:8, 0:128])
            yield

    _run("", p=kernel_powers(0, lambda v: v))
    for j in range(NCB // WG):
        for c in cp_w(j):
            c.start()
    for j in range(3):
        cp_d(j).start()

    @pl.loop(0, NCB)
    def _(i):
        @pl.when(i == 1)
        def _():
            for c in cp_rest:
                c.wait()

        clock, after = _pacer(i)
        _run(K_ORDER, s=kernel_spectrum(jnp.maximum(i - 2, 0), vec_v[...], clock),
             c=kernel_vectors(jnp.maximum(i - 1, 0), raw_v[...]),
             v=kernel_values(pw_v[...], clock),
             p=kernel_powers(jnp.minimum(i + 1, NCB - 1), after))

    for c in cp_x:
        c.wait()
    skip_v[...] = jnp.broadcast_to(dsk_v[...].astype(F32).reshape(1, D), (128, D)).T
    wr = jnp.broadcast_to(wr_v[...].astype(F32).reshape(1, D), (TOPC, D)).astype(BF16)
    eps = float(_round_to_bf16(1e-5))
    mean, score = [], []

    def token_mean():
        for t in range(0, L // 128, LT):
            m = _dot(jnp.ones((8, D), BF16), x_v[:, _tile(t, LT)]) * (1.0 / D)
            mean.extend(m[:, _tile(j)] for j in range(LT))
            yield

    def split_phases(i, ms=range(4)):
        r = rows(i)
        for m in ms:
            v = [pltpu.bitcast(xn_v[r, _tile(4 * m + q)], U32) for q in range(4)]
            v = _lane_exchange([w if q == 0 else pltpu.roll(w, q, 1) for q, w in enumerate(v)])
            for p in range(4):
                ph_v[r, _tile(4 * m + p)] = pltpu.bitcast(v[p], BF16)

    def center():
        for t in range(L // 128):
            mb, sq, cen = _rb(mean[t]), [0.0, 0.0], []
            for r in range(0, D, 16):
                x = x_v[r:r + 16, _tile(t)].astype(F32)
                d = [x[0:8] - mb, x[8:16] - mb]
                sq = [a + v * v for a, v in zip(sq, d)]
                cen.append(jnp.concatenate(d, axis=1).astype(BF16))
            var = (jnp.sum(sq[0] + sq[1], axis=0, keepdims=True) * (1.0 / D)
                   - jnp.square(mean[t] - mb))
            yield cen, 0.5 / _rb(jnp.sqrt(_rb(_rb(jnp.maximum(var, 0.0)) + eps)))

    def normalize():
        tiles = center()
        for t in range(0, L // 128, NT_):
            out = jnp.concatenate([
                jnp.concatenate([d.astype(F32)[:, _tile(j)] * inv for d in cen for j in range(2)],
                                axis=0)
                for cen, inv in [next(tiles) for _ in range(NT_)]], axis=1).astype(BF16)
            xn_v[:, _tile(t, NT_)] = out
            for i in range(EARLY):
                split_phases(i, [t // 4])
            score.append(_rb(2.0 * _dot(wr, out)))
            yield

    _run(L_ORDER, s=kernel_spectrum(NCB - 2, vec_v[...], []), c=kernel_vectors(NCB - 1, raw_v),
         t=kernel_spectrum(NCB - 1, vec_v, []), m=token_mean(), n=normalize())
    score = jnp.concatenate(score, axis=1)

    def forward(i, clock):
        for h in range(0, CB, 32):
            for p in range(2):
                a, b = [_dot(
                    jnp.concatenate([ph_v[_ds(i * CB + g, 16), _tile(4 * m + t)]
                                     for g in (h, h + 16) for m in range(4)], axis=0),
                    table(0, 2 * t, 2)) for t in (p, p + 2)]
                uf_v[4 * h:4 * h + 128, _tile(4 * p, 2)] = a + b
                uf_v[4 * h:4 * h + 128, _tile(4 * p + 2, 2)] = a - b
                for r in range(0, 128, 16):
                    clock.append(a[r:r + 8, 0:128])
                    yield

    def multiply(i, uf, after):
        def pair(src, r, t):
            return src[r, _tile(t)], src[r, _tile(t + 1)]

        for g in range(0, CB, 8):
            r = _ds(i * CB + g, 8)
            ru = [slice(64 * (g // 16) + 16 * m + g % 16, 64 * (g // 16) + 16 * m + g % 16 + 8)
                  for m in range(4)]
            for s, ops in enumerate(((_cadd, _csub), (_add_i, _sub_i))):
                ks, us = [], []
                for t, op in zip((s, s + 2), ops):
                    k = [op(pair(kf_v, r, 2 * s), pair(kf_v, r, 2 * s + 4))]
                    k += [pair(kf_v, r, 8 * m + 2 * t) for m in (1, 2, 3)]
                    k[1] = [v + k512_v[r, :] * edge_v[g:g + 8, _tile(2 * t + c)]
                            for c, v in enumerate(k[1])]
                    k = [k[0]] + [_sub_i(k[m], k[m - 1]) for m in (1, 2, 3)]
                    ks.append([(c, d - c, c + d) if M3 else (c, d) for c, d in k])
                    u = [op(pair(uf, v, 2 * s), pair(uf, v, 2 * s + 4)) for v in ru]
                    us.append([(a + b, a, b) if M3 else (a, b) for a, b in u])
                for n in range(4):
                    z = []
                    for k, u in zip(ks, us):
                        if not M3:
                            acc = _cmul(k[0], u[n] if z else (after(u[n][0]), u[n][1]))
                            for m in range(1, n + 1):
                                acc = _cadd(acc, _cmul(k[m], u[n - m]))
                            z.append(acc)
                            continue
                        acc = [v * w for v, w in zip(k[0], u[n])]
                        if not z:
                            acc[0] = after(acc[0])
                        for m in range(1, n + 1):
                            acc = [a + v * w for a, v, w in zip(acc, k[m], u[n - m])]
                        z.append((acc[0] - acc[2], acc[0] + acc[1]))
                    for t, v in enumerate(_cadd(*z) + _csub(*z)):
                        z_v[pl.ds(4 * g + 8 * n, 8), _tile(4 * s + t)] = v
                    yield

    def inverse(i, z, clock, n=32):
        for h in range(0, CB, n):
            for p, ops in enumerate(((_cadd, _csub), (_sub_i, _add_i))):
                a, c = [[z[4 * h:4 * h + 4 * n, _tile(4 * s + 2 * p + t)] for t in range(2)]
                        for s in range(2)]
                y = [_dot_nt(jnp.concatenate(op(a, c), axis=1).astype(BF16),
                             table(0, 2 * p + 4 * t, 2)) for t, op in enumerate(ops)]
                for g in range(0, n, 8):
                    for m in range(4):
                        for t in range(2):
                            y_v[_ds(i * CB + h + g, 8), _tile(4 * m + p + 2 * t)] = (
                                y[t][4 * g + 8 * m:4 * g + 8 * m + 8])
                for r in range(0, 4 * n, 16):
                    clock.append(y[0][r:r + 8])
                    yield

    bits = pltpu.bitcast(jnp.where(score == 0.0, 0.0, score), I32) >> 16
    pos = jax.lax.broadcasted_iota(I32, (TOPC, L), 1)
    key = ((bits ^ ((bits >> 15) & 0x7FFF)) << 11) + (0x38000000 + L - 1 - pos)
    key = pltpu.bitcast(key, F32)
    sub = jax.lax.broadcasted_iota(I32, (TOPC, 128), 0)
    dense = []
    for t0 in (0, 8):
        v = key[:, _tile(t0)]
        for t in range(1, 8):
            v = jnp.where(sub == t, key[:, _tile(t0 + t)], v)
        dense.append(v)
    _run("", f=forward(0, []))
    top = _merge_top(*[_sort_rows(v, (2, 4, 8)) for v in dense])
    for step, count in ((8, 16), (1, 8)):
        top = [top] + [pltpu.roll(top, step * k, 1) for k in range(1, count)]
        while len(top) > 1:
            top = [_merge_top(a, b) for a, b in zip(top[0::2], top[1::2])]
        top = top[0]
        for i in range(*{8: (EARLY, MID), 1: (MID, NCB)}[step]):
            split_phases(i)
    hot_v[...] = jnp.where(key == jnp.tile(top, (1, L // 128)), 1.0, 0.0)
    top = pltpu.bitcast(top, I32) - 0x38000000
    tb = top >> 11
    gate = _rb(jax.nn.sigmoid(pltpu.bitcast((tb ^ ((tb >> 15) & 0x7FFF)) << 16, F32)))
    tok = (L - 1) - (top & (L - 1))
    pick = (tok & 127) == jax.lax.broadcasted_iota(I32, (TOPC, 128), 1)
    xs_v[...] = xs = _dot_nt(
        jnp.concatenate([jnp.where(pick & (sub == c), 2.0, 0.0) for c in range(TOPC)],
                        axis=1).astype(BF16),
        jnp.concatenate([xn_v[:, _ds(tok[c, 0] & (L - 128), 128)] for c in range(TOPC)], axis=1))

    z_v[...] = jnp.tile(xs[:, 0:128], (4 * CB // TOPC, 8))

    def ffn_up(i):
        acc = [0.0, 0.0]
        for j in range(0, D, 128):
            n = min(128, D - j)
            for t, w in enumerate((wg_v, wu_v)):
                acc[t] = acc[t] + _dot(
                    xs_v[:, j:j + n].astype(BF16),
                    w[j:j + n, _ds(i * FB, FB)])
                yield
        h_v[:, _ds(i * FB, FB)] = _rb(_silu(_rb(acc[0]))) * _rb(acc[1])

    @pl.loop(0, NCB)
    def _(i):
        for j in range(NCB // WG):
            @pl.when(i == j * WG)
            def _():
                for c in cp_w(j):
                    c.wait()

        clock, after = _pacer(i)
        _run(C_ORDER.replace('I', 'im' * 8).replace('F', 'fm' * 8).replace('J', 'imimimim' * 2 + 'm').replace('G', 'fmfmmfmfmm' * 2).replace('E', 'fmfmmfmm' * 2 + 'fmfm').replace('H', 'f' * 8), i=inverse(jnp.maximum(i - 1, 0), z_v[...], clock),
             m=multiply(i, uf_v[...], after), u=ffn_up(i),
             f=forward(jnp.minimum(i + 1, NCB - 1), clock))

    def ffn_down(i):
        y = 0.0
        for j in range(0, F, FB):
            y = y + _dot_nt(h_v[:, j:j + FB].astype(BF16),
                            wd_v[rows(i), j:j + FB])
            if j + FB == F:
                yr_v[...] = 0.5 * _rb(_rb(y) * gate[:, :DB])
            yield

    def finish(i, yt):
        for g in range(0, DB, 32):
            r = _ds(i * CB + g, 32)
            skip = 2.0 * skip_v[r, :] + BLK * k0_v[r, :]
            for m in range(4):
                upd = _dot(yt[g:g + 32].astype(BF16), hot_v[:, _tile(4 * m, 4)].astype(BF16))
                y = _lane_exchange([y_v[r, _tile(4 * m + p)] for p in range(4)])
                y = [v if q == 0 else pltpu.roll(v, 128 - q, 1) for q, v in enumerate(y)]
                for q in (0, 2):
                    out = []
                    for t in (q, q + 1):
                        x, xn = [w[r, _tile(4 * m + t)].astype(F32)
                                 for w in (x_v, xn_v)]
                        h = xn + upd[:, _tile(t)]
                        out.append(x + (y[t] + xn * skip) * (h + h * jnp.tanh(h)))
                    o_v[r, _tile(4 * m + q, 2)] = jnp.concatenate(out, axis=1).astype(BF16)
                yield

    cp_d(0).wait()
    def first_down():
        yield from ffn_down(0)
        yt_v[...] = yr_v[...].T
        yield from ffn_down(1)

    def send(row, n):
        r = _ds(row, n)
        pltpu.make_async_copy(o_v.at[r], o_hbm.at[r], sem.at[3]).start()

    _run("", d=first_down())

    @pl.loop(0, NCB - 2)
    def _(i):
        @pl.when(i == HOLD)
        def _():
            cp_d(1).wait()
            send(0, HOLD * CB)

        pl.when(i + 2 == (D - LAST) // CB)(cp_d(2).wait)
        yt = yt_v[...]
        yt_v[...] = yr_v[...].T
        _run(D_ORDER, o=finish(i, yt), d=ffn_down(i + 2))
        pl.when(i >= HOLD)(lambda: send(i * CB, CB))

    _run(P_ORDER.replace("I", "i" * (PI // 4)), o=finish(NCB - 2, yt_v[...]),
         i=inverse(NCB - 1, z_v, [], PI))
    send(D - 2 * CB, CB)
    last = finish(NCB - 1, yr_v[...].T)
    for row in (D - CB, D - CB // 2):
        for _ in range(4):
            next(last)
        send(row, CB // 2)
    pltpu.make_async_copy(o_v, o_hbm, sem.at[3]).wait()


@jax.jit
def pallas_recurrent_scan__ssm_conv_s4__moe_arch_mod__prompt_kernel(
    A_u: jax.Array,
    A_A_re: jax.Array,
    A_A_im: jax.Array,
    A_B_re: jax.Array,
    A_B_im: jax.Array,
    A_C_re: jax.Array,
    A_C_im: jax.Array,
    A_log_dt: jax.Array,
    A_Dskip: jax.Array,
    B_x: jax.Array,
    B_w_r: jax.Array,
    B_w_gate: jax.Array,
    B_w_up: jax.Array,
    B_w_down: jax.Array,
):
    del B_x
    assert A_u.shape == (1, L, D) and A_A_re.shape == (D, N) and B_w_gate.shape == (D, F)
    hbm = pl.BlockSpec(memory_space=pl.ANY)
    vmem = pltpu.VMEM
    out = pl.pallas_call(
        _kernel,
        out_shape=jax.ShapeDtypeStruct((D, L), BF16),
        in_specs=[hbm] * 13,
        out_specs=hbm,
        scratch_shapes=[
            vmem((D // 2, L), U32), vmem((6, D, N), BF16),
            vmem((D,), BF16), vmem((D,), BF16), vmem((D,), BF16),
            vmem((D // 2, F), U32), vmem((D // 2, F), U32), vmem((D // 2, F), U32),
            vmem((5, 64, 1024), U32), vmem((CB, 1024), F32), vmem((D, L), BF16),
            vmem((D // 2, L), U32), vmem((D // 2, L), U32),
            vmem((D, 4096), F32), vmem((4 * CB, 1024), F32), vmem((4 * CB, 1024), F32),
            vmem((D, L), F32), vmem((CB, 18 * 128), F32),
            *[vmem((D, 128), F32)] * 4,
            vmem((10, CB, 128), F32), vmem((7, CB, 128), VT),
            vmem((TOPC, L), F32), vmem((TOPC, D), F32), vmem((TOPC, F), F32),
            vmem((TOPC, DB), F32), vmem((DB, TOPC), F32),
            pltpu.SemaphoreType.DMA((8 + NCB // WG,)),
        ],
        compiler_params=pltpu.CompilerParams(vmem_limit_bytes=100 * 1024 * 1024),
    )(A_u[0].T, A_A_re, A_A_im, A_B_re, A_B_im, A_C_re, A_C_im, A_log_dt, A_Dskip, B_w_r,
      B_w_gate, B_w_up, B_w_down.T)
    return out.T[None]
```

```python
import jax
import jax.numpy as jnp
import numpy as np
import jax.experimental.pallas as pl
import jax.experimental.pallas.tpu as pltpu

F32, BF16, I32, U32 = jnp.float32, jnp.bfloat16, jnp.int32, jnp.uint32

L, D, N, F = 2048, 576, 128, 4608
TOPC = 8
BLK = 512
CB = 64
NCB = D // CB
FB = F // NCB
DB = 64
NT = (((1,), (1,)), ((), ()))
Q_PAIRS = ((3, 1), (7, 5), (2, 258), (4, 260), (6, 262), (8, 264),
           (516, 772), (520, 776), (1032, 1288), (1544, 1800))
GROUPS = ((6, 7), (8, 9), (3, 5), (0, 1), (2, 4))
K_ORDER = "cssvspvpvsspvppvvpssvpspv"
C_ORDER = "mimimiimiimmimimuimimimiimimimimimumimiimimimmimimuimimimimimimimmimufmfmmffmmmfmmfmfmfmuufmfmfmfmmfmmfmmfmfmufmfmfmffmffmmfmfmuuuffffffmf"
D_ORDER = "ododododododododd"
L_ORDER = "cmssmnsssmsstsntmnttntttt"
LT = 4
NT_ = 4
EARLY = 4
MID = 5
PN = 8
PI = 32
P_ORDER = "oo I oo I oo I o I o"
M3 = True
VT = 'float32'
WG = 3
LAST = 64
HOLD = 2
PR = (0, 0, 0)
DC = 3


def _round_to_bf16(v):
    u = np.asarray(v, np.float32).view(np.uint32)
    return ((u + 0x7FFF + ((u >> 16) & 1)) & 0xFFFF0000).astype(np.uint32).view(np.float32)


def _cmul(a, b):
    return a[0] * b[0] - a[1] * b[1], a[0] * b[1] + a[1] * b[0]


def _csq(a):
    return (a[0] + a[1]) * (a[0] - a[1]), (a[0] + a[0]) * a[1]


def _cadd(a, b):
    return a[0] + b[0], a[1] + b[1]


def _csub(a, b):
    return a[0] - b[0], a[1] - b[1]


def _add_i(a, b):
    return a[0] - b[1], a[1] + b[0]


def _sub_i(a, b):
    return a[0] + b[1], a[1] - b[0]


def _lane_exchange(r):
    lane = jax.lax.broadcasted_iota(I32, r[0].shape, 1)
    a = [jnp.where((lane & 1) == 1, r[(j + 1) % 4], r[j]) for j in range(4)]
    b = [jnp.where((lane & 2) == 2, a[(j + 2) % 4], a[j]) for j in range(4)]
    return [b[-j % 4] for j in range(4)]


def _rb(v):
    return v.astype(BF16).astype(F32)


def _silu(v):
    h = 0.5 * v
    return h + h * jnp.tanh(h)


def _tile(t, n=1):
    return slice(128 * t, 128 * (t + n))


def _ds(start, size, align=None):
    if isinstance(start, int):
        return pl.ds(start, size)
    return pl.ds(pl.multiple_of(start, align or size), size)


def _dot(a, b):
    return jnp.dot(a, b, preferred_element_type=F32)


def _dot_nt(a, b):
    return jax.lax.dot_general(a, b, NT, preferred_element_type=F32)


def _run(order, **stages):
    for step in order.replace(" ", ""):
        next(stages[step])
    for stage in stages.values():
        for _ in stage:
            pass


def _pacer(step):
    clock = []

    def after(v):
        if not clock:
            return v
        always = jax.lax.broadcasted_iota(I32, v.shape, 1) < step + 128
        return jnp.where(always, v, jnp.tile(clock[-1], (v.shape[0] // 8, 1)))

    return clock, after


def _sort_rows(v, sizes):
    sub = jax.lax.broadcasted_iota(I32, v.shape, 0)
    for k in sizes:
        j = k // 2
        while j:
            w = jnp.take_along_axis(v, sub ^ j, axis=0)
            v = jnp.where(((sub & j) == 0) == ((sub & k) == 0),
                          jnp.maximum(v, w), jnp.minimum(v, w))
            j //= 2
    return v


def _merge_top(a, b):
    sub = jax.lax.broadcasted_iota(I32, a.shape, 0)
    return _sort_rows(jnp.maximum(a, jnp.take_along_axis(b, 7 - sub, axis=0)), (8,))


def _write_tables(tab_v, edge_v):
    sub = jax.lax.broadcasted_iota(I32, (8, 128), 0)
    lane = jax.lax.broadcasted_iota(I32, (8, 128), 1)
    ang = (((4 * lane + 1) << sub) & (4 * BLK - 1)).astype(F32) * (np.pi / (2 * BLK))
    bits = jnp.cos(ang), jnp.sin(ang)
    known = {1 << s: [jnp.broadcast_to(v[s:s + 1], (8, 128)) for v in bits] for s in range(8)}
    known[0] = [jnp.ones((8, 128), F32), jnp.zeros((8, 128), F32)]

    def times_i(z, n):
        for _ in range(n % 4):
            z = (-z[1], z[0])
        return z

    def power(t):
        if t >= BLK:
            return times_i(power(t - BLK), 1)
        if t not in known:
            low = t & -t if t & (t - 1) else t // 2
            known[t] = _cmul(power(t - low), power(low))
        return known[t]

    def put(cond, z, base):
        return [jnp.where(cond, v, w) for v, w in zip(z, base)]

    def lag_sum(ts, s):
        terms = [times_i(power(t), s * t) for t in ts]
        return [sum(z[c] for z in terms) for c in range(2)]

    def ramp(step):
        z = put((sub & 1) == 1, power(step), known[0])
        for b in (2, 4):
            z = _cmul(z, put((sub & b) == b, power(b * step), known[0]))
        return z

    def store(t, col, tiles):
        for c in range(2):
            tab_v[t, :, _tile(col + c)] = jnp.concatenate(
                [z[c] for z in tiles], axis=0).astype(BF16)

    ramp1, ramp8 = ramp(1), ramp(8)
    for p in range(4):
        q, z = (sub - p) & 3, known[0]
        for n in (1, 2, 3):
            z = put(q == n, power(127 * n), z)
        z = [_cmul(ramp1, z)]
        for _ in range(16):
            z.append(_cmul(z[-1], power(8)))
        store(0, 2 * p, [put(sub < q, z[16], z[0])] + z[1:16])

    lag_exp = _round_to_bf16(np.arange(L)).astype(np.int64)
    c = np.arange(128)
    gc, gd, g4, go, g2 = [
        np.concatenate([Q_PAIRS[v][e] + 8 * np.arange(32) for e in range(2) for v in vs])
        for vs in GROUPS]
    g1 = np.where((c >= 63) & (c < 127), g4, np.roll(go, 63))
    g3, ge = np.where(c < 64, go, g4), np.where(c == 127, gc, gd)
    ramps = {}

    def ramp_from(t):
        if t not in ramps:
            ramps[t] = (_cmul(ramps[t - 64], power(64)) if t - 64 in ramps
                        else _cmul(ramp8, power(t)))
        return ramps[t]

    def lags(e, m, phase=None):
        ts = [int(l) - BLK * m for l in np.nonzero(lag_exp == e)[0] if 0 < l - BLK * m <= BLK]
        return [t for t in ts if phase is None or t % 4 == phase]

    def rows(tss, s):
        z, runs = [known[0][1]] * 2, [[]] * 8
        if tss[0]:
            half = [len(ts) // 2 for ts in tss[:2]]
            t = tss[0][half[0]]
            runs = [list(range(t + 8 * r - half[r % 2], t + 8 * r + half[r % 2] + 1))
                    for r in range(8)]
            z = ramp_from(t)
            if any(half):
                assert t % 4 == 0
                even, odd = [1.0 + 2.0 * lag_sum(range(1, h + 1), s)[0] for h in half]
                z = [v * jnp.where((sub & 1) == 1, odd, even) for v in z]
        for r, ts in enumerate(tss):
            if ts != runs[r]:
                z = put(sub == r, lag_sum(ts, s), z)
        return z

    for p, g in enumerate((g4, g1, g2, g3)):
        store(1, 2 * p, [rows([lags(e, 0, p) for e in es], 0) for es in g.reshape(16, 8)])
    for m, g in ((1, gc), (2, ge), (3, gd)):
        for s in range(4):
            store(1 + m, 2 * s, [rows([lags(e, m) for e in es], s) for es in g.reshape(16, 8)])
    for s in range(4):
        edge_v[:, _tile(2 * s, 2)] = jnp.tile(
            jnp.concatenate(lag_sum(lags(BLK, 1), s), axis=1), (CB // 8, 1))


def _ssm_powers(par, dt):
    a_re, a_im, b_re, b_im, c_re, c_im = par
    mag = jnp.exp(dt * a_re)
    ang = dt * a_im
    pw = {1: (mag * jnp.cos(ang), mag * jnp.sin(ang))}
    for k in range(9):
        pw[2 << k] = _csq(pw[1 << k])
    sc = dt * (2.0 / BLK)
    w = _cmul((c_re, c_im), (b_re * sc, b_im * sc))
    w1, w2 = _cmul(w, pw[1]), _cmul(w, pw[2])
    return [pw[8], pw[16], pw[2], pw[4], pw[512],
            w1, _cmul(w1, pw[2]), w2, _cmul(w2, pw[256])], w[0]


def _ssm_products(pw):
    a8, a16, a2, a4, a512, w1, w3, w2, w258 = pw
    sub = jax.lax.broadcasted_iota(I32, (8, 128), 0)
    lane = jax.lax.broadcasted_iota(I32, (8, 128), 1)
    lo = sub < 4

    def pick(z, rows):
        return [jnp.take_along_axis(v, rows, axis=0) for v in z]

    def pair(x, y, h):
        r = [pltpu.roll(v, 4, 0) for v in y]
        return [jnp.where(lo, s, v) if h else jnp.where(lo, v, s) for v, s in zip(x, r)]

    out = []
    for h in range(2):
        p_rows, q_rows = 4 * h + ((sub + 2 * h) & 3), 4 * h + (sub & 3)
        step, s2, s512 = pick(a16, p_rows), pick(a2, q_rows), pick(a512, q_rows)
        p = [[jnp.where(lo, one, v) for one, v in zip((1.0, 0.0), pick(a8, p_rows))]]
        for _ in range(15):
            p.append(_cmul(p[-1], step))
        q = [pair(w3, w1, h)]
        q += [_cmul(q[0], pick(a4, q_rows)), pair(w2, w258, h)]
        for _ in range(3):
            q.append(_cmul(q[-1], s2))
        q += [_cmul(q[3], s512), _cmul(q[5], s512)]
        for _ in range(2):
            q.append(_cmul(q[-1], s512))
        out.append([_dot_nt(*[jnp.concatenate([z[j] for z in zs], axis=0).astype(BF16)
                              for zs in (q, p)]) for j in range(2)])
    first = ((lane - sub) & 3) == 0
    return [jnp.where(first, out[0][0][v:v + 8], out[1][0][v:v + 8])
            - jnp.where(first, out[0][1][v:v + 8], out[1][1][v:v + 8]) for v in range(0, 80, 8)]


def _compute(x_hbm, are_hbm, aim_hbm, bre_hbm, bim_hbm, cre_hbm, cim_hbm, ldt_hbm, dsk_hbm, wr_hbm,
            wg_hbm, wu_hbm, wd_hbm, o_hbm,
            x_v, par_v, ldt_v, dsk_v, wr_v, wg_v, wu_v, wd_v, tab_v, edge_v, o_v,
            xn_v, ph_v, kf_v, uf_v, z_v, y_v, pw_v, dt_v, k0_v, k512_v, skip_v, raw_v, vec_v,
            hot_v, xs_v, h_v, yr_v, yt_v, out_sem, sem):
    def rows(i):
        return _ds(i * CB, CB)

    x_v, wg_v, wu_v, wd_v, tab_v, xn_v, ph_v = [
        v.bitcast(BF16) for v in (x_v, wg_v, wu_v, wd_v, tab_v, xn_v, ph_v)]

    pars = (are_hbm, aim_hbm, bre_hbm, bim_hbm, cre_hbm, cim_hbm)
    cp_dt = pltpu.make_async_copy(ldt_hbm, ldt_v, sem.at[0])
    cp_head, cp_rest = [
        [pltpu.make_async_copy(p.at[r], par_v.at[j, r], sem.at[k]) for j, p in enumerate(pars)]
        for k, r in ((1, pl.ds(0, 2 * CB)), (4, pl.ds(2 * CB, D - 2 * CB)))]
    cp_x = [pltpu.make_async_copy(s, d, sem.at[2])
            for s, d in ((x_hbm, x_v), (dsk_hbm, dsk_v), (wr_hbm, wr_v))]

    def cp_w(i):
        c = _ds(i * WG * FB, WG * FB)
        return [pltpu.make_async_copy(s.at[:, c], d.at[:, c], sem.at[5 + i])
                for s, d in ((wg_hbm, wg_v), (wu_hbm, wu_v))]

    def cp_d(i):
        cuts = (0, (HOLD + 2) * CB, D - LAST, D)
        r = pl.ds(cuts[i], cuts[i + 1] - cuts[i])
        return [pltpu.make_async_copy(wd_hbm.at[r, pl.ds(c, F // DC)], wd_v.at[r, pl.ds(c, F // DC)],
                                      sem.at[5 + NCB // WG + i]) for c in range(0, F, F // DC)]

    def wait_d(i):
        for c in cp_d(i):
            c.wait()

    for c in [cp_dt] + cp_head + cp_rest + cp_x:
        c.start()

    def table(t, lo, n):
        return tab_v[t, :, _tile(lo, n)]

    raw_v[...] = jnp.zeros(raw_v.shape, F32)
    vec_v[...] = jnp.zeros(vec_v.shape, VT)
    _write_tables(tab_v, edge_v)

    cp_dt.wait()
    dt_row = _rb(jnp.exp(ldt_v[...].astype(F32).reshape(1, D)))
    dt_v[...] = jnp.broadcast_to(dt_row, (128, D)).T
    for c in cp_head:
        c.wait()

    def kernel_powers(i, after):
        par = [par_v[t, rows(i), :].astype(F32) for t in range(6)]
        k0 = []
        for g in range(0, CB, PN):
            pw, w = _ssm_powers([v[g:g + PN] for v in par], after(dt_v[_ds(i * CB + g, PN), :]))
            pw_v[g:g + PN, :] = jnp.concatenate([v for z in pw for v in z], axis=1)
            k0_v[_ds(i * CB + g, PN), :] = jnp.broadcast_to(
                jnp.sum(w, axis=1, keepdims=True), (PN, 128))
            yield

    def kernel_values(pw, clock):
        for g in range(0, CB, 8):
            out = _ssm_products([(pw[g:g + 8, _tile(2 * t)], pw[g:g + 8, _tile(2 * t + 1)])
                                 for t in range(9)])
            for v in range(10):
                raw_v[v, g:g + 8, :] = out[v]
            clock.append(out[0])
            yield

    def kernel_vectors(i, raw):
        sub = jax.lax.broadcasted_iota(I32, (8, 128), 0)
        lane = jax.lax.broadcasted_iota(I32, (8, 128), 1)
        odd = ((lane - sub) & 1) == 1
        own = ((lane - sub) & 2) == ((sub & 4) >> 1)
        perm = (4 * (lane & 31) + ((sub + ((sub & 4) >> 1)) & 3) + (lane >> 5)) & 127
        u = [jnp.where(odd, pltpu.roll(raw[v1, g:g + 8], 1, 1), raw[v0, g:g + 8])
             for v0, v1 in GROUPS for g in range(0, CB, 8)]
        u = [jnp.where(own, v, pltpu.roll(pltpu.roll(v, 4, 0), 2, 1)) for v in u]
        u = [jnp.take_along_axis(v, perm, axis=1) for v in u]
        gc, gd, g4, go, g2 = [u[t:t + CB // 8] for t in range(0, len(u), CB // 8)]
        mid, last = (lane >= 63) & (lane < 127), lane == 127
        g1 = [jnp.where(mid, a, pltpu.roll(b, 63, 1)) for a, b in zip(g4, go)]
        g3 = [jnp.where(lane < 64, b, a) for a, b in zip(g4, go)]
        ge = [jnp.where(last, a, b) for a, b in zip(gc, gd)]
        for t, v in enumerate((g4, g1, g2, g3, gc, ge, gd)):
            vec_v[t] = jnp.concatenate(v, axis=0).astype(VT)
        k512_v[rows(i), :] = jnp.broadcast_to(jnp.sum(
            jnp.concatenate([jnp.where(last, a, 0.0) for a in g4], axis=0),
            axis=1, keepdims=True), (CB, 128))
        yield

    def kernel_spectrum(i, vec, clock):
        for m in (1, 3, 2):
            for t in (0, 4):
                f = _dot(vec[3 + m].astype(BF16), table(1 + m, t, 4))
                kf_v[rows(i), _tile(8 * m + t, 4)] = f
                clock.append(f[0:8, 0:128])
                yield
        for p in range(2):
            a, b = [_dot(vec[t].astype(BF16), table(1, 2 * t, 2)) for t in (p, p + 2)]
            kf_v[rows(i), _tile(4 * p, 2)] = a + b
            kf_v[rows(i), _tile(4 * p + 2, 2)] = a - b
            clock.append(a[0:8, 0:128])
            yield

    _run("", p=kernel_powers(0, lambda v: v))
    for j in range(NCB // WG):
        for c in cp_w(j):
            c.start()
    for j in range(3):
        for c in cp_d(j):
            c.start()

    @pl.loop(0, NCB)
    def _(i):
        @pl.when(i == 1)
        def _():
            for c in cp_rest:
                c.wait()

        clock, after = _pacer(i)
        _run(K_ORDER, s=kernel_spectrum(jnp.maximum(i - 2, 0), vec_v[...], clock),
             c=kernel_vectors(jnp.maximum(i - 1, 0), raw_v[...]),
             v=kernel_values(pw_v[...], clock),
             p=kernel_powers(jnp.minimum(i + 1, NCB - 1), after))

    for c in cp_x:
        c.wait()
    skip_v[...] = jnp.broadcast_to(dsk_v[...].astype(F32).reshape(1, D), (128, D)).T
    wr = jnp.broadcast_to(wr_v[...].astype(F32).reshape(1, D), (TOPC, D)).astype(BF16)
    eps = float(_round_to_bf16(1e-5))
    mean, score = [], []

    def token_mean():
        for t in range(0, L // 128, LT):
            m = _dot(jnp.ones((8, D), BF16), x_v[:, _tile(t, LT)]) * (1.0 / D)
            mean.extend(m[:, _tile(j)] for j in range(LT))
            yield

    def split_phases(i, ms=range(4)):
        r = rows(i)
        for m in ms:
            v = [pltpu.bitcast(xn_v[r, _tile(4 * m + q)], U32) for q in range(4)]
            v = _lane_exchange([w if q == 0 else pltpu.roll(w, q, 1) for q, w in enumerate(v)])
            for p in range(4):
                ph_v[r, _tile(4 * m + p)] = pltpu.bitcast(v[p], BF16)

    def center():
        for t in range(L // 128):
            mb, sq, cen = _rb(mean[t]), [0.0, 0.0], []
            for r in range(0, D, 16):
                x = x_v[r:r + 16, _tile(t)].astype(F32)
                d = [x[0:8] - mb, x[8:16] - mb]
                sq = [a + v * v for a, v in zip(sq, d)]
                cen.append(jnp.concatenate(d, axis=1).astype(BF16))
            var = (jnp.sum(sq[0] + sq[1], axis=0, keepdims=True) * (1.0 / D)
                   - jnp.square(mean[t] - mb))
            yield cen, 0.5 / _rb(jnp.sqrt(_rb(_rb(jnp.maximum(var, 0.0)) + eps)))

    def normalize():
        tiles = center()
        for t in range(0, L // 128, NT_):
            out = jnp.concatenate([
                jnp.concatenate([d.astype(F32)[:, _tile(j)] * inv for d in cen for j in range(2)],
                                axis=0)
                for cen, inv in [next(tiles) for _ in range(NT_)]], axis=1).astype(BF16)
            xn_v[:, _tile(t, NT_)] = out
            for i in range(EARLY):
                split_phases(i, [t // 4])
            score.append(_rb(2.0 * _dot(wr, out)))
            yield

    _run(L_ORDER, s=kernel_spectrum(NCB - 2, vec_v[...], []), c=kernel_vectors(NCB - 1, raw_v),
         t=kernel_spectrum(NCB - 1, vec_v, []), m=token_mean(), n=normalize())
    score = jnp.concatenate(score, axis=1)

    def forward(i, clock):
        for h in range(0, CB, 32):
            for p in range(2):
                a, b = [_dot(
                    jnp.concatenate([ph_v[_ds(i * CB + g, 16), _tile(4 * m + t)]
                                     for g in (h, h + 16) for m in range(4)], axis=0),
                    table(0, 2 * t, 2)) for t in (p, p + 2)]
                uf_v[4 * h:4 * h + 128, _tile(4 * p, 2)] = a + b
                uf_v[4 * h:4 * h + 128, _tile(4 * p + 2, 2)] = a - b
                for r in range(0, 128, 16):
                    clock.append(a[r:r + 8, 0:128])
                    yield

    def multiply(i, uf, after):
        def pair(src, r, t):
            return src[r, _tile(t)], src[r, _tile(t + 1)]

        for g in range(0, CB, 8):
            r = _ds(i * CB + g, 8)
            ru = [slice(64 * (g // 16) + 16 * m + g % 16, 64 * (g // 16) + 16 * m + g % 16 + 8)
                  for m in range(4)]
            for s, ops in enumerate(((_cadd, _csub), (_add_i, _sub_i))):
                ks, us = [], []
                for t, op in zip((s, s + 2), ops):
                    k = [op(pair(kf_v, r, 2 * s), pair(kf_v, r, 2 * s + 4))]
                    k += [pair(kf_v, r, 8 * m + 2 * t) for m in (1, 2, 3)]
                    k[1] = [v + k512_v[r, :] * edge_v[g:g + 8, _tile(2 * t + c)]
                            for c, v in enumerate(k[1])]
                    k = [k[0]] + [_sub_i(k[m], k[m - 1]) for m in (1, 2, 3)]
                    ks.append([(c, d - c, c + d) if M3 else (c, d) for c, d in k])
                    u = [op(pair(uf, v, 2 * s), pair(uf, v, 2 * s + 4)) for v in ru]
                    us.append([(a + b, a, b) if M3 else (a, b) for a, b in u])
                for n in range(4):
                    z = []
                    for k, u in zip(ks, us):
                        if not M3:
                            acc = _cmul(k[0], u[n] if z else (after(u[n][0]), u[n][1]))
                            for m in range(1, n + 1):
                                acc = _cadd(acc, _cmul(k[m], u[n - m]))
                            z.append(acc)
                            continue
                        acc = [v * w for v, w in zip(k[0], u[n])]
                        if not z:
                            acc[0] = after(acc[0])
                        for m in range(1, n + 1):
                            acc = [a + v * w for a, v, w in zip(acc, k[m], u[n - m])]
                        z.append((acc[0] - acc[2], acc[0] + acc[1]))
                    for t, v in enumerate(_cadd(*z) + _csub(*z)):
                        z_v[pl.ds(4 * g + 8 * n, 8), _tile(4 * s + t)] = v
                    yield

    def inverse(i, z, clock, n=32):
        for h in range(0, CB, n):
            for p, ops in enumerate(((_cadd, _csub), (_sub_i, _add_i))):
                a, c = [[z[4 * h:4 * h + 4 * n, _tile(4 * s + 2 * p + t)] for t in range(2)]
                        for s in range(2)]
                y = [_dot_nt(jnp.concatenate(op(a, c), axis=1).astype(BF16),
                             table(0, 2 * p + 4 * t, 2)) for t, op in enumerate(ops)]
                for g in range(0, n, 8):
                    for m in range(4):
                        for t in range(2):
                            y_v[_ds(i * CB + h + g, 8), _tile(4 * m + p + 2 * t)] = (
                                y[t][4 * g + 8 * m:4 * g + 8 * m + 8])
                for r in range(0, 4 * n, 16):
                    clock.append(y[0][r:r + 8])
                    yield

    bits = pltpu.bitcast(jnp.where(score == 0.0, 0.0, score), I32) >> 16
    pos = jax.lax.broadcasted_iota(I32, (TOPC, L), 1)
    key = ((bits ^ ((bits >> 15) & 0x7FFF)) << 11) + (0x38000000 + L - 1 - pos)
    key = pltpu.bitcast(key, F32)
    sub = jax.lax.broadcasted_iota(I32, (TOPC, 128), 0)
    dense = []
    for t0 in (0, 8):
        v = key[:, _tile(t0)]
        for t in range(1, 8):
            v = jnp.where(sub == t, key[:, _tile(t0 + t)], v)
        dense.append(v)
    _run("", f=forward(0, []))
    top = _merge_top(*[_sort_rows(v, (2, 4, 8)) for v in dense])
    for step, count in ((8, 16), (1, 8)):
        top = [top] + [pltpu.roll(top, step * k, 1) for k in range(1, count)]
        while len(top) > 1:
            top = [_merge_top(a, b) for a, b in zip(top[0::2], top[1::2])]
        top = top[0]
        for i in range(*{8: (EARLY, MID), 1: (MID, NCB)}[step]):
            split_phases(i)
    hot_v[...] = jnp.where(key == jnp.tile(top, (1, L // 128)), 1.0, 0.0)
    top = pltpu.bitcast(top, I32) - 0x38000000
    tb = top >> 11
    gate = _rb(jax.nn.sigmoid(pltpu.bitcast((tb ^ ((tb >> 15) & 0x7FFF)) << 16, F32)))
    tok = (L - 1) - (top & (L - 1))
    pick = (tok & 127) == jax.lax.broadcasted_iota(I32, (TOPC, 128), 1)
    xs_v[...] = xs = _dot_nt(
        jnp.concatenate([jnp.where(pick & (sub == c), 2.0, 0.0) for c in range(TOPC)],
                        axis=1).astype(BF16),
        jnp.concatenate([xn_v[:, _ds(tok[c, 0] & (L - 128), 128)] for c in range(TOPC)], axis=1))

    z_v[...] = jnp.tile(xs[:, 0:128], (4 * CB // TOPC, 8))

    def ffn_up(i):
        acc = [0.0, 0.0]
        for j in range(0, D, 128):
            n = min(128, D - j)
            for t, w in enumerate((wg_v, wu_v)):
                acc[t] = acc[t] + _dot(
                    xs_v[:, j:j + n].astype(BF16),
                    w[j:j + n, _ds(i * FB, FB)])
                yield
        h_v[:, _ds(i * FB, FB)] = _rb(_silu(_rb(acc[0]))) * _rb(acc[1])

    @pl.loop(0, NCB)
    def _(i):
        for j in range(NCB // WG):
            @pl.when(i == j * WG)
            def _():
                for c in cp_w(j):
                    c.wait()

        clock, after = _pacer(i)
        _run(C_ORDER.replace('I', 'im' * 8).replace('F', 'fm' * 8).replace('J', 'imimimim' * 2 + 'm').replace('G', 'fmfmmfmfmm' * 2).replace('E', 'fmfmmfmm' * 2 + 'fmfm').replace('H', 'f' * 8), i=inverse(jnp.maximum(i - 1, 0), z_v[...], clock),
             m=multiply(i, uf_v[...], after), u=ffn_up(i),
             f=forward(jnp.minimum(i + 1, NCB - 1), clock))

    def ffn_down(i):
        y = 0.0
        for j in range(0, F, FB):
            y = y + _dot_nt(h_v[:, j:j + FB].astype(BF16),
                            wd_v[rows(i), j:j + FB])
            if j + FB == F:
                yr_v[...] = 0.5 * _rb(_rb(y) * gate[:, :DB])
            yield

    def finish(i, yt):
        for g in range(0, DB, 32):
            r = _ds(i * CB + g, 32)
            skip = 2.0 * skip_v[r, :] + BLK * k0_v[r, :]
            for m in range(4):
                upd = _dot(yt[g:g + 32].astype(BF16), hot_v[:, _tile(4 * m, 4)].astype(BF16))
                y = _lane_exchange([y_v[r, _tile(4 * m + p)] for p in range(4)])
                y = [v if q == 0 else pltpu.roll(v, 128 - q, 1) for q, v in enumerate(y)]
                for q in (0, 2):
                    out = []
                    for t in (q, q + 1):
                        x, xn = [w[r, _tile(4 * m + t)].astype(F32)
                                 for w in (x_v, xn_v)]
                        h = xn + upd[:, _tile(t)]
                        out.append(x + (y[t] + xn * skip) * (h + h * jnp.tanh(h)))
                    o_v[r, _tile(4 * m + q, 2)] = jnp.concatenate(out, axis=1).astype(BF16)
                yield

    wait_d(0)
    def first_down():
        yield from ffn_down(0)
        yt_v[...] = yr_v[...].T
        yield from ffn_down(1)

    def send(row, n, prio=0):
        r = _ds(row, n)
        pltpu.make_async_copy(o_v.at[r], o_hbm.at[r], out_sem).start(priority=prio)

    _run("", d=first_down())

    @pl.loop(0, NCB - 2)
    def _(i):
        @pl.when(i == HOLD)
        def _():
            wait_d(1)
            send(0, HOLD * CB, PR[0])

        pl.when(i + 2 == (D - LAST) // CB)(lambda: wait_d(2))
        yt = yt_v[...]
        yt_v[...] = yr_v[...].T
        _run(D_ORDER, o=finish(i, yt), d=ffn_down(i + 2))
        pl.when(i >= HOLD)(lambda: send(i * CB, CB))

    _run(P_ORDER.replace("I", "i" * (PI // 4)), o=finish(NCB - 2, yt_v[...]),
         i=inverse(NCB - 1, z_v, [], PI))
    send(D - 2 * CB, CB, PR[1])
    last = finish(NCB - 1, yr_v[...].T)
    for row in (D - CB, D - CB // 2):
        for _ in range(4):
            next(last)
        send(row, CB // 2, PR[2] * (row // 32 % 2))


def _kernel(*refs):
    pl.run_scoped(lambda sem: _compute(*refs, sem), pltpu.SemaphoreType.DMA((8 + NCB // WG,)))
    pltpu.make_async_copy(refs[24], refs[13], refs[-1]).wait()


@jax.jit
def pallas_recurrent_scan__ssm_conv_s4__moe_arch_mod__prompt_kernel(
    A_u: jax.Array,
    A_A_re: jax.Array,
    A_A_im: jax.Array,
    A_B_re: jax.Array,
    A_B_im: jax.Array,
    A_C_re: jax.Array,
    A_C_im: jax.Array,
    A_log_dt: jax.Array,
    A_Dskip: jax.Array,
    B_x: jax.Array,
    B_w_r: jax.Array,
    B_w_gate: jax.Array,
    B_w_up: jax.Array,
    B_w_down: jax.Array,
):
    del B_x
    assert A_u.shape == (1, L, D) and A_A_re.shape == (D, N) and B_w_gate.shape == (D, F)
    hbm = pl.BlockSpec(memory_space=pl.ANY)
    vmem = pltpu.VMEM
    out = pl.pallas_call(
        _kernel,
        out_shape=jax.ShapeDtypeStruct((D, L), BF16),
        in_specs=[hbm] * 13,
        out_specs=hbm,
        scratch_shapes=[
            vmem((D // 2, L), U32), vmem((6, D, N), BF16),
            vmem((D,), BF16), vmem((D,), BF16), vmem((D,), BF16),
            vmem((D // 2, F), U32), vmem((D // 2, F), U32), vmem((D // 2, F), U32),
            vmem((5, 64, 1024), U32), vmem((CB, 1024), F32), vmem((D, L), BF16),
            vmem((D // 2, L), U32), vmem((D // 2, L), U32),
            vmem((D, 4096), F32), vmem((4 * CB, 1024), F32), vmem((4 * CB, 1024), F32),
            vmem((D, L), F32), vmem((CB, 18 * 128), F32),
            *[vmem((D, 128), F32)] * 4,
            vmem((10, CB, 128), F32), vmem((7, CB, 128), VT),
            vmem((TOPC, L), F32), vmem((TOPC, D), F32), vmem((TOPC, F), F32),
            vmem((TOPC, DB), F32), vmem((DB, TOPC), F32),
            pltpu.SemaphoreType.DMA(()),
        ],
        compiler_params=pltpu.CompilerParams(vmem_limit_bytes=100 * 1024 * 1024),
    )(A_u[0].T, A_A_re, A_A_im, A_B_re, A_B_im, A_C_re, A_C_im, A_log_dt, A_Dskip, B_w_r,
      B_w_gate, B_w_up, B_w_down.T)
    return out.T[None]
```

```python
import jax
import jax.numpy as jnp
import numpy as np
import jax.experimental.pallas as pl
import jax.experimental.pallas.tpu as pltpu

F32, BF16, I32, U32 = jnp.float32, jnp.bfloat16, jnp.int32, jnp.uint32

L, D, N, F = 2048, 576, 128, 4608
TOPC = 8
BLK = 512
CB = 64
NCB = D // CB
FB = F // NCB
HOLD = 3
DOWN_CUTS = (0, (HOLD + 2) * CB, D - 48, D)

Q_PAIRS = ((3, 1), (7, 5), (2, 258), (4, 260), (6, 262), (8, 264),
           (516, 772), (520, 776), (1032, 1288), (1544, 1800))
GROUPS = ((6, 7), (8, 9), (3, 5), (0, 1), (2, 4))

SSM_FIRST = "vvpvpvpvppvppvpv"
SSM_SECOND = "cvvpvpvpvppvppvpv"
SSM_STEADY = "cssvspvpvsspvppvvpssvpspv"
SSM_LAST = "cssvsvsvsvsvsvsvv"
NORM_ORDER = "cmssmnsssmsstsntmnttntttt"
CONV_FIRST = "mmmm" + "wmmm" * 10 + "fmfmm" * 10
CONV_STEADY = ("mimimiimiimmimimuimimimiimimimimimumimiimimimmimimuimimimimimimimmimu"
               "fmfmmffmmmfmmfmfmfmuufmfmfmfmmfmmfmmfmfmufmfmfmffmffmmfmfmuuuffffffmf")
CONV_LAST = "w" * 10 + ("imm" * 8 + "dddddd") * 3 + "imm" * 8
OUT_STEADY = "ododododododododd"
OUT_LAST = ("oo" + "i" * 8) * 3 + "o" + "i" * 8


def _round_to_bf16(v):
    u = np.asarray(v, np.float32).view(np.uint32)
    return ((u + 0x7FFF + ((u >> 16) & 1)) & 0xFFFF0000).astype(np.uint32).view(np.float32)


def _cmul(a, b):
    return a[0] * b[0] - a[1] * b[1], a[0] * b[1] + a[1] * b[0]


def _csq(a):
    return (a[0] + a[1]) * (a[0] - a[1]), (a[0] + a[0]) * a[1]


def _cadd(a, b):
    return a[0] + b[0], a[1] + b[1]


def _csub(a, b):
    return a[0] - b[0], a[1] - b[1]


def _add_i(a, b):
    return a[0] - b[1], a[1] + b[0]


def _sub_i(a, b):
    return a[0] + b[1], a[1] - b[0]


def _rb(v):
    return v.astype(BF16).astype(F32)


def _silu_of_double(h):
    return h + h * jnp.tanh(h)


def _iotas(shape=(8, 128)):
    return [jax.lax.broadcasted_iota(I32, shape, axis) for axis in range(2)]


def _tile(t, n=1):
    return slice(128 * t, 128 * (t + n))


def _ds(start, size):
    return pl.ds(start if isinstance(start, int) else pl.multiple_of(start, size), size)


def _dot(a, b):
    return jnp.dot(a, b, preferred_element_type=F32)


def _dot_nt(a, b):
    return jax.lax.dot_general(a, b, (((1,), (1,)), ((), ())), preferred_element_type=F32)


def _lane_exchange(r):
    lane = _iotas(r[0].shape)[1]
    a = [jnp.where((lane & 1) == 1, r[(j + 1) % 4], r[j]) for j in range(4)]
    b = [jnp.where((lane & 2) == 2, a[(j + 2) % 4], a[j]) for j in range(4)]
    return [b[-j % 4] for j in range(4)]


def _run(order, **stages):
    for step in order:
        next(stages[step])
    for stage in stages.values():
        for _ in stage:
            pass


def _pipeline(plans, wait, stages):
    @pl.loop(0, NCB)
    def _(i):
        wait(i)
        for first, last, order in plans:
            @pl.when((i >= first) & (i <= last))
            def _():
                _run(order, **{k: make() for k, make in stages(i).items() if k in order})


def _pacer(step):
    clock = []

    def after(v):
        if not clock:
            return v
        return jnp.where(_iotas()[1] < step + 128, v, clock[-1])

    return clock, after


def _sort_rows(v, sizes):
    sub = _iotas()[0]
    for k in sizes:
        j = k // 2
        while j:
            w = jnp.take_along_axis(v, sub ^ j, axis=0)
            v = jnp.where(((sub & j) == 0) == ((sub & k) == 0),
                          jnp.maximum(v, w), jnp.minimum(v, w))
            j //= 2
    return v


def _merge_top(a, b):
    return _sort_rows(jnp.maximum(a, jnp.take_along_axis(b, 7 - _iotas()[0], axis=0)), (8,))


def _write_tables(tab_v, edge_v):
    sub, lane = _iotas()
    ang = (((4 * lane + 1) << sub) & (4 * BLK - 1)).astype(F32) * (np.pi / (2 * BLK))
    bits = jnp.cos(ang), jnp.sin(ang)
    known = {1 << s: [jnp.broadcast_to(v[s:s + 1], (8, 128)) for v in bits] for s in range(8)}
    known[0] = [jnp.ones((8, 128), F32), jnp.zeros((8, 128), F32)]

    def times_i(z, n):
        for _ in range(n % 4):
            z = (-z[1], z[0])
        return z

    def power(t):
        if t >= BLK:
            return times_i(power(t - BLK), 1)
        if t not in known:
            low = t & -t if t & (t - 1) else t // 2
            known[t] = _cmul(power(t - low), power(low))
        return known[t]

    def put(cond, z, base):
        return [jnp.where(cond, v, w) for v, w in zip(z, base)]

    def lag_sum(ts, s):
        terms = [times_i(power(t), s * t) for t in ts]
        return [sum(z[c] for z in terms) for c in range(2)]

    def ramp(step):
        z = put((sub & 1) == 1, power(step), known[0])
        for b in (2, 4):
            z = _cmul(z, put((sub & b) == b, power(b * step), known[0]))
        return z

    def store(t, col, tiles):
        for c in range(2):
            tab_v[_tile(t), _tile(col + c)] = jnp.concatenate(
                [z[c] for z in tiles], axis=0).astype(BF16)

    ramp1, ramp8 = ramp(1), ramp(8)
    for p in range(4):
        q, z = (sub - p) & 3, known[0]
        for n in (1, 2, 3):
            z = put(q == n, power(127 * n), z)
        z = [_cmul(ramp1, z)]
        for _ in range(16):
            z.append(_cmul(z[-1], power(8)))
        store(0, 2 * p, [put(sub < q, z[16], z[0])] + z[1:16])

    lag_exp = _round_to_bf16(np.arange(L)).astype(np.int64)
    c = np.arange(128)
    gc, gd, g4, go, g2 = [
        np.concatenate([Q_PAIRS[v][e] + 8 * np.arange(32) for e in range(2) for v in vs])
        for vs in GROUPS]
    g1 = np.where((c >= 63) & (c < 127), g4, np.roll(go, 63))
    g3, ge = np.where(c < 64, go, g4), np.where(c == 127, gc, gd)
    ramps, covered = {}, []

    def ramp_from(t):
        if t not in ramps:
            ramps[t] = (_cmul(ramps[t - 64], power(64)) if t - 64 in ramps
                        else _cmul(ramp8, power(t)))
        return ramps[t]

    def lags(e, m, phase=None):
        ts = [int(l) - BLK * m for l in np.nonzero(lag_exp == e)[0] if 0 < l - BLK * m <= BLK]
        ts = [t for t in ts if phase is None or t % 4 == phase]
        covered.extend(BLK * m + t for t in ts)
        return ts

    def rows(tss, s):
        z, runs = [known[0][1]] * 2, [[]] * 8
        if tss[0]:
            half = [len(ts) // 2 for ts in tss[:2]]
            t = tss[0][half[0]]
            runs = [list(range(t + 8 * r - half[r % 2], t + 8 * r + half[r % 2] + 1))
                    for r in range(8)]
            z = ramp_from(t)
            if any(half):
                assert t % 4 == 0
                even, odd = [1.0 + 2.0 * lag_sum(range(1, h + 1), s)[0] for h in half]
                z = [v * jnp.where((sub & 1) == 1, odd, even) for v in z]
        for r, ts in enumerate(tss):
            if ts != runs[r]:
                z = put(sub == r, lag_sum(ts, s), z)
        return z

    for p, g in enumerate((g4, g1, g2, g3)):
        store(1, 2 * p, [rows([lags(e, 0, p) for e in es], 0) for es in g.reshape(16, 8)])
    for m, g in ((1, gc), (2, ge), (3, gd)):
        tiles = [[lags(e, m) for e in es] for es in g.reshape(16, 8)]
        for s in range(4):
            store(1 + m, 2 * s, [rows(tss, s) for tss in tiles])
    ts = lags(BLK, 1)
    for s in range(4):
        edge_v[:, _tile(2 * s, 2)] = jnp.tile(jnp.concatenate(lag_sum(ts, s), axis=1), (CB // 8, 1))
    assert sorted(covered) == list(range(1, L))


def _ssm_powers(par, dt):
    a_re, a_im, b_re, b_im, c_re, c_im = par
    mag = jnp.exp(dt * a_re)
    ang = dt * a_im
    pw = {1: (mag * jnp.cos(ang), mag * jnp.sin(ang))}
    for k in range(9):
        pw[2 << k] = _csq(pw[1 << k])
    sc = dt * (2.0 / BLK)
    w = _cmul((c_re, c_im), (b_re * sc, b_im * sc))
    w1, w2 = _cmul(w, pw[1]), _cmul(w, pw[2])
    return [pw[8], pw[16], pw[2], pw[4], pw[512],
            w1, _cmul(w1, pw[2]), w2, _cmul(w2, pw[256])], w[0]


def _ssm_products(pw):
    a8, a16, a2, a4, a512, w1, w3, w2, w258 = pw
    sub, lane = _iotas()
    lo = sub < 4

    def pick(z, rows):
        return [jnp.take_along_axis(v, rows, axis=0) for v in z]

    def pair(x, y, h):
        r = [pltpu.roll(v, 4, 0) for v in y]
        return [jnp.where(lo, s, v) if h else jnp.where(lo, v, s) for v, s in zip(x, r)]

    out = []
    for h in range(2):
        p_rows, q_rows = 4 * h + ((sub + 2 * h) & 3), 4 * h + (sub & 3)
        step, s2, s512 = pick(a16, p_rows), pick(a2, q_rows), pick(a512, q_rows)
        p = [[jnp.where(lo, one, v) for one, v in zip((1.0, 0.0), pick(a8, p_rows))]]
        for _ in range(15):
            p.append(_cmul(p[-1], step))
        q = [pair(w3, w1, h)]
        q += [_cmul(q[0], pick(a4, q_rows)), pair(w2, w258, h)]
        for _ in range(3):
            q.append(_cmul(q[-1], s2))
        q += [_cmul(q[3], s512), _cmul(q[5], s512)]
        for _ in range(2):
            q.append(_cmul(q[-1], s512))
        out.append([_dot_nt(*[jnp.concatenate([z[j] for z in zs], axis=0).astype(BF16)
                              for zs in (q, p)]) for j in range(2)])
    first = ((lane - sub) & 3) == 0
    return [jnp.where(first, out[0][0][v:v + 8], out[1][0][v:v + 8])
            - jnp.where(first, out[0][1][v:v + 8], out[1][1][v:v + 8]) for v in range(0, 80, 8)]


def _compute(o_hbm, o_v, out_sem, sem,
             x_hbm, are_hbm, aim_hbm, bre_hbm, bim_hbm, cre_hbm, cim_hbm, ldt_hbm, dsk_hbm,
             wr_hbm, wg_hbm, wu_hbm, wd_hbm,
             x_v, xn_v, ph_v, wg_v, wu_v, wd_v, tab_v, par_v, ldt_v, dsk_v, wr_v,
             dt_v, k0_v, k512_v, skip_v, edge_v, pw_v, raw_v, vec_v, kf_v, uf_v, z_v, y_v,
             hot_v, xs_v, h_v, yr_v, yt_v):
    x_v, xn_v, ph_v, wg_v, wu_v, wd_v, tab_v = [
        v.bitcast(BF16) for v in (x_v, xn_v, ph_v, wg_v, wu_v, wd_v, tab_v)]

    def rows(i):
        return _ds(i * CB, CB)

    def table(t, lo, n):
        return tab_v[_tile(t), _tile(lo, n)]

    def lanes_to_rows(v):
        return jnp.broadcast_to(v, (128, D)).T

    def copies(k, pairs):
        return [pltpu.make_async_copy(s, d, sem.at[k]) for s, d in pairs]

    def wait(group):
        for c in group:
            c.wait()

    pars = (are_hbm, aim_hbm, bre_hbm, bim_hbm, cre_hbm, cim_hbm)
    thirds = [pl.ds(c, F // 3) for c in range(0, F, F // 3)]
    cp_dt = copies(0, [(ldt_hbm, ldt_v)])
    cp_par = [copies(1 + k, [(p.at[r], par_v.at[j, r]) for j, p in enumerate(pars)])
              for k, r in enumerate((pl.ds(0, 2 * CB), pl.ds(2 * CB, D - 2 * CB)))]
    cp_x = copies(3, [(x_hbm, x_v), (dsk_hbm, dsk_v), (wr_hbm, wr_v)])
    cp_up = [copies(4 + k, [(wg_hbm.at[:, c], wg_v.at[:, c]), (wu_hbm.at[:, c], wu_v.at[:, c])])
             for k, c in enumerate(thirds)]
    cp_down = [copies(7 + k, [(wd_hbm.at[pl.ds(a, b - a), c], wd_v.at[pl.ds(a, b - a), c])
                              for c in thirds])
               for k, (a, b) in enumerate(zip(DOWN_CUTS, DOWN_CUTS[1:]))]
    for c in cp_dt + cp_par[0] + cp_par[1] + cp_x:
        c.start()

    _write_tables(tab_v, edge_v)
    wait(cp_dt)
    dt_v[...] = lanes_to_rows(_rb(jnp.exp(ldt_v[...].astype(F32).reshape(1, D))))
    wait(cp_par[0])

    def ssm_powers(i, after):
        par = [par_v[t, rows(i), :].astype(F32) for t in range(6)]
        for g in range(0, CB, 8):
            r = _ds(i * CB + g, 8)
            pw, w = _ssm_powers([v[g:g + 8] for v in par], after(dt_v[r, :]))
            pw_v[g:g + 8, :] = jnp.concatenate([v for z in pw for v in z], axis=1)
            k0_v[r, :] = jnp.broadcast_to(jnp.sum(w, axis=1, keepdims=True), (8, 128))
            yield

    def ssm_values(pw, clock):
        for g in range(0, CB, 8):
            out = _ssm_products([(pw[g:g + 8, _tile(2 * t)], pw[g:g + 8, _tile(2 * t + 1)])
                                 for t in range(9)])
            for v in range(10):
                raw_v[v, g:g + 8, :] = out[v]
            clock.append(out[0])
            yield

    def ssm_vectors(i, raw):
        sub, lane = _iotas()
        odd = ((lane - sub) & 1) == 1
        own = ((lane - sub) & 2) == ((sub & 4) >> 1)
        perm = (4 * (lane & 31) + ((sub + ((sub & 4) >> 1)) & 3) + (lane >> 5)) & 127
        u = [jnp.where(odd, pltpu.roll(raw[v1, g:g + 8], 1, 1), raw[v0, g:g + 8])
             for v0, v1 in GROUPS for g in range(0, CB, 8)]
        u = [jnp.where(own, v, pltpu.roll(pltpu.roll(v, 4, 0), 2, 1)) for v in u]
        u = [jnp.take_along_axis(v, perm, axis=1) for v in u]
        gc, gd, g4, go, g2 = [u[t:t + CB // 8] for t in range(0, len(u), CB // 8)]
        mid, last = (lane >= 63) & (lane < 127), lane == 127
        g1 = [jnp.where(mid, a, pltpu.roll(b, 63, 1)) for a, b in zip(g4, go)]
        g3 = [jnp.where(lane < 64, b, a) for a, b in zip(g4, go)]
        ge = [jnp.where(last, a, b) for a, b in zip(gc, gd)]
        for t, v in enumerate((g4, g1, g2, g3, gc, ge, gd)):
            vec_v[t] = jnp.concatenate(v, axis=0)
        k512_v[rows(i), :] = jnp.broadcast_to(jnp.sum(
            jnp.concatenate([jnp.where(last, a, 0.0) for a in g4], axis=0),
            axis=1, keepdims=True), (CB, 128))
        yield

    def ssm_spectrum(i, vec, clock):
        for m in (1, 3, 2):
            for t in (0, 4):
                f = _dot(vec[3 + m].astype(BF16), table(1 + m, t, 4))
                kf_v[rows(i), _tile(8 * m + t, 4)] = f
                clock.append(f[0:8, 0:128])
                yield
        for p in range(2):
            a, b = [_dot(vec[t].astype(BF16), table(1, 2 * t, 2)) for t in (p, p + 2)]
            kf_v[rows(i), _tile(4 * p, 2)] = a + b
            kf_v[rows(i), _tile(4 * p + 2, 2)] = a - b
            clock.append(a[0:8, 0:128])
            yield

    def ssm_stages(i):
        clock, after = _pacer(i)
        return dict(s=lambda: ssm_spectrum(jnp.maximum(i - 2, 0), vec_v[...], clock),
                    c=lambda: ssm_vectors(jnp.maximum(i - 1, 0), raw_v[...]),
                    v=lambda: ssm_values(pw_v[...], clock),
                    p=lambda: ssm_powers(jnp.minimum(i + 1, NCB - 1), after))

    _run("", p=ssm_powers(0, lambda v: v))
    for group in cp_up + cp_down:
        for c in group:
            c.start()
    _pipeline(((0, 0, SSM_FIRST), (1, 1, SSM_SECOND), (2, NCB - 2, SSM_STEADY),
               (NCB - 1, NCB - 1, SSM_LAST)),
              lambda i: pl.when(i == 1)(lambda: wait(cp_par[1])), ssm_stages)

    wait(cp_x)
    skip_v[...] = lanes_to_rows(dsk_v[...].astype(F32).reshape(1, D))
    wr = jnp.broadcast_to(wr_v[...].astype(F32).reshape(1, D), (TOPC, D)).astype(BF16)
    eps = float(_round_to_bf16(1e-5))
    mean, score = [], []

    def token_mean():
        for m in range(4):
            v = _dot(jnp.ones((8, D), BF16), x_v[:, _tile(4 * m, 4)]) * (1.0 / D)
            mean.extend(v[:, _tile(q)] for q in range(4))
            yield

    def center(t):
        mb, sq, cen = _rb(mean[t]), [0.0, 0.0], []
        for r in range(0, D, 16):
            x = x_v[r:r + 16, _tile(t)].astype(F32)
            d = [x[0:8] - mb, x[8:16] - mb]
            sq = [a + v * v for a, v in zip(sq, d)]
            cen.append(jnp.concatenate(d, axis=1).astype(BF16))
        var = jnp.sum(sq[0] + sq[1], axis=0, keepdims=True) * (1.0 / D) - jnp.square(mean[t] - mb)
        return cen, 0.5 / _rb(jnp.sqrt(_rb(_rb(jnp.maximum(var, 0.0)) + eps)))

    def split_phases(i, m):
        v = [pltpu.bitcast(xn_v[rows(i), _tile(4 * m + q)], U32) for q in range(4)]
        v = _lane_exchange([w if q == 0 else pltpu.roll(w, q, 1) for q, w in enumerate(v)])
        for p in range(4):
            ph_v[rows(i), _tile(4 * m + p)] = pltpu.bitcast(v[p], BF16)

    def normalize():
        for m in range(4):
            out = jnp.concatenate([
                jnp.concatenate([d.astype(F32)[:, _tile(j)] * inv for d in cen for j in range(2)],
                                axis=0)
                for cen, inv in [center(4 * m + q) for q in range(4)]], axis=1).astype(BF16)
            xn_v[:, _tile(4 * m, 4)] = out
            for i in range(4):
                split_phases(i, m)
            score.append(_rb(2.0 * _dot(wr, out)))
            yield

    _run(NORM_ORDER, s=ssm_spectrum(NCB - 2, vec_v[...], []), c=ssm_vectors(NCB - 1, raw_v),
         t=ssm_spectrum(NCB - 1, vec_v, []), m=token_mean(), n=normalize())
    score = jnp.concatenate(score, axis=1)

    def forward(i, clock):
        for h in range(0, CB, 32):
            for p in range(2):
                a, b = [_dot(jnp.concatenate([ph_v[_ds(i * CB + g, 16), _tile(4 * m + t)]
                                              for g in (h, h + 16) for m in range(4)], axis=0),
                             table(0, 2 * t, 2)) for t in (p, p + 2)]
                uf_v[4 * h:4 * h + 128, _tile(4 * p, 2)] = a + b
                uf_v[4 * h:4 * h + 128, _tile(4 * p + 2, 2)] = a - b
                for r in range(0, 128, 16):
                    clock.append(a[r:r + 8, 0:128])
                    yield

    def multiply(i, uf, after):
        def pair(src, r, t):
            return src[r, _tile(t)], src[r, _tile(t + 1)]

        for g in range(0, CB, 8):
            r = _ds(i * CB + g, 8)
            ru = [64 * (g // 16) + 16 * m + g % 16 for m in range(4)]
            for s, ops in enumerate(((_cadd, _csub), (_add_i, _sub_i))):
                ks, us = [], []
                for t, op in zip((s, s + 2), ops):
                    k = [op(pair(kf_v, r, 2 * s), pair(kf_v, r, 2 * s + 4))]
                    k += [pair(kf_v, r, 8 * m + 2 * t) for m in (1, 2, 3)]
                    k[1] = [v + k512_v[r, :] * edge_v[g:g + 8, _tile(2 * t + c)]
                            for c, v in enumerate(k[1])]
                    k = [k[0]] + [_sub_i(k[m], k[m - 1]) for m in (1, 2, 3)]
                    ks.append([(c, d - c, c + d) for c, d in k])
                    u = [op(pair(uf, slice(v, v + 8), 2 * s), pair(uf, slice(v, v + 8), 2 * s + 4))
                         for v in ru]
                    us.append([(a + b, a, b) for a, b in u])
                for n in range(4):
                    z = []
                    for k, u in zip(ks, us):
                        acc = [v * w for v, w in zip(k[0], u[n])]
                        if not z:
                            acc[0] = after(acc[0])
                        for m in range(1, n + 1):
                            acc = [a + v * w for a, v, w in zip(acc, k[m], u[n - m])]
                        z.append((acc[0] - acc[2], acc[0] + acc[1]))
                    for t, v in enumerate(_cadd(*z) + _csub(*z)):
                        z_v[pl.ds(4 * g + 8 * n, 8), _tile(4 * s + t)] = v
                    yield

    def inverse(i, z, clock):
        for h in range(0, CB, 32):
            for p, ops in enumerate(((_cadd, _csub), (_sub_i, _add_i))):
                a, c = [[z[4 * h:4 * h + 128, _tile(4 * s + 2 * p + t)] for t in range(2)]
                        for s in range(2)]
                y = [_dot_nt(jnp.concatenate(op(a, c), axis=1).astype(BF16),
                             table(0, 2 * p + 4 * t, 2)) for t, op in enumerate(ops)]
                for g in range(0, 32, 8):
                    for m in range(4):
                        for t in range(2):
                            y_v[_ds(i * CB + h + g, 8), _tile(4 * m + p + 2 * t)] = (
                                y[t][4 * g + 8 * m:4 * g + 8 * m + 8])
                for r in range(0, 128, 16):
                    clock.append(y[0][r:r + 8])
                    yield

    sub, lane = _iotas()
    bits = pltpu.bitcast(jnp.where(score == 0.0, 0.0, score), I32) >> 16
    key = ((bits ^ ((bits >> 15) & 0x7FFF)) << 11) + (0x38000000 + L - 1 - _iotas((TOPC, L))[1])
    key = pltpu.bitcast(key, F32)
    dense = []
    for t0 in (0, 8):
        v = key[:, _tile(t0)]
        for t in range(1, 8):
            v = jnp.where(sub == t, key[:, _tile(t0 + t)], v)
        dense.append(v)
    _run("", f=forward(0, []))
    top = _merge_top(*[_sort_rows(v, (2, 4, 8)) for v in dense])
    for step, count, blocks in ((8, 16, range(4, 5)), (1, 8, range(5, NCB))):
        top = [top] + [pltpu.roll(top, step * k, 1) for k in range(1, count)]
        while len(top) > 1:
            top = [_merge_top(a, b) for a, b in zip(top[0::2], top[1::2])]
        top = top[0]
        for i in blocks:
            for m in range(4):
                split_phases(i, m)
    hot_v[...] = jnp.where(key == jnp.tile(top, (1, L // 128)), 1.0, 0.0)
    top = pltpu.bitcast(top, I32) - 0x38000000
    bits = top >> 11
    gate = _rb(jax.nn.sigmoid(pltpu.bitcast((bits ^ ((bits >> 15) & 0x7FFF)) << 16, F32)))
    tok = (L - 1) - (top & (L - 1))
    xs_v[...] = _dot_nt(
        jnp.concatenate([jnp.where(((tok & 127) == lane) & (sub == c), 2.0, 0.0)
                         for c in range(TOPC)], axis=1).astype(BF16),
        jnp.concatenate([xn_v[:, _ds(tok[c, 0] & (L - 128), 128)] for c in range(TOPC)], axis=1))

    def ffn_up(i, clock):
        acc = [0.0, 0.0]
        for j in range(0, D, 128):
            n = min(128, D - j)
            for t, w in enumerate((wg_v, wu_v)):
                acc[t] = acc[t] + _dot(xs_v[:, j:j + n].astype(BF16), w[j:j + n, _ds(i * FB, FB)])
                clock.append(acc[t][:, 0:128])
                if t and j + n == D:
                    h_v[:, _ds(i * FB, FB)] = _rb(_silu_of_double(0.5 * _rb(acc[0]))) * _rb(acc[1])
                yield

    def ffn_down(i):
        y = 0.0
        for j in range(0, F, FB):
            y = y + _dot_nt(h_v[:, j:j + FB].astype(BF16), wd_v[rows(i), j:j + FB])
            if j + FB == F:
                yr_v[...] = 0.5 * _rb(_rb(y) * gate[:, :CB])
            yield

    def first_down():
        yield from ffn_down(0)
        yt_v[...] = yr_v[...].T
        yield from ffn_down(1)

    def conv_wait(i):
        for k in range(3):
            pl.when(i == k * NCB // 3)(lambda: wait(cp_up[k]))
        pl.when(i == NCB - 1)(lambda: wait(cp_down[0]))

    def conv_stages(i):
        clock, after = _pacer(i)
        return dict(i=lambda: inverse(jnp.maximum(i - 1, 0), z_v[...], clock),
                    m=lambda: multiply(i, uf_v[...], after),
                    u=lambda: ffn_up(i, []), w=lambda: ffn_up(i, clock),
                    f=lambda: forward(jnp.minimum(i + 1, NCB - 1), clock), d=first_down)

    _pipeline(((0, 0, CONV_FIRST), (1, NCB - 2, CONV_STEADY), (NCB - 1, NCB - 1, CONV_LAST)),
              conv_wait, conv_stages)

    def finish(i, yt):
        for g in range(0, CB, 32):
            r = _ds(i * CB + g, 32)
            skip = 2.0 * skip_v[r, :] + BLK * k0_v[r, :]
            for m in range(4):
                upd = _dot(yt[g:g + 32].astype(BF16), hot_v[:, _tile(4 * m, 4)].astype(BF16))
                y = _lane_exchange([y_v[r, _tile(4 * m + p)] for p in range(4)])
                y = [v if q == 0 else pltpu.roll(v, 128 - q, 1) for q, v in enumerate(y)]
                for q in (0, 2):
                    out = []
                    for t in (q, q + 1):
                        x, xn = [w[r, _tile(4 * m + t)].astype(F32) for w in (x_v, xn_v)]
                        out.append(x + (y[t] + xn * skip) * _silu_of_double(xn + upd[:, _tile(t)]))
                    o_v[r, _tile(4 * m + q, 2)] = jnp.concatenate(out, axis=1).astype(BF16)
                yield

    def send(row, n):
        pltpu.make_async_copy(o_v.at[_ds(row, n)], o_hbm.at[_ds(row, n)], out_sem).start()

    @pl.loop(0, NCB - 2)
    def _(i):
        @pl.when(i == HOLD)
        def _():
            wait(cp_down[1])
            send(0, HOLD * CB)

        pl.when(i + 2 == DOWN_CUTS[2] // CB)(lambda: wait(cp_down[2]))
        yt = yt_v[...]
        yt_v[...] = yr_v[...].T
        _run(OUT_STEADY, o=finish(i, yt), d=ffn_down(i + 2))
        pl.when(i >= HOLD)(lambda: send(i * CB, CB))

    _run(OUT_LAST, o=finish(NCB - 2, yt_v[...]), i=inverse(NCB - 1, z_v, []))
    send(D - 2 * CB, CB)
    last = finish(NCB - 1, yr_v[...].T)
    for row in (D - CB, D - CB // 2):
        for _ in range(4):
            next(last)
        send(row, CB // 2)


def _kernel(*refs):
    inputs, (o_hbm, o_v, out_sem), scratch = refs[:13], refs[13:16], refs[16:]
    pl.run_scoped(lambda sem: _compute(o_hbm, o_v, out_sem, sem, *inputs, *scratch),
                  pltpu.SemaphoreType.DMA((10,)))
    pltpu.make_async_copy(o_v, o_hbm, out_sem).wait()


@jax.jit
def pallas_recurrent_scan__ssm_conv_s4__moe_arch_mod__prompt_kernel(
    A_u: jax.Array,
    A_A_re: jax.Array,
    A_A_im: jax.Array,
    A_B_re: jax.Array,
    A_B_im: jax.Array,
    A_C_re: jax.Array,
    A_C_im: jax.Array,
    A_log_dt: jax.Array,
    A_Dskip: jax.Array,
    B_x: jax.Array,
    B_w_r: jax.Array,
    B_w_gate: jax.Array,
    B_w_up: jax.Array,
    B_w_down: jax.Array,
):
    del B_x
    assert A_u.shape == (1, L, D) and A_A_re.shape == (D, N) and B_w_gate.shape == (D, F)
    assert A_u.dtype == A_A_re.dtype == BF16
    hbm = pl.BlockSpec(memory_space=pl.ANY)
    vmem = pltpu.VMEM
    out = pl.pallas_call(
        _kernel,
        out_shape=jax.ShapeDtypeStruct((D, L), BF16),
        in_specs=[hbm] * 13,
        out_specs=hbm,
        scratch_shapes=[
            vmem((D, L), BF16), pltpu.SemaphoreType.DMA(()),
            *[vmem((D // 2, L), U32)] * 3, *[vmem((D // 2, F), U32)] * 3, vmem((5 * 64, 1024), U32),
            vmem((6, D, N), BF16), *[vmem((D,), BF16)] * 3, *[vmem((D, 128), F32)] * 4,
            vmem((CB, 1024), F32), vmem((CB, 18 * 128), F32),
            vmem((10, CB, 128), F32), vmem((7, CB, 128), F32), vmem((D, 4096), F32),
            vmem((4 * CB, 1024), F32), vmem((4 * CB, 1024), F32), vmem((D, L), F32),
            vmem((TOPC, L), F32), vmem((TOPC, D), F32), vmem((TOPC, F), F32),
            vmem((TOPC, CB), F32), vmem((CB, TOPC), F32),
        ],
        compiler_params=pltpu.CompilerParams(vmem_limit_bytes=100 * 1024 * 1024),
    )(A_u[0].T, A_A_re, A_A_im, A_B_re, A_B_im, A_C_re, A_C_im, A_log_dt, A_Dskip, B_w_r,
      B_w_gate, B_w_up, B_w_down.T)
    return out.T[None]
```

```python
import jax
import jax.numpy as jnp
import numpy as np
import jax.experimental.pallas as pl
import jax.experimental.pallas.tpu as pltpu

F32, BF16, I32, U32 = jnp.float32, jnp.bfloat16, jnp.int32, jnp.uint32

L, D, N, F = 2048, 576, 128, 4608
TOPC = 8
BLK = 512
CB = 64
NCB = D // CB
FB = F // NCB
HOLD = 3
DOWN_CUTS = (0, (HOLD + 2) * CB, D - 32, D)

Q_PAIRS = ((3, 1), (7, 5), (2, 258), (4, 260), (6, 262), (8, 264),
           (516, 772), (520, 776), (1032, 1288), (1544, 1800))
GROUPS = ((6, 7), (8, 9), (3, 5), (0, 1), (2, 4))

SSM_FIRST = "vpvvpvvpvppvpvpp"
SSM_SECOND = "cpvvvpvpvvpvppvpp"
SSM_STEADY = "cssvpvspvsspvppvvpssvpspv"
SSM_LAST = "cssvvssvvssvvssvv"
NORM_ORDER = "cmssmnsssmsstsntmntttnttt"
CONV_FIRST = ("mmmmmwmwmmmwmmmmmmwmmwmmmwmmmmmmwwmmwmmmwmm"
              "fmffmfmmfmffmmfmmmmfmmffmmfmfmmfmmfmmmmmfmfmmfffmfmfmffffffffff")
CONV_STEADY = ("mimimiimiimmimimuimimimiimimimimimumimiimimimmimimuimmimimimimimmimmu"
               "fimfmmffmmfmmfmfmfuufmmfmmfmfmfmmfmmfmfmufmfmfmffmffmmfmfmuuuffffffmf")
CONV_LAST = ("mwwmwwwwwwwwmmimmiimimmimmiimmimmdmddddmmdmimmimmimimimmiimmimm"
             "ddddmddimmimmimmimmimmmmidmimimdddddmmmimmmimimmimimmimmimmmi")
OUT_STEADY = "odoododododododdd"
OUT_LAST = "ooiiiiiiiioiioiiiiiiooiiiiioiioiiiiiiiii"


def _round_to_bf16(v):
    u = np.asarray(v, np.float32).view(np.uint32)
    return ((u + 0x7FFF + ((u >> 16) & 1)) & 0xFFFF0000).astype(np.uint32).view(np.float32)


def _cmul(a, b):
    return a[0] * b[0] - a[1] * b[1], a[0] * b[1] + a[1] * b[0]


def _csq(a):
    return (a[0] + a[1]) * (a[0] - a[1]), (a[0] + a[0]) * a[1]


def _cadd(a, b):
    return a[0] + b[0], a[1] + b[1]


def _csub(a, b):
    return a[0] - b[0], a[1] - b[1]


def _add_i(a, b):
    return a[0] - b[1], a[1] + b[0]


def _sub_i(a, b):
    return a[0] + b[1], a[1] - b[0]


def _rb(v):
    return v.astype(BF16).astype(F32)


def _silu_of_double(h):
    return h + h * jnp.tanh(h)


def _iotas(shape=(8, 128)):
    return [jax.lax.broadcasted_iota(I32, shape, axis) for axis in range(2)]


def _tile(t, n=1):
    return slice(128 * t, 128 * (t + n))


def _ds(start, size):
    return pl.ds(start if isinstance(start, int) else pl.multiple_of(start, size), size)


def _dot(a, b):
    return jnp.dot(a, b, preferred_element_type=F32)


def _dot_nt(a, b):
    return jax.lax.dot_general(a, b, (((1,), (1,)), ((), ())), preferred_element_type=F32)


def _lane_exchange(r):
    lane = _iotas(r[0].shape)[1]
    a = [jnp.where((lane & 1) == 1, r[(j + 1) % 4], r[j]) for j in range(4)]
    b = [jnp.where((lane & 2) == 2, a[(j + 2) % 4], a[j]) for j in range(4)]
    return [b[-j % 4] for j in range(4)]


def _run(order, **stages):
    for step in order:
        next(stages[step])
    for stage in stages.values():
        for _ in stage:
            pass


def _pipeline(plans, wait, stages):
    @pl.loop(0, NCB)
    def _(i):
        wait(i)
        for first, last, order in plans:
            @pl.when((i >= first) & (i <= last))
            def _():
                _run(order, **{k: make() for k, make in stages(i).items() if k in order})


def _pacer(step):
    clock = []

    def after(v):
        if not clock:
            return v
        return jnp.where(_iotas()[1] < step + 128, v, clock[-1])

    return clock, after


def _sort_rows(v, sizes):
    sub = _iotas()[0]
    for k in sizes:
        j = k // 2
        while j:
            w = jnp.take_along_axis(v, sub ^ j, axis=0)
            v = jnp.where(((sub & j) == 0) == ((sub & k) == 0),
                          jnp.maximum(v, w), jnp.minimum(v, w))
            j //= 2
    return v


def _merge_top(a, b):
    return _sort_rows(jnp.maximum(a, jnp.take_along_axis(b, 7 - _iotas()[0], axis=0)), (8,))


def _write_tables(tab_v, edge_v):
    sub, lane = _iotas()
    ang = (((4 * lane + 1) << sub) & (4 * BLK - 1)).astype(F32) * (np.pi / (2 * BLK))
    bits = jnp.cos(ang), jnp.sin(ang)
    known = {1 << s: [jnp.broadcast_to(v[s:s + 1], (8, 128)) for v in bits] for s in range(8)}
    known[0] = [jnp.ones((8, 128), F32), jnp.zeros((8, 128), F32)]

    def times_i(z, n):
        for _ in range(n % 4):
            z = (-z[1], z[0])
        return z

    def power(t):
        if t >= BLK:
            return times_i(power(t - BLK), 1)
        if t not in known:
            low = t & -t if t & (t - 1) else t // 2
            known[t] = _cmul(power(t - low), power(low))
        return known[t]

    def put(cond, z, base):
        return [jnp.where(cond, v, w) for v, w in zip(z, base)]

    def lag_sum(ts, s):
        terms = [times_i(power(t), s * t) for t in ts]
        return [sum(z[c] for z in terms) for c in range(2)]

    def ramp(step):
        z = put((sub & 1) == 1, power(step), known[0])
        for b in (2, 4):
            z = _cmul(z, put((sub & b) == b, power(b * step), known[0]))
        return z

    def store(t, col, tiles):
        for c in range(2):
            tab_v[_tile(t), _tile(col + c)] = jnp.concatenate(
                [z[c] for z in tiles], axis=0).astype(BF16)

    ramp1, ramp8 = ramp(1), ramp(8)
    for p in range(4):
        q, z = (sub - p) & 3, known[0]
        for n in (1, 2, 3):
            z = put(q == n, power(127 * n), z)
        z = [_cmul(ramp1, z)]
        for _ in range(16):
            z.append(_cmul(z[-1], power(8)))
        store(0, 2 * p, [put(sub < q, z[16], z[0])] + z[1:16])

    lag_exp = _round_to_bf16(np.arange(L)).astype(np.int64)
    c = np.arange(128)
    gc, gd, g4, go, g2 = [
        np.concatenate([Q_PAIRS[v][e] + 8 * np.arange(32) for e in range(2) for v in vs])
        for vs in GROUPS]
    g1 = np.where((c >= 63) & (c < 127), g4, np.roll(go, 63))
    g3, ge = np.where(c < 64, go, g4), np.where(c == 127, gc, gd)
    ramps, covered = {}, []

    def ramp_from(t):
        if t not in ramps:
            ramps[t] = (_cmul(ramps[t - 64], power(64)) if t - 64 in ramps
                        else _cmul(ramp8, power(t)))
        return ramps[t]

    def lags(e, m, phase=None):
        ts = [int(l) - BLK * m for l in np.nonzero(lag_exp == e)[0] if 0 < l - BLK * m <= BLK]
        ts = [t for t in ts if phase is None or t % 4 == phase]
        covered.extend(BLK * m + t for t in ts)
        return ts

    def rows(tss, s):
        z, runs = [known[0][1]] * 2, [[]] * 8
        if tss[0]:
            half = [len(ts) // 2 for ts in tss[:2]]
            t = tss[0][half[0]]
            runs = [list(range(t + 8 * r - half[r % 2], t + 8 * r + half[r % 2] + 1))
                    for r in range(8)]
            z = ramp_from(t)
            if any(half):
                assert t % 4 == 0
                even, odd = [1.0 + 2.0 * lag_sum(range(1, h + 1), s)[0] for h in half]
                z = [v * jnp.where((sub & 1) == 1, odd, even) for v in z]
        for r, ts in enumerate(tss):
            if ts != runs[r]:
                z = put(sub == r, lag_sum(ts, s), z)
        return z

    for p, g in enumerate((g4, g1, g2, g3)):
        store(1, 2 * p, [rows([lags(e, 0, p) for e in es], 0) for es in g.reshape(16, 8)])
    for m, g in ((1, gc), (2, ge), (3, gd)):
        tiles = [[lags(e, m) for e in es] for es in g.reshape(16, 8)]
        for s in range(4):
            store(1 + m, 2 * s, [rows(tss, s) for tss in tiles])
    ts = lags(BLK, 1)
    for s in range(4):
        edge_v[:, _tile(2 * s, 2)] = jnp.tile(jnp.concatenate(lag_sum(ts, s), axis=1), (CB // 8, 1))
    assert sorted(covered) == list(range(1, L))


def _ssm_powers(par, dt):
    a_re, a_im, b_re, b_im, c_re, c_im = par
    mag = jnp.exp(dt * a_re)
    ang = dt * a_im
    pw = {1: (mag * jnp.cos(ang), mag * jnp.sin(ang))}
    for k in range(9):
        pw[2 << k] = _csq(pw[1 << k])
    sc = dt * (2.0 / BLK)
    w = _cmul((c_re, c_im), (b_re * sc, b_im * sc))
    w1, w2 = _cmul(w, pw[1]), _cmul(w, pw[2])
    return [pw[8], pw[16], pw[2], pw[4], pw[512],
            w1, _cmul(w1, pw[2]), w2, _cmul(w2, pw[256])], w[0]


def _ssm_products(pw):
    a8, a16, a2, a4, a512, w1, w3, w2, w258 = pw
    sub, lane = _iotas()
    lo = sub < 4

    def pick(z, rows):
        return [jnp.take_along_axis(v, rows, axis=0) for v in z]

    def pair(x, y, h):
        r = [pltpu.roll(v, 4, 0) for v in y]
        return [jnp.where(lo, s, v) if h else jnp.where(lo, v, s) for v, s in zip(x, r)]

    out = []
    for h in range(2):
        p_rows, q_rows = 4 * h + ((sub + 2 * h) & 3), 4 * h + (sub & 3)
        step, s2, s512 = pick(a16, p_rows), pick(a2, q_rows), pick(a512, q_rows)
        p = [[jnp.where(lo, one, v) for one, v in zip((1.0, 0.0), pick(a8, p_rows))]]
        for _ in range(15):
            p.append(_cmul(p[-1], step))
        q = [pair(w3, w1, h)]
        q += [_cmul(q[0], pick(a4, q_rows)), pair(w2, w258, h)]
        for _ in range(3):
            q.append(_cmul(q[-1], s2))
        q += [_cmul(q[3], s512), _cmul(q[5], s512)]
        for _ in range(2):
            q.append(_cmul(q[-1], s512))
        out.append([_dot_nt(*[jnp.concatenate([z[j] for z in zs], axis=0).astype(BF16)
                              for zs in (q, p)]) for j in range(2)])
    first = ((lane - sub) & 3) == 0
    return [jnp.where(first, out[0][0][v:v + 8], out[1][0][v:v + 8])
            - jnp.where(first, out[0][1][v:v + 8], out[1][1][v:v + 8]) for v in range(0, 80, 8)]


def _compute(o_hbm, o_v, out_sem, sem,
             x_hbm, are_hbm, aim_hbm, bre_hbm, bim_hbm, cre_hbm, cim_hbm, ldt_hbm, dsk_hbm,
             wr_hbm, wg_hbm, wu_hbm, wd_hbm,
             x_v, xn_v, ph_v, wg_v, wu_v, wd_v, tab_v, par_v, ldt_v, dsk_v, wr_v,
             dt_v, k0_v, k512_v, skip_v, edge_v, pw_v, raw_v, vec_v, kf_v, uf_v, z_v, y_v,
             hot_v, xs_v, h_v, yr_v, yt_v):
    x_v, xn_v, ph_v, wg_v, wu_v, tab_v = [
        v.bitcast(BF16) for v in (x_v, xn_v, ph_v, wg_v, wu_v, tab_v)]

    def rows(i):
        return _ds(i * CB, CB)

    def table(t, lo, n):
        return tab_v[_tile(t), _tile(lo, n)]

    def lanes_to_rows(v):
        return jnp.broadcast_to(v, (128, D)).T

    def copies(k, pairs):
        return [pltpu.make_async_copy(s, d, sem.at[k]) for s, d in pairs]

    def wait(group):
        for c in group:
            c.wait()

    pars = (are_hbm, aim_hbm, bre_hbm, bim_hbm, cre_hbm, cim_hbm)
    thirds = [pl.ds(c, F // 3) for c in range(0, F, F // 3)]
    cp_dt = copies(0, [(ldt_hbm, ldt_v)])
    cp_par = [copies(1 + k, [(p.at[r], par_v.at[j, r]) for j, p in enumerate(pars)])
              for k, r in enumerate((pl.ds(0, 2 * CB), pl.ds(2 * CB, D - 2 * CB)))]
    cp_x = copies(3, [(x_hbm, x_v), (dsk_hbm, dsk_v), (wr_hbm, wr_v)])
    cp_up = [copies(4 + k, [(wg_hbm.at[:, c], wg_v.at[:, c]), (wu_hbm.at[:, c], wu_v.at[:, c])])
             for k, c in enumerate(thirds)]
    cp_down = [copies(7 + k, [(wd_hbm.at[pl.ds(a, b - a)], wd_v.at[pl.ds(a, b - a)])])
               for k, (a, b) in enumerate(zip(DOWN_CUTS, DOWN_CUTS[1:]))]
    for c in cp_dt + cp_par[0] + cp_par[1] + cp_x:
        c.start()

    _write_tables(tab_v, edge_v)
    wait(cp_dt)
    dt_v[...] = lanes_to_rows(_rb(jnp.exp(ldt_v[...].astype(F32).reshape(1, D))))
    wait(cp_par[0])

    def ssm_powers(i, after):
        par = [par_v[t, rows(i), :].astype(F32) for t in range(6)]
        for g in range(0, CB, 8):
            r = _ds(i * CB + g, 8)
            pw, w = _ssm_powers([v[g:g + 8] for v in par], after(dt_v[r, :]))
            pw_v[g:g + 8, :] = jnp.concatenate([v for z in pw for v in z], axis=1)
            k0_v[r, :] = jnp.broadcast_to(jnp.sum(w, axis=1, keepdims=True), (8, 128))
            yield

    def ssm_values(pw, clock):
        for g in range(0, CB, 8):
            out = _ssm_products([(pw[g:g + 8, _tile(2 * t)], pw[g:g + 8, _tile(2 * t + 1)])
                                 for t in range(9)])
            for v in range(10):
                raw_v[v, g:g + 8, :] = out[v]
            clock.append(out[0])
            yield

    def ssm_vectors(i, raw):
        sub, lane = _iotas()
        odd = ((lane - sub) & 1) == 1
        own = ((lane - sub) & 2) == ((sub & 4) >> 1)
        perm = (4 * (lane & 31) + ((sub + ((sub & 4) >> 1)) & 3) + (lane >> 5)) & 127
        u = [jnp.where(odd, pltpu.roll(raw[v1, g:g + 8], 1, 1), raw[v0, g:g + 8])
             for v0, v1 in GROUPS for g in range(0, CB, 8)]
        u = [jnp.where(own, v, pltpu.roll(pltpu.roll(v, 4, 0), 2, 1)) for v in u]
        u = [jnp.take_along_axis(v, perm, axis=1) for v in u]
        gc, gd, g4, go, g2 = [u[t:t + CB // 8] for t in range(0, len(u), CB // 8)]
        mid, last = (lane >= 63) & (lane < 127), lane == 127
        g1 = [jnp.where(mid, a, pltpu.roll(b, 63, 1)) for a, b in zip(g4, go)]
        g3 = [jnp.where(lane < 64, b, a) for a, b in zip(g4, go)]
        ge = [jnp.where(last, a, b) for a, b in zip(gc, gd)]
        for t, v in enumerate((g4, g1, g2, g3, gc, ge, gd)):
            vec_v[t] = jnp.concatenate(v, axis=0)
        k512_v[rows(i), :] = jnp.broadcast_to(jnp.sum(
            jnp.concatenate([jnp.where(last, a, 0.0) for a in g4], axis=0),
            axis=1, keepdims=True), (CB, 128))
        yield

    def ssm_spectrum(i, vec, clock):
        for m in (1, 3, 2):
            for t in (0, 4):
                f = _dot(vec[3 + m].astype(BF16), table(1 + m, t, 4))
                kf_v[rows(i), _tile(8 * m + t, 4)] = f
                clock.append(f[0:8, 0:128])
                yield
        for p in range(2):
            a, b = [_dot(vec[t].astype(BF16), table(1, 2 * t, 2)) for t in (p, p + 2)]
            kf_v[rows(i), _tile(4 * p, 2)] = a + b
            kf_v[rows(i), _tile(4 * p + 2, 2)] = a - b
            clock.append(a[0:8, 0:128])
            yield

    def ssm_stages(i):
        clock, after = _pacer(i)
        return dict(s=lambda: ssm_spectrum(jnp.maximum(i - 2, 0), vec_v[...], clock),
                    c=lambda: ssm_vectors(jnp.maximum(i - 1, 0), raw_v[...]),
                    v=lambda: ssm_values(pw_v[...], clock),
                    p=lambda: ssm_powers(jnp.minimum(i + 1, NCB - 1), after))

    _run("", p=ssm_powers(0, lambda v: v))
    for group in cp_up + cp_down:
        for c in group:
            c.start()
    _pipeline(((0, 0, SSM_FIRST), (1, 1, SSM_SECOND), (2, NCB - 2, SSM_STEADY),
               (NCB - 1, NCB - 1, SSM_LAST)),
              lambda i: pl.when(i == 1)(lambda: wait(cp_par[1])), ssm_stages)

    wait(cp_x)
    skip_v[...] = lanes_to_rows(dsk_v[...].astype(F32).reshape(1, D))
    wr = jnp.broadcast_to(wr_v[...].astype(F32).reshape(1, D), (TOPC, D)).astype(BF16)
    eps = float(_round_to_bf16(1e-5))
    mean, score = [], []

    def token_mean():
        for m in range(4):
            v = _dot(jnp.ones((8, D), BF16), x_v[:, _tile(4 * m, 4)]) * (1.0 / D)
            mean.extend(v[:, _tile(q)] for q in range(4))
            yield

    def center(t):
        mb, sq, cen = _rb(mean[t]), [0.0, 0.0], []
        for r in range(0, D, 16):
            x = x_v[r:r + 16, _tile(t)].astype(F32)
            d = [x[0:8] - mb, x[8:16] - mb]
            sq = [a + v * v for a, v in zip(sq, d)]
            cen.append(jnp.concatenate(d, axis=1).astype(BF16))
        var = jnp.sum(sq[0] + sq[1], axis=0, keepdims=True) * (1.0 / D) - jnp.square(mean[t] - mb)
        return cen, 0.5 / _rb(jnp.sqrt(_rb(_rb(jnp.maximum(var, 0.0)) + eps)))

    def split_phases(i, m):
        v = [pltpu.bitcast(xn_v[rows(i), _tile(4 * m + q)], U32) for q in range(4)]
        v = _lane_exchange([w if q == 0 else pltpu.roll(w, q, 1) for q, w in enumerate(v)])
        for p in range(4):
            ph_v[rows(i), _tile(4 * m + p)] = pltpu.bitcast(v[p], BF16)

    def normalize():
        for m in range(4):
            out = jnp.concatenate([
                jnp.concatenate([d.astype(F32)[:, _tile(j)] * inv for d in cen for j in range(2)],
                                axis=0)
                for cen, inv in [center(4 * m + q) for q in range(4)]], axis=1).astype(BF16)
            xn_v[:, _tile(4 * m, 4)] = out
            for i in range(4):
                split_phases(i, m)
            score.append(_rb(2.0 * _dot(wr, out)))
            yield

    _run(NORM_ORDER, s=ssm_spectrum(NCB - 2, vec_v[...], []), c=ssm_vectors(NCB - 1, raw_v),
         t=ssm_spectrum(NCB - 1, vec_v, []), m=token_mean(), n=normalize())
    score = jnp.concatenate(score, axis=1)

    def forward(i, clock):
        for h in range(0, CB, 32):
            for p in range(2):
                a, b = [_dot(jnp.concatenate([ph_v[_ds(i * CB + g, 16), _tile(4 * m + t)]
                                              for g in (h, h + 16) for m in range(4)], axis=0),
                             table(0, 2 * t, 2)) for t in (p, p + 2)]
                uf_v[4 * h:4 * h + 128, _tile(4 * p, 2)] = a + b
                uf_v[4 * h:4 * h + 128, _tile(4 * p + 2, 2)] = a - b
                for r in range(0, 128, 16):
                    clock.append(a[r:r + 8, 0:128])
                    yield

    def multiply(i, uf, after):
        def pair(src, r, t):
            return src[r, _tile(t)], src[r, _tile(t + 1)]

        for g in range(0, CB, 8):
            r = _ds(i * CB + g, 8)
            ru = [64 * (g // 16) + 16 * m + g % 16 for m in range(4)]
            for s, ops in enumerate(((_cadd, _csub), (_add_i, _sub_i))):
                ks, us = [], []
                for t, op in zip((s, s + 2), ops):
                    k = [op(pair(kf_v, r, 2 * s), pair(kf_v, r, 2 * s + 4))]
                    k += [pair(kf_v, r, 8 * m + 2 * t) for m in (1, 2, 3)]
                    k[1] = [v + k512_v[r, :] * edge_v[g:g + 8, _tile(2 * t + c)]
                            for c, v in enumerate(k[1])]
                    k = [k[0]] + [_sub_i(k[m], k[m - 1]) for m in (1, 2, 3)]
                    ks.append([(c, d - c, c + d) for c, d in k])
                    u = [op(pair(uf, slice(v, v + 8), 2 * s), pair(uf, slice(v, v + 8), 2 * s + 4))
                         for v in ru]
                    us.append([(a + b, a, b) for a, b in u])
                for n in range(4):
                    z = []
                    for k, u in zip(ks, us):
                        acc = [v * w for v, w in zip(k[0], u[n])]
                        if not z:
                            acc[0] = after(acc[0])
                        for m in range(1, n + 1):
                            acc = [a + v * w for a, v, w in zip(acc, k[m], u[n - m])]
                        z.append((acc[0] - acc[2], acc[0] + acc[1]))
                    for t, v in enumerate(_cadd(*z) + _csub(*z)):
                        z_v[pl.ds(4 * g + 8 * n, 8), _tile(4 * s + t)] = v
                    yield

    def inverse(i, z, clock):
        for h in range(0, CB, 32):
            for p, ops in enumerate(((_cadd, _csub), (_sub_i, _add_i))):
                a, c = [[z[4 * h:4 * h + 128, _tile(4 * s + 2 * p + t)] for t in range(2)]
                        for s in range(2)]
                y = [_dot_nt(jnp.concatenate(op(a, c), axis=1).astype(BF16),
                             table(0, 2 * p + 4 * t, 2)) for t, op in enumerate(ops)]
                for g in range(0, 32, 8):
                    for m in range(4):
                        for t in range(2):
                            y_v[_ds(i * CB + h + g, 8), _tile(4 * m + p + 2 * t)] = (
                                y[t][4 * g + 8 * m:4 * g + 8 * m + 8])
                for r in range(0, 128, 16):
                    clock.append(y[0][r:r + 8])
                    yield

    sub, lane = _iotas()
    bits = pltpu.bitcast(jnp.where(score == 0.0, 0.0, score), I32) >> 16
    key = ((bits ^ ((bits >> 15) & 0x7FFF)) << 11) + (0x38000000 + L - 1 - _iotas((TOPC, L))[1])
    key = pltpu.bitcast(key, F32)
    dense = []
    for t0 in (0, 8):
        v = key[:, _tile(t0)]
        for t in range(1, 8):
            v = jnp.where(sub == t, key[:, _tile(t0 + t)], v)
        dense.append(v)
    _run("", f=forward(0, []))
    top = _merge_top(*[_sort_rows(v, (2, 4, 8)) for v in dense])
    for step, count, blocks in ((8, 16, range(4, 5)), (1, 8, range(5, NCB))):
        top = [top] + [pltpu.roll(top, step * k, 1) for k in range(1, count)]
        while len(top) > 1:
            top = [_merge_top(a, b) for a, b in zip(top[0::2], top[1::2])]
        top = top[0]
        for i in blocks:
            for m in range(4):
                split_phases(i, m)
    hot_v[...] = jnp.where(key == jnp.tile(top, (1, L // 128)), 1.0, 0.0)
    top = pltpu.bitcast(top, I32) - 0x38000000
    bits = top >> 11
    gate = _rb(jax.nn.sigmoid(pltpu.bitcast((bits ^ ((bits >> 15) & 0x7FFF)) << 16, F32)))
    tok = (L - 1) - (top & (L - 1))
    xs_v[...] = _dot_nt(
        jnp.concatenate([jnp.where(((tok & 127) == lane) & (sub == c), 2.0, 0.0)
                         for c in range(TOPC)], axis=1).astype(BF16),
        jnp.concatenate([xn_v[:, _ds(tok[c, 0] & (L - 128), 128)] for c in range(TOPC)], axis=1))

    def ffn_up(i, clock):
        acc = [0.0, 0.0]
        for j in range(0, D, 128):
            n = min(128, D - j)
            for t, w in enumerate((wg_v, wu_v)):
                acc[t] = acc[t] + _dot(xs_v[:, j:j + n].astype(BF16), w[j:j + n, _ds(i * FB, FB)])
                clock.append(acc[t][:, 0:128])
                if t and j + n == D:
                    h_v[:, _ds(i * FB, FB)] = _rb(_silu_of_double(0.5 * _rb(acc[0]))) * _rb(acc[1])
                yield

    def ffn_down(i):
        y = 0.0
        for j in range(0, F, FB):
            y = y + _dot_nt(h_v[:, j:j + FB].astype(BF16), wd_v[rows(i), j:j + FB])
            if j + FB == F:
                yr_v[...] = 0.5 * _rb(_rb(y) * gate[:, :CB])
            yield

    def first_down():
        yield from ffn_down(0)
        yt_v[...] = yr_v[...].T
        yield from ffn_down(1)

    def conv_wait(i):
        for k in range(3):
            pl.when(i == k * NCB // 3)(lambda: wait(cp_up[k]))
        pl.when(i == NCB - 1)(lambda: wait(cp_down[0]))

    def conv_stages(i):
        clock, after = _pacer(i)
        return dict(i=lambda: inverse(jnp.maximum(i - 1, 0), z_v[...], clock),
                    m=lambda: multiply(i, uf_v[...], after),
                    u=lambda: ffn_up(i, []), w=lambda: ffn_up(i, clock),
                    f=lambda: forward(jnp.minimum(i + 1, NCB - 1), clock), d=first_down)

    _pipeline(((0, 0, CONV_FIRST), (1, NCB - 2, CONV_STEADY), (NCB - 1, NCB - 1, CONV_LAST)),
              conv_wait, conv_stages)

    def finish(i, yt):
        for g in range(0, CB, 32):
            r = _ds(i * CB + g, 32)
            skip = 2.0 * skip_v[r, :] + BLK * k0_v[r, :]
            for m in range(4):
                upd = _dot(yt[g:g + 32].astype(BF16), hot_v[:, _tile(4 * m, 4)].astype(BF16))
                y = _lane_exchange([y_v[r, _tile(4 * m + p)] for p in range(4)])
                y = [v if q == 0 else pltpu.roll(v, 128 - q, 1) for q, v in enumerate(y)]
                for q in (0, 2):
                    out = []
                    for t in (q, q + 1):
                        x, xn = [w[r, _tile(4 * m + t)].astype(F32) for w in (x_v, xn_v)]
                        out.append(x + (y[t] + xn * skip) * _silu_of_double(xn + upd[:, _tile(t)]))
                    o_v[r, _tile(4 * m + q, 2)] = jnp.concatenate(out, axis=1).astype(BF16)
                yield

    def send(row, n):
        for k in range(2):
            r = _ds(row + k * (n // 2), n // 2)
            pltpu.make_async_copy(o_v.at[r], o_hbm.at[r], out_sem).start(priority=k)

    @pl.loop(0, NCB - 2)
    def _(i):
        @pl.when(i == HOLD)
        def _():
            wait(cp_down[1])
            send(0, HOLD * CB)

        pl.when(i + 2 == DOWN_CUTS[2] // CB)(lambda: wait(cp_down[2]))
        yt = yt_v[...]
        yt_v[...] = yr_v[...].T
        _run(OUT_STEADY, o=finish(i, yt), d=ffn_down(i + 2))
        pl.when(i >= HOLD)(lambda: send(i * CB, CB))

    _run(OUT_LAST, o=finish(NCB - 2, yt_v[...]), i=inverse(NCB - 1, z_v, []))
    send(D - 2 * CB, CB)
    last = finish(NCB - 1, yr_v[...].T)
    for row in (D - CB, D - CB // 2):
        for _ in range(4):
            next(last)
        send(row, CB // 2)


def _kernel(*refs):
    inputs, (o_hbm, o_v, out_sem), scratch = refs[:13], refs[13:16], refs[16:]
    pl.run_scoped(lambda sem: _compute(o_hbm, o_v, out_sem, sem, *inputs, *scratch),
                  pltpu.SemaphoreType.DMA((10,)))
    pltpu.make_async_copy(o_v, o_hbm, out_sem).wait()


@jax.jit
def pallas_recurrent_scan__ssm_conv_s4__moe_arch_mod__prompt_kernel(
    A_u: jax.Array,
    A_A_re: jax.Array,
    A_A_im: jax.Array,
    A_B_re: jax.Array,
    A_B_im: jax.Array,
    A_C_re: jax.Array,
    A_C_im: jax.Array,
    A_log_dt: jax.Array,
    A_Dskip: jax.Array,
    B_x: jax.Array,
    B_w_r: jax.Array,
    B_w_gate: jax.Array,
    B_w_up: jax.Array,
    B_w_down: jax.Array,
):
    del B_x
    assert A_u.shape == (1, L, D) and A_A_re.shape == (D, N) and B_w_gate.shape == (D, F)
    assert A_u.dtype == A_A_re.dtype == BF16
    hbm = pl.BlockSpec(memory_space=pl.ANY)
    vmem = pltpu.VMEM
    out = pl.pallas_call(
        _kernel,
        out_shape=jax.ShapeDtypeStruct((D, L), BF16),
        in_specs=[hbm] * 13,
        out_specs=hbm,
        scratch_shapes=[
            vmem((D, L), BF16), pltpu.SemaphoreType.DMA(()),
            *[vmem((D // 2, L), U32)] * 3, *[vmem((D // 2, F), U32)] * 2, vmem((D, F), BF16), vmem((5 * 64, 1024), U32),
            vmem((6, D, N), BF16), *[vmem((D,), BF16)] * 3, *[vmem((D, 128), F32)] * 4,
            vmem((CB, 1024), F32), vmem((CB, 18 * 128), F32),
            vmem((10, CB, 128), F32), vmem((7, CB, 128), F32), vmem((D, 4096), F32),
            vmem((4 * CB, 1024), F32), vmem((4 * CB, 1024), F32), vmem((D, L), F32),
            vmem((TOPC, L), F32), vmem((TOPC, D), F32), vmem((TOPC, F), F32),
            vmem((TOPC, CB), F32), vmem((CB, TOPC), F32),
        ],
        compiler_params=pltpu.CompilerParams(vmem_limit_bytes=100 * 1024 * 1024),
    )(A_u[0].T, A_A_re, A_A_im, A_B_re, A_B_im, A_C_re, A_C_im, A_log_dt, A_Dskip, B_w_r,
      B_w_gate, B_w_up, B_w_down.T)
    return out.T[None]
```

```python
import jax
import jax.numpy as jnp
import numpy as np
import jax.experimental.pallas as pl
import jax.experimental.pallas.tpu as pltpu

F32, BF16, I32, U32 = jnp.float32, jnp.bfloat16, jnp.int32, jnp.uint32

L, D, N, F = 2048, 576, 128, 4608
TOPC = 8
BLK = 512
CB = 64
NCB = D // CB
FB = F // NCB
HOLD = 3
DOWN_CUTS = (0, (HOLD + 2) * CB, D - 48, D)

Q_PAIRS = ((3, 1), (7, 5), (2, 258), (4, 260), (6, 262), (8, 264),
           (516, 772), (520, 776), (1032, 1288), (1544, 1800))
GROUPS = ((6, 7), (8, 9), (3, 5), (0, 1), (2, 4))

SSM_FIRST = "vpvvpvvpvppvpvpp"
SSM_SECOND = "cpvvvpvpvvpvppvpp"
SSM_STEADY = "cssvpvspvssvpvpvpspsvpspv"
SSM_LAST = "cssvvssvvssvvssvv"
NORM_ORDER = "cmssmnsssmsstsntmntttnttt"
CONV_FIRST = ("mmmmmmwmwmmmwmmmmmmmmwmwmwmmmmmmmwwmwmmwmm"
              "fmmffmfmmfmffmmfmmmmmfmfmmffmmfmmfmmmmmmfmffmffmfmfmffmfffffffff")
CONV_STEADY = ("immimiimiimmimimuimimimiimmiimimimmuimiimimimmmimiuimmimimimimimmimmu"
               "fimfmmffmmfmmfmfmfuufmmfmmfmfmfmfmmfmfmufmfmffmfmfmfmfmfufffffmfmmfuu")
CONV_LAST = ("mwwmwwwwmwwwwmmimmiiimimmiimmmidmddmddmmmdmmimmimmimiimmimimimm"
             "ddddmddimmimimmimmmimmmmidmimimddmdddmmmimmmimimmimimimmimmmi")
OUT_STEADY = "ododododoodododdd"
OUT_LAST = "ooiiiiiiioiiiiioiiiiioooiiiioiiiiiiiiiii"


def _round_to_bf16(v):
    u = np.asarray(v, np.float32).view(np.uint32)
    return ((u + 0x7FFF + ((u >> 16) & 1)) & 0xFFFF0000).astype(np.uint32).view(np.float32)


def _cmul(a, b):
    return a[0] * b[0] - a[1] * b[1], a[0] * b[1] + a[1] * b[0]


def _csq(a):
    return (a[0] + a[1]) * (a[0] - a[1]), (a[0] + a[0]) * a[1]


def _cadd(a, b):
    return a[0] + b[0], a[1] + b[1]


def _csub(a, b):
    return a[0] - b[0], a[1] - b[1]


def _add_i(a, b):
    return a[0] - b[1], a[1] + b[0]


def _sub_i(a, b):
    return a[0] + b[1], a[1] - b[0]


def _rb(v):
    return v.astype(BF16).astype(F32)


def _silu_of_double(h):
    return h + h * jnp.tanh(h)


def _iotas(shape=(8, 128)):
    return [jax.lax.broadcasted_iota(I32, shape, axis) for axis in range(2)]


def _tile(t, n=1):
    return slice(128 * t, 128 * (t + n))


def _ds(start, size):
    return pl.ds(start if isinstance(start, int) else pl.multiple_of(start, size), size)


def _dot(a, b):
    return jnp.dot(a, b, preferred_element_type=F32)


def _dot_nt(a, b):
    return jax.lax.dot_general(a, b, (((1,), (1,)), ((), ())), preferred_element_type=F32)


def _lane_exchange(r):
    lane = _iotas(r[0].shape)[1]
    a = [jnp.where((lane & 1) == 1, r[(j + 1) % 4], r[j]) for j in range(4)]
    b = [jnp.where((lane & 2) == 2, a[(j + 2) % 4], a[j]) for j in range(4)]
    return [b[-j % 4] for j in range(4)]


def _run(order, **stages):
    for step in order:
        next(stages[step])
    for stage in stages.values():
        for _ in stage:
            pass


def _pipeline(plans, wait, stages):
    @pl.loop(0, NCB)
    def _(i):
        wait(i)
        for first, last, order in plans:
            @pl.when((i >= first) & (i <= last))
            def _():
                _run(order, **{k: make() for k, make in stages(i).items() if k in order})


def _pacer(step):
    clock = []

    def after(v):
        if not clock:
            return v
        return jnp.where(_iotas()[1] < step + 128, v, clock[-1])

    return clock, after


def _sort_rows(v, sizes):
    sub = _iotas()[0]
    for k in sizes:
        j = k // 2
        while j:
            w = jnp.take_along_axis(v, sub ^ j, axis=0)
            v = jnp.where(((sub & j) == 0) == ((sub & k) == 0),
                          jnp.maximum(v, w), jnp.minimum(v, w))
            j //= 2
    return v


def _merge_top(a, b):
    return _sort_rows(jnp.maximum(a, jnp.take_along_axis(b, 7 - _iotas()[0], axis=0)), (8,))


def _write_tables(tab_v, edge_v):
    sub, lane = _iotas()
    ang = (((4 * lane + 1) << sub) & (4 * BLK - 1)).astype(F32) * (np.pi / (2 * BLK))
    bits = jnp.cos(ang), jnp.sin(ang)
    known = {1 << s: [jnp.broadcast_to(v[s:s + 1], (8, 128)) for v in bits] for s in range(8)}
    known[0] = [jnp.ones((8, 128), F32), jnp.zeros((8, 128), F32)]

    def times_i(z, n):
        for _ in range(n % 4):
            z = (-z[1], z[0])
        return z

    def power(t):
        if t >= BLK:
            return times_i(power(t - BLK), 1)
        if t not in known:
            low = t & -t if t & (t - 1) else t // 2
            known[t] = _cmul(power(t - low), power(low))
        return known[t]

    def put(cond, z, base):
        return [jnp.where(cond, v, w) for v, w in zip(z, base)]

    def lag_sum(ts, s):
        terms = [times_i(power(t), s * t) for t in ts]
        return [sum(z[c] for z in terms) for c in range(2)]

    def ramp(step):
        z = put((sub & 1) == 1, power(step), known[0])
        for b in (2, 4):
            z = _cmul(z, put((sub & b) == b, power(b * step), known[0]))
        return z

    def store(t, col, tiles):
        for c in range(2):
            tab_v[64 * t:64 * t + 64, _tile(col + c)] = pltpu.bitcast(
                jnp.concatenate([z[c] for z in tiles], axis=0).astype(BF16), U32)

    ramp1, ramp8 = ramp(1), ramp(8)
    for p in range(4):
        q, z = (sub - p) & 3, known[0]
        for n in (1, 2, 3):
            z = put(q == n, power(127 * n), z)
        z = [_cmul(ramp1, z)]
        for _ in range(16):
            z.append(_cmul(z[-1], power(8)))
        store(0, 2 * p, [put(sub < q, z[16], z[0])] + z[1:16])

    lag_exp = _round_to_bf16(np.arange(L)).astype(np.int64)
    c = np.arange(128)
    gc, gd, g4, go, g2 = [
        np.concatenate([Q_PAIRS[v][e] + 8 * np.arange(32) for e in range(2) for v in vs])
        for vs in GROUPS]
    g1 = np.where((c >= 63) & (c < 127), g4, np.roll(go, 63))
    g3, ge = np.where(c < 64, go, g4), np.where(c == 127, gc, gd)
    ramps, covered = {}, []

    def ramp_from(t):
        if t not in ramps:
            ramps[t] = (_cmul(ramps[t - 64], power(64)) if t - 64 in ramps
                        else _cmul(ramp8, power(t)))
        return ramps[t]

    def lags(e, m, phase=None):
        ts = [int(l) - BLK * m for l in np.nonzero(lag_exp == e)[0] if 0 < l - BLK * m <= BLK]
        ts = [t for t in ts if phase is None or t % 4 == phase]
        covered.extend(BLK * m + t for t in ts)
        return ts

    def rows(tss, s):
        z, runs = [known[0][1]] * 2, [[]] * 8
        if tss[0]:
            half = [len(ts) // 2 for ts in tss[:2]]
            t = tss[0][half[0]]
            runs = [list(range(t + 8 * r - half[r % 2], t + 8 * r + half[r % 2] + 1))
                    for r in range(8)]
            z = ramp_from(t)
            if any(half):
                assert t % 4 == 0
                even, odd = [1.0 + 2.0 * lag_sum(range(1, h + 1), s)[0] for h in half]
                z = [v * jnp.where((sub & 1) == 1, odd, even) for v in z]
        for r, ts in enumerate(tss):
            if ts != runs[r]:
                z = put(sub == r, lag_sum(ts, s), z)
        return z

    for p, g in enumerate((g4, g1, g2, g3)):
        store(1, 2 * p, [rows([lags(e, 0, p) for e in es], 0) for es in g.reshape(16, 8)])
    for m, g in ((1, gc), (2, ge), (3, gd)):
        tiles = [[lags(e, m) for e in es] for es in g.reshape(16, 8)]
        for s in range(4):
            store(1 + m, 2 * s, [rows(tss, s) for tss in tiles])
    ts = lags(BLK, 1)
    for s in range(4):
        edge_v[:, _tile(2 * s, 2)] = jnp.tile(jnp.concatenate(lag_sum(ts, s), axis=1), (CB // 8, 1))
    assert sorted(covered) == list(range(1, L))


def _ssm_powers(par, dt):
    a_re, a_im, b_re, b_im, c_re, c_im = par
    mag = jnp.exp(dt * a_re)
    ang = dt * a_im
    pw = {1: (mag * jnp.cos(ang), mag * jnp.sin(ang))}
    for k in range(9):
        pw[2 << k] = _csq(pw[1 << k])
    sc = dt * (2.0 / BLK)
    w = _cmul((c_re, c_im), (b_re * sc, b_im * sc))
    w1, w2 = _cmul(w, pw[1]), _cmul(w, pw[2])
    return [pw[8], pw[16], pw[2], pw[4], pw[512],
            w1, _cmul(w1, pw[2]), w2, _cmul(w2, pw[256])], w[0]


def _ssm_products(pw):
    a8, a16, a2, a4, a512, w1, w3, w2, w258 = pw
    sub, lane = _iotas()
    lo = sub < 4

    def pick(z, rows):
        return [jnp.take_along_axis(v, rows, axis=0) for v in z]

    def pair(x, y, h):
        r = [pltpu.roll(v, 4, 0) for v in y]
        return [jnp.where(lo, s, v) if h else jnp.where(lo, v, s) for v, s in zip(x, r)]

    out = []
    for h in range(2):
        p_rows, q_rows = 4 * h + ((sub + 2 * h) & 3), 4 * h + (sub & 3)
        step, s2, s512 = pick(a16, p_rows), pick(a2, q_rows), pick(a512, q_rows)
        p = [[jnp.where(lo, one, v) for one, v in zip((1.0, 0.0), pick(a8, p_rows))]]
        for _ in range(15):
            p.append(_cmul(p[-1], step))
        q = [pair(w3, w1, h)]
        q += [_cmul(q[0], pick(a4, q_rows)), pair(w2, w258, h)]
        for _ in range(3):
            q.append(_cmul(q[-1], s2))
        q += [_cmul(q[3], s512), _cmul(q[5], s512)]
        for _ in range(2):
            q.append(_cmul(q[-1], s512))
        out.append([_dot_nt(*[jnp.concatenate([z[j] for z in zs], axis=0).astype(BF16)
                              for zs in (q, p)]) for j in range(2)])
    first = ((lane - sub) & 3) == 0
    return [jnp.where(first, out[0][0][v:v + 8], out[1][0][v:v + 8])
            - jnp.where(first, out[0][1][v:v + 8], out[1][1][v:v + 8]) for v in range(0, 80, 8)]


def _compute(o_hbm, o_v, out_sem, sem,
             x_hbm, are_hbm, aim_hbm, bre_hbm, bim_hbm, cre_hbm, cim_hbm, ldt_hbm, dsk_hbm,
             wr_hbm, wg_hbm, wu_hbm, wd_hbm,
             x_v, xn_v, ph_v, wg_v, wu_v, wd_v, tab_v, par_v, ldt_v, dsk_v, wr_v,
             dt_v, k0_v, k512_v, skip_v, edge_v, pw_v, raw_v, vec_v, kf_v, uf_v, z_v, y_v,
             hot_v, xs_v, h_v, yr_v, yt_v):
    def rows(i):
        return _ds(i * CB, CB)

    def table(t, lo, n):
        return pltpu.bitcast(tab_v[64 * t:64 * t + 64, _tile(lo, n)], BF16)

    def lanes_to_rows(v):
        return jnp.broadcast_to(v, (128, D)).T

    def copies(k, pairs):
        return [pltpu.make_async_copy(s, d, sem.at[k]) for s, d in pairs]

    def wait(group):
        for c in group:
            c.wait()

    pars = (are_hbm, aim_hbm, bre_hbm, bim_hbm, cre_hbm, cim_hbm)
    thirds = [pl.ds(c, F // 3) for c in range(0, F, F // 3)]
    cp_dt = copies(0, [(ldt_hbm, ldt_v)])
    cp_par = [copies(1 + k, [(p.at[r], par_v.at[j, r]) for j, p in enumerate(pars)])
              for k, r in enumerate((pl.ds(0, 2 * CB), pl.ds(2 * CB, D - 2 * CB)))]
    cp_x = copies(3, [(x_hbm, x_v), (dsk_hbm, dsk_v), (wr_hbm, wr_v)])
    cp_up = [copies(4 + k, [(wg_hbm.at[:, c], wg_v.at[:, c]), (wu_hbm.at[:, c], wu_v.at[:, c])])
             for k, c in enumerate(thirds)]
    cp_down = [copies(7 + k, [(wd_hbm.at[pl.ds(a, b - a)], wd_v.at[pl.ds(a, b - a)])])
               for k, (a, b) in enumerate(zip(DOWN_CUTS, DOWN_CUTS[1:]))]
    for c in cp_dt + cp_par[0] + cp_par[1] + cp_x:
        c.start()

    _write_tables(tab_v, edge_v)
    wait(cp_dt)
    dt_v[...] = lanes_to_rows(_rb(jnp.exp(ldt_v[...].astype(F32).reshape(1, D))))
    wait(cp_par[0])

    def ssm_powers(i, after):
        par = [par_v[t, rows(i), :].astype(F32) for t in range(6)]
        for g in range(0, CB, 8):
            r = _ds(i * CB + g, 8)
            pw, w = _ssm_powers([v[g:g + 8] for v in par], after(dt_v[r, :]))
            pw_v[g:g + 8, :] = jnp.concatenate([v for z in pw for v in z], axis=1)
            k0_v[r, :] = jnp.broadcast_to(jnp.sum(w, axis=1, keepdims=True), (8, 128))
            yield

    def ssm_values(pw, clock):
        for g in range(0, CB, 8):
            out = _ssm_products([(pw[g:g + 8, _tile(2 * t)], pw[g:g + 8, _tile(2 * t + 1)])
                                 for t in range(9)])
            for v in range(10):
                raw_v[v, g:g + 8, :] = out[v]
            clock.append(out[0])
            yield

    def ssm_vectors(i, raw):
        sub, lane = _iotas()
        odd = ((lane - sub) & 1) == 1
        own = ((lane - sub) & 2) == ((sub & 4) >> 1)
        perm = (4 * (lane & 31) + ((sub + ((sub & 4) >> 1)) & 3) + (lane >> 5)) & 127
        u = [jnp.where(odd, pltpu.roll(raw[v1, g:g + 8], 1, 1), raw[v0, g:g + 8])
             for v0, v1 in GROUPS for g in range(0, CB, 8)]
        u = [jnp.where(own, v, pltpu.roll(pltpu.roll(v, 4, 0), 2, 1)) for v in u]
        u = [jnp.take_along_axis(v, perm, axis=1) for v in u]
        gc, gd, g4, go, g2 = [u[t:t + CB // 8] for t in range(0, len(u), CB // 8)]
        mid, last = (lane >= 63) & (lane < 127), lane == 127
        g1 = [jnp.where(mid, a, pltpu.roll(b, 63, 1)) for a, b in zip(g4, go)]
        g3 = [jnp.where(lane < 64, b, a) for a, b in zip(g4, go)]
        ge = [jnp.where(last, a, b) for a, b in zip(gc, gd)]
        for t, v in enumerate((g4, g1, g2, g3, gc, ge, gd)):
            vec_v[t] = jnp.concatenate(v, axis=0)
        k512_v[rows(i), :] = jnp.broadcast_to(jnp.sum(
            jnp.concatenate([jnp.where(last, a, 0.0) for a in g4], axis=0),
            axis=1, keepdims=True), (CB, 128))
        yield

    def ssm_spectrum(i, vec, clock):
        for m in (1, 3, 2):
            for t in (0, 4):
                f = _dot(vec[3 + m].astype(BF16), table(1 + m, t, 4))
                kf_v[rows(i), _tile(8 * m + t, 4)] = f
                clock.append(f[0:8, 0:128])
                yield
        for p in range(2):
            a, b = [_dot(vec[t].astype(BF16), table(1, 2 * t, 2)) for t in (p, p + 2)]
            kf_v[rows(i), _tile(4 * p, 2)] = a + b
            kf_v[rows(i), _tile(4 * p + 2, 2)] = a - b
            clock.append(a[0:8, 0:128])
            yield

    def ssm_stages(i):
        clock, after = _pacer(i)
        return dict(s=lambda: ssm_spectrum(jnp.maximum(i - 2, 0), vec_v[...], clock),
                    c=lambda: ssm_vectors(jnp.maximum(i - 1, 0), raw_v[...]),
                    v=lambda: ssm_values(pw_v[...], clock),
                    p=lambda: ssm_powers(jnp.minimum(i + 1, NCB - 1), after))

    _run("", p=ssm_powers(0, lambda v: v))
    for group in cp_up + cp_down:
        for c in group:
            c.start()
    _pipeline(((0, 0, SSM_FIRST), (1, 1, SSM_SECOND), (2, NCB - 2, SSM_STEADY),
               (NCB - 1, NCB - 1, SSM_LAST)),
              lambda i: pl.when(i == 1)(lambda: wait(cp_par[1])), ssm_stages)

    wait(cp_x)
    skip_v[...] = lanes_to_rows(dsk_v[...].astype(F32).reshape(1, D))
    wr = jnp.broadcast_to(wr_v[...].astype(F32).reshape(1, D), (TOPC, D)).astype(BF16)
    eps = float(_round_to_bf16(1e-5))
    mean, score = [], []

    def token_mean():
        for m in range(4):
            v = _dot(jnp.ones((8, D), BF16), x_v[:, _tile(4 * m, 4)]) * (1.0 / D)
            mean.extend(v[:, _tile(q)] for q in range(4))
            yield

    def center(t):
        mb, sq, cen = _rb(mean[t]), [0.0, 0.0], []
        for r in range(0, D, 16):
            x = x_v[r:r + 16, _tile(t)].astype(F32)
            d = [x[0:8] - mb, x[8:16] - mb]
            sq = [a + v * v for a, v in zip(sq, d)]
            cen.append(jnp.concatenate(d, axis=1).astype(BF16))
        var = jnp.sum(sq[0] + sq[1], axis=0, keepdims=True) * (1.0 / D) - jnp.square(mean[t] - mb)
        return cen, 0.5 / _rb(jnp.sqrt(_rb(_rb(jnp.maximum(var, 0.0)) + eps)))

    def split_phases(i, m):
        r = _ds(i * CB // 2, CB // 2)
        v = [xn_v[r, _tile(4 * m + q)] for q in range(4)]
        v = _lane_exchange([w if q == 0 else pltpu.roll(w, q, 1) for q, w in enumerate(v)])
        for p in range(4):
            ph_v[r, _tile(4 * m + p)] = v[p]

    def normalize():
        for m in range(4):
            out = jnp.concatenate([
                jnp.concatenate([d.astype(F32)[:, _tile(j)] * inv for d in cen for j in range(2)],
                                axis=0)
                for cen, inv in [center(4 * m + q) for q in range(4)]], axis=1).astype(BF16)
            xn_v[:, _tile(4 * m, 4)] = pltpu.bitcast(out, U32)
            for i in range(4):
                split_phases(i, m)
            score.append(_rb(2.0 * _dot(wr, out)))
            yield

    _run(NORM_ORDER, s=ssm_spectrum(NCB - 2, vec_v[...], []), c=ssm_vectors(NCB - 1, raw_v),
         t=ssm_spectrum(NCB - 1, vec_v, []), m=token_mean(), n=normalize())
    score = jnp.concatenate(score, axis=1)

    def forward(i, clock):
        for h in range(0, CB, 32):
            for p in range(2):
                a, b = [_dot(pltpu.bitcast(jnp.concatenate(
                    [ph_v[_ds(i * (CB // 2) + g // 2, 8), _tile(4 * m + t)]
                     for g in (h, h + 16) for m in range(4)], axis=0), BF16),
                    table(0, 2 * t, 2)) for t in (p, p + 2)]
                uf_v[4 * h:4 * h + 128, _tile(4 * p, 2)] = a + b
                uf_v[4 * h:4 * h + 128, _tile(4 * p + 2, 2)] = a - b
                for r in range(0, 128, 16):
                    clock.append(a[r:r + 8, 0:128])
                    yield

    def multiply(i, uf, after):
        def pair(src, r, t):
            return src[r, _tile(t)], src[r, _tile(t + 1)]

        for g in range(0, CB, 8):
            r = _ds(i * CB + g, 8)
            ru = [64 * (g // 16) + 16 * m + g % 16 for m in range(4)]
            for s, ops in enumerate(((_cadd, _csub), (_add_i, _sub_i))):
                ks, us = [], []
                for t, op in zip((s, s + 2), ops):
                    k = [op(pair(kf_v, r, 2 * s), pair(kf_v, r, 2 * s + 4))]
                    k += [pair(kf_v, r, 8 * m + 2 * t) for m in (1, 2, 3)]
                    k[1] = [v + k512_v[r, :] * edge_v[g:g + 8, _tile(2 * t + c)]
                            for c, v in enumerate(k[1])]
                    k = [k[0]] + [_sub_i(k[m], k[m - 1]) for m in (1, 2, 3)]
                    ks.append([(c, d - c, c + d) for c, d in k])
                    u = [op(pair(uf, slice(v, v + 8), 2 * s), pair(uf, slice(v, v + 8), 2 * s + 4))
                         for v in ru]
                    us.append([(a + b, a, b) for a, b in u])
                for n in range(4):
                    z = []
                    for k, u in zip(ks, us):
                        acc = [v * w for v, w in zip(k[0], u[n])]
                        if not z:
                            acc[0] = after(acc[0])
                        for m in range(1, n + 1):
                            acc = [a + v * w for a, v, w in zip(acc, k[m], u[n - m])]
                        z.append((acc[0] - acc[2], acc[0] + acc[1]))
                    for t, v in enumerate(_cadd(*z) + _csub(*z)):
                        z_v[pl.ds(4 * g + 8 * n, 8), _tile(4 * s + t)] = v
                    yield

    def inverse(i, z, clock):
        for h in range(0, CB, 32):
            for p, ops in enumerate(((_cadd, _csub), (_sub_i, _add_i))):
                a, c = [[z[4 * h:4 * h + 128, _tile(4 * s + 2 * p + t)] for t in range(2)]
                        for s in range(2)]
                y = [_dot_nt(jnp.concatenate(op(a, c), axis=1).astype(BF16),
                             table(0, 2 * p + 4 * t, 2)) for t, op in enumerate(ops)]
                for g in range(0, 32, 8):
                    for m in range(4):
                        for t in range(2):
                            y_v[_ds(i * CB + h + g, 8), _tile(4 * m + p + 2 * t)] = (
                                y[t][4 * g + 8 * m:4 * g + 8 * m + 8])
                for r in range(0, 128, 16):
                    clock.append(y[0][r:r + 8])
                    yield

    sub, lane = _iotas()
    bits = pltpu.bitcast(jnp.where(score == 0.0, 0.0, score), I32) >> 16
    key = ((bits ^ ((bits >> 15) & 0x7FFF)) << 11) + (0x38000000 + L - 1 - _iotas((TOPC, L))[1])
    key = pltpu.bitcast(key, F32)
    dense = []
    for t0 in (0, 8):
        v = key[:, _tile(t0)]
        for t in range(1, 8):
            v = jnp.where(sub == t, key[:, _tile(t0 + t)], v)
        dense.append(v)
    _run("", f=forward(0, []))
    top = _merge_top(*[_sort_rows(v, (2, 4, 8)) for v in dense])
    for step, count, blocks in ((8, 16, range(4, 5)), (1, 8, range(5, NCB))):
        top = [top] + [pltpu.roll(top, step * k, 1) for k in range(1, count)]
        while len(top) > 1:
            top = [_merge_top(a, b) for a, b in zip(top[0::2], top[1::2])]
        top = top[0]
        for i in blocks:
            for m in range(4):
                split_phases(i, m)
    hot_v[...] = jnp.where(key == jnp.tile(top, (1, L // 128)), 1.0, 0.0)
    top = pltpu.bitcast(top, I32) - 0x38000000
    bits = top >> 11
    gate = _rb(jax.nn.sigmoid(pltpu.bitcast((bits ^ ((bits >> 15) & 0x7FFF)) << 16, F32)))
    tok = (L - 1) - (top & (L - 1))
    xs_v[...] = _dot_nt(
        jnp.concatenate([jnp.where(((tok & 127) == lane) & (sub == c), 2.0, 0.0)
                         for c in range(TOPC)], axis=1).astype(BF16),
        pltpu.bitcast(jnp.concatenate(
            [xn_v[:, _ds(tok[c, 0] & (L - 128), 128)] for c in range(TOPC)], axis=1), BF16))

    def ffn_up(i, clock):
        acc = [0.0, 0.0]
        for j in range(0, D, 128):
            n = min(128, D - j)
            for t, w in enumerate((wg_v, wu_v)):
                acc[t] = acc[t] + _dot(xs_v[:, j:j + n].astype(BF16), w[j:j + n, _ds(i * FB, FB)])
                clock.append(acc[t][:, 0:128])
                if t and j + n == D:
                    h_v[:, _ds(i * FB, FB)] = _rb(_silu_of_double(0.5 * _rb(acc[0]))) * _rb(acc[1])
                yield

    def ffn_down(i):
        y = 0.0
        for j in range(0, F, FB):
            y = y + _dot_nt(h_v[:, j:j + FB].astype(BF16), wd_v[rows(i), j:j + FB])
            if j + FB == F:
                yr_v[...] = 0.5 * _rb(_rb(y) * gate[:, :CB])
            yield

    def first_down():
        yield from ffn_down(0)
        yt_v[...] = yr_v[...].T
        yield from ffn_down(1)

    def conv_wait(i):
        for k in range(3):
            pl.when(i == k * NCB // 3)(lambda: wait(cp_up[k]))
        pl.when(i == NCB - 1)(lambda: wait(cp_down[0]))

    def conv_stages(i):
        clock, after = _pacer(i)
        return dict(i=lambda: inverse(jnp.maximum(i - 1, 0), z_v[...], clock),
                    m=lambda: multiply(i, uf_v[...], after),
                    u=lambda: ffn_up(i, []), w=lambda: ffn_up(i, clock),
                    f=lambda: forward(jnp.minimum(i + 1, NCB - 1), clock), d=first_down)

    _pipeline(((0, 0, CONV_FIRST), (1, NCB - 2, CONV_STEADY), (NCB - 1, NCB - 1, CONV_LAST)),
              conv_wait, conv_stages)

    def finish(i, yt):
        for g in range(0, CB, 32):
            r = _ds(i * CB + g, 32)
            skip = 2.0 * skip_v[r, :] + BLK * k0_v[r, :]
            for m in range(4):
                upd = _dot(yt[g:g + 32].astype(BF16), hot_v[:, _tile(4 * m, 4)].astype(BF16))
                y = _lane_exchange([y_v[r, _tile(4 * m + p)] for p in range(4)])
                y = [v if q == 0 else pltpu.roll(v, 128 - q, 1) for q, v in enumerate(y)]
                for q in (0, 2):
                    out = []
                    for t in (q, q + 1):
                        xn = pltpu.bitcast(xn_v[_ds(i * (CB // 2) + g // 2, 16), _tile(4 * m + t)],
                                           BF16).astype(F32)
                        x = x_v[r, _tile(4 * m + t)].astype(F32)
                        out.append(x + (y[t] + xn * skip) * _silu_of_double(xn + upd[:, _tile(t)]))
                    o_v[r, _tile(4 * m + q, 2)] = jnp.concatenate(out, axis=1).astype(BF16)
                yield

    def send(row, n):
        for k in range(2):
            r = _ds(row + k * (n // 2), n // 2)
            pltpu.make_async_copy(o_v.at[r], o_hbm.at[r], out_sem).start(priority=k)

    @pl.loop(0, NCB - 2)
    def _(i):
        @pl.when(i == HOLD)
        def _():
            wait(cp_down[1])
            send(0, HOLD * CB)

        pl.when(i + 2 == DOWN_CUTS[2] // CB)(lambda: wait(cp_down[2]))
        yt = yt_v[...]
        yt_v[...] = yr_v[...].T
        _run(OUT_STEADY, o=finish(i, yt), d=ffn_down(i + 2))
        pl.when(i >= HOLD)(lambda: send(i * CB, CB))

    _run(OUT_LAST, o=finish(NCB - 2, yt_v[...]), i=inverse(NCB - 1, z_v, []))
    send(D - 2 * CB, CB)
    last = finish(NCB - 1, yr_v[...].T)
    for row in (D - CB, D - CB // 2):
        for _ in range(4):
            next(last)
        send(row, CB // 2)


def _kernel(*refs):
    inputs, (o_hbm, o_v, out_sem), scratch = refs[:13], refs[13:16], refs[16:]
    pl.run_scoped(lambda sem: _compute(o_hbm, o_v, out_sem, sem, *inputs, *scratch),
                  pltpu.SemaphoreType.DMA((10,)))
    pltpu.make_async_copy(o_v, o_hbm, out_sem).wait()


@jax.jit
def pallas_recurrent_scan__ssm_conv_s4__moe_arch_mod__prompt_kernel(
    A_u: jax.Array,
    A_A_re: jax.Array,
    A_A_im: jax.Array,
    A_B_re: jax.Array,
    A_B_im: jax.Array,
    A_C_re: jax.Array,
    A_C_im: jax.Array,
    A_log_dt: jax.Array,
    A_Dskip: jax.Array,
    B_x: jax.Array,
    B_w_r: jax.Array,
    B_w_gate: jax.Array,
    B_w_up: jax.Array,
    B_w_down: jax.Array,
):
    del B_x
    assert A_u.shape == (1, L, D) and A_A_re.shape == (D, N) and B_w_gate.shape == (D, F)
    assert A_u.dtype == A_A_re.dtype == BF16
    hbm = pl.BlockSpec(memory_space=pl.ANY)
    vmem = pltpu.VMEM
    out = pl.pallas_call(
        _kernel,
        out_shape=jax.ShapeDtypeStruct((D, L), BF16),
        in_specs=[hbm] * 13,
        out_specs=hbm,
        scratch_shapes=[
            vmem((D, L), BF16), pltpu.SemaphoreType.DMA(()),
            vmem((D, L), BF16), *[vmem((D // 2, L), U32)] * 2, *[vmem((D, F), BF16)] * 3, vmem((5 * 64, 1024), U32),
            vmem((6, D, N), BF16), *[vmem((D,), BF16)] * 3, *[vmem((D, 128), F32)] * 4,
            vmem((CB, 1024), F32), vmem((CB, 18 * 128), F32),
            vmem((10, CB, 128), F32), vmem((7, CB, 128), F32), vmem((D, 4096), F32),
            vmem((4 * CB, 1024), F32), vmem((4 * CB, 1024), F32), vmem((D, L), F32),
            vmem((TOPC, L), F32), vmem((TOPC, D), F32), vmem((TOPC, F), F32),
            vmem((TOPC, CB), F32), vmem((CB, TOPC), F32),
        ],
        compiler_params=pltpu.CompilerParams(vmem_limit_bytes=100 * 1024 * 1024),
    )(A_u[0].T, A_A_re, A_A_im, A_B_re, A_B_im, A_C_re, A_C_im, A_log_dt, A_Dskip, B_w_r,
      B_w_gate, B_w_up, B_w_down.T)
    return out.T[None]
```
